```python
import jax
import jax.numpy as jnp

def _softmax(x, axis=-1):
    return jax.nn.softmax(x, axis=axis)
def _gelu(x):
    return jax.nn.gelu(x, approximate=True)
def _silu(x):
    return jax.nn.silu(x)
def _sigmoid(x):
    return jax.nn.sigmoid(x)
def _layernorm(x, axis=-1, eps=1e-5):
    m = jnp.mean(x, axis=axis, keepdims=True)
    v = jnp.var(x, axis=axis, keepdims=True)
    return (x - m) / jnp.sqrt(v + eps)
def _scatter_add(tgt, idx, src, axis=0):
    return tgt.at[idx].add(src)
def _segment_sum(src, seg, n):
    return jax.ops.segment_sum(src, seg, n)
class _Rng:
    def __init__(self, key):
        self._k = key
    def _next(self):
        self._k, sub = jax.random.split(self._k)
        return sub
    def normal(self, shape):
        return jax.random.normal(self._next(), shape, dtype=jnp.bfloat16)
    def randint(self, lo, hi, shape):
        return jax.random.randint(self._next(), shape, lo, hi, dtype=jnp.int32)
    def uniform(self, shape, lo=0.0, hi=1.0):
        return jax.random.uniform(self._next(), shape, jnp.bfloat16, lo, hi)
    def permutation(self, n):
        return jax.random.permutation(self._next(), n)


kernel_name = 'interleave_layers__sliding_block_cached__glu_gated_swiglu__decode'

def setup_inputs():
    _rng = _Rng(jax.random.key(int.from_bytes(__import__("os").urandom(4), "little")))
    _w = (lambda a: (lambda t: t.astype(jnp.bfloat16) if jnp.issubdtype(t.dtype, jnp.floating) else t)(jnp.asarray(a)))
    def _A_setup():
        B, Sq, D = 1, 1, 640
        Hq, Hkv, Sk, Dh = 32, 32, 32768, 192
        assert Hq % Hkv == 0, (Hq, Hkv)
        return {
            "x": _w((lambda *s: _rng.normal(s) * 0.05)(B, Sq, D)),
            "k_cache": _w((lambda *s: _rng.normal(s) * 0.05)(B, Hkv, Sk, Dh)),
            "v_cache": _w((lambda *s: _rng.normal(s) * 0.05)(B, Hkv, Sk, Dh)),
            "wq": _w((lambda *s: _rng.normal(s) * 0.05)(D, Hq * Dh) * (D ** -0.5)),
            "wo": _w((lambda *s: _rng.normal(s) * 0.05)(Hq * Dh, D) * ((Hq * Dh) ** -0.5)),
        }
    _A_in = _A_setup()

    def _B_setup():
        B, S, D, F = 1, 1, 640, 1536
        return {
            "x": _w((lambda *s: _rng.normal(s) * 0.05)(B, S, D)),
            "w1": _w((lambda *s: _rng.normal(s) * 0.05)(D, F) * (2.0 / D) ** 0.5),
            "w3": _w((lambda *s: _rng.normal(s) * 0.05)(D, F) * (2.0 / D) ** 0.5),
            "w2": _w((lambda *s: _rng.normal(s) * 0.05)(F, D) * (2.0 / F) ** 0.5),
        }
    _B_in = _B_setup()

    return {
        "A_x": _A_in["x"],
        "A_k_cache": _A_in["k_cache"],
        "A_v_cache": _A_in["v_cache"],
        "A_wq": _A_in["wq"],
        "A_wo": _A_in["wo"],
        "B_x": _B_in["x"],
        "B_w1": _B_in["w1"],
        "B_w3": _B_in["w3"],
        "B_w2": _B_in["w2"],
    }

def reference(A_x, A_k_cache, A_v_cache, A_wq, A_wo, B_x, B_w1, B_w3, B_w2):
    def _A_ref(x, k_cache, v_cache, wq, wo):
        B, Sq, D = x.shape
        Hq, Dh = 32, 192
        Hkv, Sk = k_cache.shape[1], k_cache.shape[2]
        W = min(4096, max(256, Sk // 4))
        rep = Hq // Hkv
        q = (lambda x, *d: x.transpose(*d))((x @ wq).reshape(B, Sq, Hq, Dh), 0, 2, 1, 3)
        k = jnp.repeat(k_cache[:, :, Sk - W:, :], rep, axis=1)
        v = jnp.repeat(v_cache[:, :, Sk - W:, :], rep, axis=1)
        scores = jnp.einsum("bhqd,bhkd->bhqk", q, k) * (Dh ** -0.5)
        p = _softmax(scores, axis=-1)
        o = jnp.einsum("bhqk,bhkd->bhqd", p, v)
        return (lambda x, *d: x.transpose(*d))(o, 0, 2, 1, 3).reshape(B, Sq, Hq * Dh) @ wo

    def _B_ref(x, w1, w3, w2):
        gate = jnp.einsum("bsd,df->bsf", x, w1)
        up = jnp.einsum("bsd,df->bsf", x, w3)
        h = _silu(gate) * up
        out = jnp.einsum("bsf,fd->bsd", h, w2)
        return out

    x = A_x
    x = x + _A_ref(_layernorm(x, axis=-1), A_k_cache, A_v_cache, A_wq, A_wo)
    x = x + _B_ref(_layernorm(x, axis=-1), B_w1, B_w3, B_w2)
    x = x + _A_ref(_layernorm(x, axis=-1), A_k_cache, A_v_cache, A_wq, A_wo)
    x = x + _B_ref(_layernorm(x, axis=-1), B_w1, B_w3, B_w2)
    return x
```

```python
import jax
import jax.numpy as jnp
from jax import lax
import jax.experimental.pallas as pl
import jax.experimental.pallas.tpu as pltpu

H, DH, D, F = 32, 192, 640, 1536
HD = H * DH
EPS = 1e-5
HC = 4
NCH = H // HC


def _ln(x):
    m = jnp.mean(x, axis=-1, keepdims=True)
    xc = x - m
    v = jnp.mean(xc * xc, axis=-1, keepdims=True)
    return xc * lax.rsqrt(v + EPS)


def _make_kernel(SK, W):
    def kernel(x_ref, k_hbm, v_hbm, wq_hbm, wo_hbm, w1_hbm, w3_hbm, w2_hbm, o_ref,
               kb, vb, wq, wo, w1, w3, w2, qs, os_, sk, sv, sw):
        def kcp(c):
            r = pl.ds(c * HC * DH, HC * DH)
            return pltpu.make_async_copy(k_hbm.at[r, pl.ds(SK - W, W)], kb.at[r, :], sk.at[c])

        def vcp(c):
            r = pl.ds(c * HC * DH, HC * DH)
            return pltpu.make_async_copy(v_hbm.at[r, pl.ds(SK - W, W)], vb.at[r, :], sv.at[c])

        wcp = [pltpu.make_async_copy(s, d, sw.at[i]) for i, (s, d) in enumerate(
            [(wq_hbm, wq), (wo_hbm, wo), (w1_hbm, w1), (w3_hbm, w3), (w2_hbm, w2)])]
        wcp[0].start()
        for c in range(NCH):
            kcp(c).start()
            vcp(c).start()
        for i in range(1, 5):
            wcp[i].start()

        row = lax.broadcasted_iota(jnp.int32, (8, 2 * DH), 0)
        col = lax.broadcasted_iota(jnp.int32, (8, 2 * DH), 1)
        diag = (col // DH) == row
        scale = DH ** -0.5

        x = jnp.broadcast_to(x_ref[...].astype(jnp.float32), (8, D))
        for layer in range(2):
            if layer == 0:
                wcp[0].wait()
            xn = _ln(x).astype(jnp.bfloat16)
            qs[...] = jnp.dot(xn, wq[...], preferred_element_type=jnp.float32)
            for c in range(NCH):
                if layer == 0:
                    kcp(c).wait()
                    vcp(c).wait()

                def pair(g, carry):
                    r0 = pl.multiple_of(g * (2 * DH), 128)
                    q = jnp.where(diag, qs[:, pl.ds(r0, 2 * DH)], 0.0).astype(jnp.bfloat16)
                    s = jnp.dot(q, kb[pl.ds(r0, 2 * DH), :], preferred_element_type=jnp.float32) * scale
                    m = jnp.max(s, axis=-1, keepdims=True)
                    p = jnp.exp(s - m)
                    l = jnp.sum(p, axis=-1, keepdims=True)
                    o = lax.dot_general(p.astype(jnp.bfloat16), vb[pl.ds(r0, 2 * DH), :],
                                        (((1,), (1,)), ((), ())), preferred_element_type=jnp.float32)
                    os_[:, pl.ds(r0, 2 * DH)] = jnp.where(diag, o / l, 0.0)
                    return carry
                lax.fori_loop(c * HC // 2, (c + 1) * HC // 2, pair, 0)
            if layer == 0:
                wcp[1].wait()
            a = jnp.dot(os_[...].astype(jnp.bfloat16), wo[...], preferred_element_type=jnp.float32)
            x = x + jnp.sum(a, axis=0, keepdims=True)
            if layer == 0:
                wcp[2].wait()
                wcp[3].wait()
            xn = _ln(x).astype(jnp.bfloat16)
            g = jnp.dot(xn, w1[...], preferred_element_type=jnp.float32)
            u = jnp.dot(xn, w3[...], preferred_element_type=jnp.float32)
            hh = (g * jax.nn.sigmoid(g) * u).astype(jnp.bfloat16)
            if layer == 0:
                wcp[4].wait()
            x = x + jnp.dot(hh, w2[...], preferred_element_type=jnp.float32)
        o_ref[...] = x[0:1].astype(o_ref.dtype)
    return kernel


@jax.jit
def pallas_interleave_layers__sliding_block_cached__glu_gated_swiglu__decode_kernel(
    A_x: jax.Array,
    A_k_cache: jax.Array,
    A_v_cache: jax.Array,
    A_wq: jax.Array,
    A_wo: jax.Array,
    B_x: jax.Array,
    B_w1: jax.Array,
    B_w3: jax.Array,
    B_w2: jax.Array,
):
    SK = A_k_cache.shape[2]
    W = min(4096, max(256, SK // 4))
    kt = jnp.swapaxes(A_k_cache, 2, 3).reshape(HD, SK)
    vt = jnp.swapaxes(A_v_cache, 2, 3).reshape(HD, SK)
    any_ = pl.BlockSpec(memory_space=pl.ANY)
    vm = pl.BlockSpec(memory_space=pltpu.VMEM)
    bf = jnp.bfloat16
    out = pl.pallas_call(
        _make_kernel(SK, W),
        out_shape=jax.ShapeDtypeStruct((1, D), A_x.dtype),
        in_specs=[vm] + [any_] * 7,
        out_specs=vm,
        scratch_shapes=[
            pltpu.VMEM((HD, W), bf), pltpu.VMEM((HD, W), bf),
            pltpu.VMEM((D, HD), bf), pltpu.VMEM((HD, D), bf),
            pltpu.VMEM((D, F), bf), pltpu.VMEM((D, F), bf), pltpu.VMEM((F, D), bf),
            pltpu.VMEM((8, HD), jnp.float32), pltpu.VMEM((8, HD), jnp.float32),
            pltpu.SemaphoreType.DMA((NCH,)), pltpu.SemaphoreType.DMA((NCH,)),
            pltpu.SemaphoreType.DMA((5,)),
        ],
        compiler_params=pltpu.CompilerParams(vmem_limit_bytes=124 * 1024 * 1024),
    )(A_x.reshape(1, D), kt, vt, A_wq, A_wo, B_w1, B_w3, B_w2)
    return out.reshape(1, 1, D)
```

```python
import math
import jax
import jax.numpy as jnp
from jax import lax
import jax.experimental.pallas as pl
import jax.experimental.pallas.tpu as pltpu

H, DH, D, F = 32, 192, 640, 1536
HD = H * DH
EPS = 1e-5
NA = HD // 8
AH = DH // 8
NP = H // 2
HC = 4
NCH = H // HC
NL = 2
JOBF = 1
AB = 4
f32, bf16, u32 = jnp.float32, jnp.bfloat16, jnp.uint32


def _ln(x):
    m = jnp.mean(x, axis=-1, keepdims=True)
    xc = x - m
    v = jnp.mean(xc * xc, axis=-1, keepdims=True)
    return xc * lax.rsqrt(v + EPS)


def _pack(x8):
    return pltpu.bitcast(jnp.concatenate([x8, x8], axis=0).astype(bf16), u32)


def _mm(lhs_u32, w_u32):
    lhs = pltpu.bitcast(lhs_u32, bf16)
    w = pltpu.bitcast(w_u32.reshape(64, 128), bf16)
    return jnp.dot(lhs, w, preferred_element_type=f32)[0:8]


def _make_kernel(SK, W):
    NC2 = W // 256
    R0 = (SK - W) // 16
    RW = W // 16
    qscale = DH ** -0.5 * math.log2(math.e)

    def kernel(x_ref, k_hbm, v_hbm, wq_hbm, wo_hbm, w1_hbm, w3_hbm, w2_hbm, o_ref,
               kb, vb, wqb, wob, w1, w3, w2,
               xs, lx, qraw, lq, sra, srb, pa, pb, ltab, oacc, ohalf, lo, woraw, xacc,
               sk, sv, sw):
        k32 = kb.bitcast(u32)
        wq32 = wqb.bitcast(u32)
        wo32 = wob.bitcast(u32)

        def kcp(c):
            r = pl.ds(c * (HC * AH), HC * AH)
            return pltpu.make_async_copy(k_hbm.at[r, pl.ds(R0, RW), :], kb.at[r], sk.at[c])

        def vcp(c):
            r = pl.ds(c * (HC * AH), HC * AH)
            return pltpu.make_async_copy(v_hbm.at[r, pl.ds(R0, RW), :], vb.at[r], sv.at[c])

        wcp = [pltpu.make_async_copy(s, d, sw.at[i]) for i, (s, d) in enumerate(
            [(wq_hbm, wqb), (wo_hbm, wob), (w1_hbm, w1), (w3_hbm, w3), (w2_hbm, w2)])]
        wcp[0].start()
        wcp[1].start()
        for c in range(NCH):
            kcp(c).start()
            vcp(c).start()
        for i in range(2, 5):
            wcp[i].start()

        xs[...] = jnp.broadcast_to(x_ref[...].astype(f32), (8, D))

        wcp[0].wait()

        def retile_wq(r, c):
            a = wq32[r, 0:24, 4:8, :]
            b = wq32[r, 24:48, 0:4, :]
            wq32[r, 0:24, 4:8, :] = b
            wq32[r, 24:48, 0:4, :] = a
            return c
        lax.fori_loop(0, D // 16, retile_wq, 0)
        wcp[1].wait()

        def retile_wo(rb, c):
            r = pl.ds(rb * 4, 4)
            vals = {(e, cc): wo32[r, 4 * (5 * e + cc):4 * (5 * e + cc) + 4, :]
                    for e in range(2) for cc in range(5)}
            for (e, cc), v in vals.items():
                wo32[r, 8 * cc + 4 * e:8 * cc + 4 * e + 4, :] = v
            return c
        lax.fori_loop(0, HD // 64, retile_wo, 0)

        sub = lax.broadcasted_iota(jnp.int32, (8, 128), 0)
        lane = lax.broadcasted_iota(jnp.int32, (8, 128), 1)

        def qproj_jobs(p):
            jobs = []
            for t in range(3):
                c = 3 * p + t
                slot = (c % 2) * 24 + c // 2
                for kk in range(5):
                    def job(t=t, kk=kk, slot=slot):
                        qraw[5 * t + kk] = _mm(lx[kk], wq32[8 * kk:8 * kk + 8, slot])
                    jobs.append(job)
            return jobs

        def run(jobs):
            for j in jobs:
                j()

        def qproj(p):
            run(qproj_jobs(p))

        def qprep():
            hmask = ((lane >> 3) & 1) == (sub >> 2)
            base = ((lane >> 4) << 3) + (lane & 7)
            for t in range(3):
                q = ((qraw[5 * t] + qraw[5 * t + 1]) + (qraw[5 * t + 2] + qraw[5 * t + 3])
                     + qraw[5 * t + 4]) * qscale
                for hf in range(2):
                    e = jnp.take_along_axis(q, base + 64 * hf, axis=1)
                    lq[2 * t + hf] = _pack(jnp.where(hmask, e, 0.0))

        def qk_jobs(h, par, sraw):
            jobs = []
            for b in range(3):
                a0 = h * AH + 8 * b
                for c2 in range(NC2):
                    def job(b=b, c2=c2, a0=a0):
                        sraw[NC2 * b + c2] = _mm(lq[3 * par + b], k32[pl.ds(a0, 8), 8 * c2:8 * c2 + 8, :])
                    jobs.append(job)
            return jobs

        def qk(h, par, sraw):
            run(qk_jobs(h, par, sraw))

        def softmax(h, sraw, pbuf):
            s = [sraw[c2] + sraw[NC2 + c2] + sraw[2 * NC2 + c2] for c2 in range(NC2)]
            mv = s[0]
            for c2 in range(1, NC2):
                mv = jnp.maximum(mv, s[c2])
            m = jnp.max(jnp.max(mv, axis=0, keepdims=True), axis=1, keepdims=True)
            sv_ = None
            for c2 in range(NC2):
                p = jnp.exp2(s[c2] - m)
                sv_ = p if sv_ is None else sv_ + p
                pbuf[2 * c2] = jnp.broadcast_to(p[0:1], (8, 128))
                pbuf[2 * c2 + 1] = jnp.broadcast_to(p[4:5], (8, 128))
            ltab[h] = sv_

        def pv(h, par, pbuf, jobs):
            nstep = (AH // AB) * NC2
            step = 0
            done = 0
            for a0 in range(0, AH, AB):
                accs = [None] * AB
                for c2 in range(NC2):
                    step += 1
                    upto = min(len(jobs), int(math.ceil(len(jobs) * step * JOBF / nstep)))
                    run(jobs[done:upto])
                    done = max(done, upto)
                    p0 = pbuf[2 * c2]
                    p1 = pbuf[2 * c2 + 1]
                    for i in range(AB):
                        v = vb[h * AH + a0 + i, 16 * c2:16 * c2 + 16, :].astype(f32)
                        t = v[0:8] * p0 + v[8:16] * p1
                        accs[i] = t if accs[i] is None else accs[i] + t
                for i in range(AB):
                    r = 8 * (a0 + i)
                    oacc[par, r:r + 8, :] = accs[i]

        def oreduce(h, par):
            l = jnp.sum(jnp.sum(ltab[h], axis=0, keepdims=True), axis=1, keepdims=True)
            inv = 4.0 / l
            o = []
            for r0 in (0, 64):
                tt = oacc[par, r0:r0 + 128, :].T
                o.append(jnp.broadcast_to(jnp.sum(tt, axis=0, keepdims=True) * inv, (8, 128)))
            if par == 0:
                lo[0] = _pack(o[0])
                ohalf[...] = pltpu.roll(o[1], 64, 1)
            else:
                lo[1] = _pack(jnp.where(lane < 64, ohalf[...], pltpu.roll(o[0], 64, 1)))
                lo[2] = _pack(o[1])

        def woproj_jobs(p):
            jobs = []
            for t in range(3):
                r0 = 24 * p + 8 * t
                for cc in range(5):
                    def job(t=t, cc=cc, r0=r0):
                        woraw[5 * t + cc] = _mm(lo[t], wo32[pl.ds(r0, 8), 8 * cc:8 * cc + 8, :])
                    jobs.append(job)
            return jobs

        def woproj(p):
            run(woproj_jobs(p))

        def woacc():
            for cc in range(5):
                xacc[cc] = xacc[cc] + (woraw[cc] + woraw[5 + cc] + woraw[10 + cc])

        def layer_body(layer, carry):
            first = layer == 0
            x = xs[...]
            xn = _ln(x)
            for kk in range(5):
                lx[kk] = _pack(xn[:, 128 * kk:128 * kk + 128])
            oacc[1] = jnp.zeros((DH, 128), f32)
            ohalf[...] = jnp.zeros_like(ohalf)
            lo[...] = jnp.zeros_like(lo)
            woraw[...] = jnp.zeros_like(woraw)
            xacc[...] = jnp.zeros_like(xacc)

            @pl.when(first)
            def _():
                kcp(0).wait()
            qproj(0)
            qprep()
            qk(0, 0, sra)
            qk(1, 1, srb)
            softmax(0, sra, pa)
            qproj(1)
            qprep()

            def body(h, c):
                @pl.when(first)
                def _():
                    @pl.when(h % HC == 0)
                    def _():
                        vcp(h // HC).wait()

                    @pl.when(jnp.logical_and((h + 2) % HC == 0, h + 2 < H))
                    def _():
                        kcp((h + 2) // HC).wait()
                i = h // 2
                hn = jnp.minimum(h + 2, H - 1)

                def even():
                    woacc()
                    softmax(h + 1, srb, pb)
                    oreduce(jnp.maximum(h - 1, 0), 1)
                    pv(h, 0, pa, qk_jobs(hn, 0, sra) + qproj_jobs(jnp.minimum(i + 2, NP - 1)))

                def odd():
                    softmax(h + 1, sra, pa)
                    pv(h, 1, pb, woproj_jobs(jnp.maximum(i - 1, 0)) + [lambda: oreduce(h - 1, 0)]
                       + qk_jobs(hn, 1, srb) + [qprep])
                lax.cond(h % 2 == 0, even, odd)
                return c
            lax.fori_loop(0, H, body, 0)
            woacc()
            oreduce(H - 1, 1)
            woproj(NP - 1)
            woacc()
            x = x + jnp.concatenate([xacc[cc] for cc in range(5)], axis=1)

            @pl.when(first)
            def _():
                wcp[2].wait()
                wcp[3].wait()
            xn = _ln(x).astype(bf16)
            g = jnp.dot(xn, w1[...], preferred_element_type=f32)
            u = jnp.dot(xn, w3[...], preferred_element_type=f32)
            hh = (g * jax.nn.sigmoid(g) * u).astype(bf16)

            @pl.when(first)
            def _():
                wcp[4].wait()
            xs[...] = x + jnp.dot(hh, w2[...], preferred_element_type=f32)
            return carry
        lax.fori_loop(0, NL, layer_body, 0)
        o_ref[...] = xs[0:1, :].astype(o_ref.dtype)
    return kernel


def _tile_linear(c):
    sk = c.shape[2]
    return (jnp.swapaxes(c, 2, 3).reshape(NA, 8, sk // 128, 128)
            .transpose(0, 2, 1, 3).reshape(NA, sk // 16, 128))


@jax.jit
def pallas_interleave_layers__sliding_block_cached__glu_gated_swiglu__decode_kernel(
    A_x: jax.Array,
    A_k_cache: jax.Array,
    A_v_cache: jax.Array,
    A_wq: jax.Array,
    A_wo: jax.Array,
    B_x: jax.Array,
    B_w1: jax.Array,
    B_w3: jax.Array,
    B_w2: jax.Array,
):
    SK = A_k_cache.shape[2]
    W = min(4096, max(256, SK // 4))
    kx = _tile_linear(A_k_cache)
    vx = _tile_linear(A_v_cache)
    wqz = (A_wq.reshape(D // 16, 2, 8, 24, 2, 128).transpose(0, 1, 3, 4, 2, 5)
           .reshape(D // 16, 48, 16, 128))
    woz = (A_wo.reshape(HD // 16, 2, 8, 5, 128).transpose(0, 1, 3, 2, 4)
           .reshape(HD // 16, 80, 128))
    any_ = pl.BlockSpec(memory_space=pl.ANY)
    vm = pl.BlockSpec(memory_space=pltpu.VMEM)
    nc2 = W // 256
    out = pl.pallas_call(
        _make_kernel(SK, W),
        out_shape=jax.ShapeDtypeStruct((1, D), A_x.dtype),
        in_specs=[vm] + [any_] * 7,
        out_specs=vm,
        scratch_shapes=[
            pltpu.VMEM((NA, W // 16, 128), bf16), pltpu.VMEM((NA, W // 16, 128), bf16),
            pltpu.VMEM((D // 16, 48, 16, 128), bf16), pltpu.VMEM((HD // 16, 80, 128), bf16),
            pltpu.VMEM((D, F), bf16), pltpu.VMEM((D, F), bf16), pltpu.VMEM((F, D), bf16),
            pltpu.VMEM((8, D), f32),
            pltpu.VMEM((5, 8, 128), u32),
            pltpu.VMEM((15, 8, 128), f32),
            pltpu.VMEM((6, 8, 128), u32),
            pltpu.VMEM((3 * nc2, 8, 128), f32),
            pltpu.VMEM((3 * nc2, 8, 128), f32),
            pltpu.VMEM((2 * nc2, 8, 128), f32),
            pltpu.VMEM((2 * nc2, 8, 128), f32),
            pltpu.VMEM((H + 1, 8, 128), f32),
            pltpu.VMEM((2, DH, 128), f32),
            pltpu.VMEM((8, 128), f32),
            pltpu.VMEM((3, 8, 128), u32),
            pltpu.VMEM((15, 8, 128), f32),
            pltpu.VMEM((5, 8, 128), f32),
            pltpu.SemaphoreType.DMA((NCH,)), pltpu.SemaphoreType.DMA((NCH,)),
            pltpu.SemaphoreType.DMA((5,)),
        ],
        compiler_params=pltpu.CompilerParams(vmem_limit_bytes=124 * 1024 * 1024),
    )(A_x.reshape(1, D), kx, vx, wqz, woz, B_w1, B_w3, B_w2)
    return out.reshape(1, 1, D)
```

```python
import math
import jax
import jax.numpy as jnp
from jax import lax
import jax.experimental.pallas as pl
import jax.experimental.pallas.tpu as pltpu

H, DH, D, F = 32, 192, 640, 1536
HD = H * DH
EPS = 1e-5
NA = HD // 8
AH = DH // 8
NP = H // 2
HC = 4
NCH = H // HC
NL = 2
JOBF = 1.1
DELAY = 0
ORG = 4
SMG = 2
SIDEF = 0.9
AB = 4
f32, bf16, u32 = jnp.float32, jnp.bfloat16, jnp.uint32


def _ln(x):
    m = jnp.mean(x, axis=-1, keepdims=True)
    xc = x - m
    v = jnp.mean(xc * xc, axis=-1, keepdims=True)
    return xc * lax.rsqrt(v + EPS)


def _pack(x8):
    return pltpu.bitcast(jnp.concatenate([x8, x8], axis=0).astype(bf16), u32)


def _mm(lhs_u32, w_u32):
    lhs = pltpu.bitcast(lhs_u32, bf16)
    w = pltpu.bitcast(w_u32.reshape(64, 128), bf16)
    return jnp.dot(lhs, w, preferred_element_type=f32)[0:8]


def _st(ref, idx, val):
    def go():
        ref[idx] = val
    return go


def _tree(op, xs):
    xs = list(xs)
    while len(xs) > 1:
        xs = [op(xs[i], xs[i + 1]) if i + 1 < len(xs) else xs[i] for i in range(0, len(xs), 2)]
    return xs[0]


def _merge(main, side):
    out = []
    k = 0
    for n, j in enumerate(main):
        while k < len(side) and k * SIDEF * len(main) <= n * len(side):
            out.append(side[k])
            k += 1
        out.append(j)
    return out + side[k:]


def _make_kernel(SK, W):
    NC2 = W // 256
    R0 = (SK - W) // 16
    RW = W // 16
    qscale = DH ** -0.5 * math.log2(math.e)

    def kernel(x_ref, k_hbm, v_hbm, wq_hbm, wo_hbm, w1_hbm, w3_hbm, w2_hbm, o_ref,
               kb, vb, wqb, wob, w1, w3, w2,
               xs, lx, qraw, lq, sra, srb, pa, pb, st, oacc, oscl, rsum, ohold, lo, woraw, xacc,
               sk, sv, sw):
        sr, pp = (sra, srb), (pa, pb)
        k32 = kb.bitcast(u32)
        wq32 = wqb.bitcast(u32)
        wo32 = wob.bitcast(u32)

        def kcp(c):
            r = pl.ds(c * (HC * AH), HC * AH)
            return pltpu.make_async_copy(k_hbm.at[r, pl.ds(R0, RW), :], kb.at[r], sk.at[c])

        def vcp(c):
            r = pl.ds(c * (HC * AH), HC * AH)
            return pltpu.make_async_copy(v_hbm.at[r, pl.ds(R0, RW), :], vb.at[r], sv.at[c])

        wcp = [pltpu.make_async_copy(s, d, sw.at[i]) for i, (s, d) in enumerate(
            [(wq_hbm, wqb), (wo_hbm, wob), (w1_hbm, w1), (w3_hbm, w3), (w2_hbm, w2)])]
        wcp[0].start()
        wcp[1].start()
        for c in range(NCH):
            kcp(c).start()
            vcp(c).start()
        for i in range(2, 5):
            wcp[i].start()

        xs[...] = jnp.broadcast_to(x_ref[...].astype(f32), (8, D))

        wcp[0].wait()

        def retile_wq(r, c):
            a = wq32[r, 0:24, 4:8, :]
            b = wq32[r, 24:48, 0:4, :]
            wq32[r, 0:24, 4:8, :] = b
            wq32[r, 24:48, 0:4, :] = a
            return c
        lax.fori_loop(0, D // 16, retile_wq, 0)
        wcp[1].wait()

        def retile_wo(rb, c):
            r = pl.ds(rb * 4, 4)
            vals = {(e, cc): wo32[r, 4 * (5 * e + cc):4 * (5 * e + cc) + 4, :]
                    for e in range(2) for cc in range(5)}
            for (e, cc), v in vals.items():
                wo32[r, 8 * cc + 4 * e:8 * cc + 4 * e + 4, :] = v
            return c
        lax.fori_loop(0, HD // 64, retile_wo, 0)

        sub = lax.broadcasted_iota(jnp.int32, (8, 128), 0)
        lane = lax.broadcasted_iota(jnp.int32, (8, 128), 1)

        def qproj_jobs(p):
            jobs = []
            for t in range(3):
                c = 3 * p + t
                slot = (c & 1) * 24 + (c >> 1)
                for kk in range(5):
                    def job(t=t, kk=kk, slot=slot):
                        return _st(qraw, 5 * t + kk, _mm(lx[kk], wq32[8 * kk:8 * kk + 8, slot]))
                    jobs.append(job)
            return jobs

        def run(jobs):
            for j in jobs:
                r = j()
                if r is not None:
                    r()

        def qproj(p):
            run(qproj_jobs(p))

        def qprep():
            valid = ((lane >> 3) & 1) == ((sub >> 1) & 1)
            base = ((lane >> 4) << 3) + (lane & 7)
            for t in range(3):
                q = ((qraw[5 * t] + qraw[5 * t + 1]) + (qraw[5 * t + 2] + qraw[5 * t + 3])
                     + qraw[5 * t + 4]) * qscale
                qp = pltpu.bitcast(_pack(q), jnp.int32)
                for hf in range(2):
                    z = jnp.where((lane >> 6) == hf, qp, 0)
                    idx = jnp.where(valid, base + 64 * hf, 64 * (1 - hf))
                    lq[2 * t + hf] = pltpu.bitcast(jnp.take_along_axis(z, idx, axis=1), u32)

        def qk_jobs(h, par):
            jobs = []
            sraw = sr[par]
            for b in range(3):
                a0 = h * AH + 8 * b
                for c2 in range(NC2):
                    def job(b=b, c2=c2, a0=a0):
                        return _st(sraw, NC2 * b + c2,
                                   _mm(lq[3 * par + b], k32[pl.ds(a0, 8), 8 * c2:8 * c2 + 8, :]))
                    jobs.append(job)
            return jobs

        def qk(h, par):
            run(qk_jobs(h, par))

        def bc(x):
            return jnp.broadcast_to(x, (8, 128))

        def sm1_jobs(par):
            sraw, pbuf = sr[par], pp[par]
            env = {}

            def head():
                s = [sraw[c2] + sraw[NC2 + c2] + sraw[2 * NC2 + c2] for c2 in range(NC2)]
                mv = _tree(jnp.maximum, s)
                mv = jnp.maximum(mv, pltpu.roll(mv, 4, 0))
                st[par, 0] = mv
                env["s"], env["mv"], env["ls"] = s, mv, None

            def mk(c0):
                def job():
                    ps = []
                    for c2 in range(c0, c0 + SMG):
                        p = jnp.exp2(env["s"][c2] - env["mv"])
                        ps.append(p)
                        pbuf[2 * c2] = bc(p[0:1])
                        pbuf[2 * c2 + 1] = bc(p[4:5])
                    t = _tree(jnp.add, ps)
                    env["ls"] = t if env["ls"] is None else env["ls"] + t
                    if c0 + SMG == NC2:
                        st[par, 1] = env["ls"] + pltpu.roll(env["ls"], 4, 0)
                return job
            return [head] + [mk(c0) for c0 in range(0, NC2, SMG)]

        def xmax(par):
            st[par, 2] = bc(jnp.max(st[par, 0], axis=1, keepdims=True))

        def scale_jobs(par):
            env = {}

            def head():
                env["w"] = jnp.exp2(st[par, 0] - st[par, 2])
                oscl[par, AH] = env["w"] * st[par, 1]

            def mk(g):
                def job():
                    for a in range(ORG * g, ORG * g + ORG):
                        oscl[par, a] = oacc[par, 8 * a:8 * a + 8, :] * env["w"]
                return job
            return [head] + [mk(g) for g in range(AH // ORG)]

        def xsum(par):
            for a in range(AH + 1):
                rsum[par, a] = bc(jnp.sum(oscl[par, a], axis=1, keepdims=True))

        def pv(h, par, jobs):
            pbuf = pp[par]
            nstep = (AH // AB) * NC2
            step = 0
            done = 0
            pend = []
            for a0 in range(0, AH, AB):
                accs = [None] * AB
                for c2 in range(NC2):
                    step += 1
                    upto = min(len(jobs), int(math.ceil(len(jobs) * step * JOBF / nstep)))
                    for j in jobs[done:upto]:
                        r = j()
                        if r is not None:
                            pend.append((step + DELAY, r))
                    done = max(done, upto)
                    while pend and pend[0][0] <= step:
                        pend.pop(0)[1]()
                    p0 = pbuf[2 * c2]
                    p1 = pbuf[2 * c2 + 1]
                    for i in range(AB):
                        v = vb[h * AH + a0 + i, 16 * c2:16 * c2 + 16, :].astype(f32)
                        t = v[0:8] * p0 + v[8:16] * p1
                        accs[i] = t if accs[i] is None else accs[i] + t
                for i in range(AB):
                    r = 8 * (a0 + i)
                    oacc[par, r:r + 8, :] = accs[i]
            for _, r in pend:
                r()

        def or2(par):
            def sel(bit, x, y):
                return jnp.where(((lane >> bit) & 1) == 0, x, y)
            inv = 1.0 / rsum[par, AH]
            vals = []
            for g in range(3):
                r = [rsum[par, 8 * g + k] for k in range(8)]
                r = [sel(3, r[2 * k], r[2 * k + 1]) for k in range(4)]
                r = [sel(4, r[2 * k], r[2 * k + 1]) for k in range(2)]
                vals.append(sel(5, r[0], r[1]))
            if par == 0:
                ohold[0] = sel(6, vals[0], vals[1]) * inv
                ohold[1] = vals[2] * inv
            else:
                diag = (lane & 7) == sub
                lo[0] = _pack(jnp.where(diag, ohold[0], 0.0))
                lo[1] = _pack(jnp.where(diag, sel(6, ohold[1], vals[0] * inv), 0.0))
                lo[2] = _pack(jnp.where(diag, sel(6, vals[1], vals[2]) * inv, 0.0))

        def woproj_jobs(p):
            jobs = []
            for t in range(3):
                r0 = 24 * p + 8 * t
                for cc in range(5):
                    def job(t=t, cc=cc, r0=r0):
                        return _st(woraw, 5 * t + cc,
                                   _mm(lo[t], wo32[pl.ds(r0, 8), 8 * cc:8 * cc + 8, :]))
                    jobs.append(job)
            return jobs

        def woproj(p):
            run(woproj_jobs(p))

        def woacc():
            for cc in range(5):
                xacc[cc] = xacc[cc] + (woraw[cc] + woraw[5 + cc] + woraw[10 + cc])

        def layer_body(layer, carry):
            first = layer == 0
            x = xs[...]
            xn = _ln(x)
            for kk in range(5):
                lx[kk] = _pack(xn[:, 128 * kk:128 * kk + 128])
            one = jnp.ones((8, 128), f32)
            oacc[1] = jnp.zeros((DH, 128), f32)
            oscl[0, 0:AH] = jnp.zeros((AH, 8, 128), f32)
            oscl[0, AH] = one
            rsum[1, 0:AH] = jnp.zeros((AH, 8, 128), f32)
            rsum[1, AH] = one
            st[...] = jnp.ones_like(st)
            ohold[...] = jnp.zeros_like(ohold)
            woraw[...] = jnp.zeros_like(woraw)
            xacc[...] = jnp.zeros_like(xacc)

            @pl.when(first)
            def _():
                kcp(0).wait()
            qproj(0)
            qprep()
            qk(0, 0)
            qk(1, 1)
            run(sm1_jobs(0))
            qproj(1)
            qprep()

            def body(h, c):
                @pl.when(first)
                def _():
                    @pl.when((h & 3) == 0)
                    def _():
                        vcp(h >> 2).wait()

                    @pl.when(jnp.logical_and((h & 3) == 2, h + 2 < H))
                    def _():
                        kcp((h + 2) >> 2).wait()
                i = h >> 1
                hn = jnp.minimum(h + 2, H - 1)

                def side(par):
                    return ([lambda: or2(1 - par), lambda: xsum(par), lambda: xmax(par)]
                            + scale_jobs(1 - par) + sm1_jobs(1 - par))

                def even():
                    mx = qk_jobs(hn, 0) + qproj_jobs(jnp.minimum(i + 2, NP - 1))
                    pv(h, 0, _merge(mx, [woacc] + side(0)))

                def odd():
                    mx = woproj_jobs(jnp.maximum(i - 2, 0)) + qk_jobs(hn, 1)
                    pv(h, 1, _merge(mx, side(1)) + [qprep])
                lax.cond((h & 1) == 0, even, odd)
                return c
            lax.fori_loop(0, H, body, 0)
            woacc()
            or2(1)
            woproj(NP - 2)
            woacc()
            xsum(0)
            run(scale_jobs(1))
            xsum(1)
            or2(0)
            or2(1)
            woproj(NP - 1)
            woacc()
            x = x + jnp.sum(jnp.concatenate([xacc[cc] for cc in range(5)], axis=1), axis=0, keepdims=True)

            @pl.when(first)
            def _():
                wcp[2].wait()
                wcp[3].wait()
            xn = _ln(x).astype(bf16)
            g = jnp.dot(xn, w1[...], preferred_element_type=f32)
            u = jnp.dot(xn, w3[...], preferred_element_type=f32)
            hh = (g * jax.nn.sigmoid(g) * u).astype(bf16)

            @pl.when(first)
            def _():
                wcp[4].wait()
            xs[...] = x + jnp.dot(hh, w2[...], preferred_element_type=f32)
            return carry
        lax.fori_loop(0, NL, layer_body, 0)
        o_ref[...] = xs[0:1, :].astype(o_ref.dtype)
    return kernel


def _tile_linear(c):
    sk = c.shape[2]
    return (jnp.swapaxes(c, 2, 3).reshape(NA, 8, sk // 128, 128)
            .transpose(0, 2, 1, 3).reshape(NA, sk // 16, 128))


@jax.jit
def pallas_interleave_layers__sliding_block_cached__glu_gated_swiglu__decode_kernel(
    A_x: jax.Array,
    A_k_cache: jax.Array,
    A_v_cache: jax.Array,
    A_wq: jax.Array,
    A_wo: jax.Array,
    B_x: jax.Array,
    B_w1: jax.Array,
    B_w3: jax.Array,
    B_w2: jax.Array,
):
    SK = A_k_cache.shape[2]
    W = min(4096, max(256, SK // 4))
    kx = _tile_linear(A_k_cache)
    vx = _tile_linear(A_v_cache)
    wqz = (A_wq.reshape(D // 16, 2, 8, 24, 2, 128).transpose(0, 1, 3, 4, 2, 5)
           .reshape(D // 16, 48, 16, 128))
    woz = (A_wo.reshape(HD // 16, 2, 8, 5, 128).transpose(0, 1, 3, 2, 4)
           .reshape(HD // 16, 80, 128))
    any_ = pl.BlockSpec(memory_space=pl.ANY)
    vm = pl.BlockSpec(memory_space=pltpu.VMEM)
    nc2 = W // 256
    out = pl.pallas_call(
        _make_kernel(SK, W),
        out_shape=jax.ShapeDtypeStruct((1, D), A_x.dtype),
        in_specs=[vm] + [any_] * 7,
        out_specs=vm,
        scratch_shapes=[
            pltpu.VMEM((NA, W // 16, 128), bf16), pltpu.VMEM((NA, W // 16, 128), bf16),
            pltpu.VMEM((D // 16, 48, 16, 128), bf16), pltpu.VMEM((HD // 16, 80, 128), bf16),
            pltpu.VMEM((D, F), bf16), pltpu.VMEM((D, F), bf16), pltpu.VMEM((F, D), bf16),
            pltpu.VMEM((8, D), f32),
            pltpu.VMEM((5, 8, 128), u32),
            pltpu.VMEM((15, 8, 128), f32),
            pltpu.VMEM((6, 8, 128), u32),
            pltpu.VMEM((3 * nc2, 8, 128), f32),
            pltpu.VMEM((3 * nc2, 8, 128), f32),
            pltpu.VMEM((2 * nc2, 8, 128), f32),
            pltpu.VMEM((2 * nc2, 8, 128), f32),
            pltpu.VMEM((2, 3, 8, 128), f32),
            pltpu.VMEM((2, DH, 128), f32),
            pltpu.VMEM((2, AH + 1, 8, 128), f32),
            pltpu.VMEM((2, AH + 1, 8, 128), f32),
            pltpu.VMEM((2, 8, 128), f32),
            pltpu.VMEM((3, 8, 128), u32),
            pltpu.VMEM((15, 8, 128), f32),
            pltpu.VMEM((5, 8, 128), f32),
            pltpu.SemaphoreType.DMA((NCH,)), pltpu.SemaphoreType.DMA((NCH,)),
            pltpu.SemaphoreType.DMA((5,)),
        ],
        compiler_params=pltpu.CompilerParams(vmem_limit_bytes=124 * 1024 * 1024),
    )(A_x.reshape(1, D), kx, vx, wqz, woz, B_w1, B_w3, B_w2)
    return out.reshape(1, 1, D)
```

```python
import math
import jax
import jax.numpy as jnp
from jax import lax
import jax.experimental.pallas as pl
import jax.experimental.pallas.tpu as pltpu

H, DH, D, F = 32, 192, 640, 1536
HD = H * DH
EPS = 1e-5
NA = HD // 8
AH = DH // 8
NP = H // 2
HC = 4
NCH = H // HC
NL = 2
NREP = 1
MX0 = 0.35
MX1 = 1.1
AB = 4
SMG = 4
SMH = 8
ORG = 4
DYNP = 0
SMB0 = 0.1
SMB1 = 0.8
f32, bf16, u32 = jnp.float32, jnp.bfloat16, jnp.uint32


def _ln(x):
    m = jnp.mean(x, axis=-1, keepdims=True)
    xc = x - m
    v = jnp.mean(xc * xc, axis=-1, keepdims=True)
    return xc * lax.rsqrt(v + EPS)


def _pack(x8):
    return pltpu.bitcast(jnp.concatenate([x8, x8], axis=0).astype(bf16), u32)


def _mm(lhs_u32, w_u32, half=0):
    lhs = pltpu.bitcast(lhs_u32, bf16)
    w = pltpu.bitcast(w_u32.reshape(64, 128), bf16)
    r = jnp.dot(lhs, w, preferred_element_type=f32)
    return r if half is None else r[8 * half:8 * half + 8]


def _bc(x):
    return jnp.broadcast_to(x, (8, 128))


def _tree(op, xs):
    xs = list(xs)
    while len(xs) > 1:
        xs = [op(xs[i], xs[i + 1]) if i + 1 < len(xs) else xs[i] for i in range(0, len(xs), 2)]
    return xs[0]


def _run(jobs):
    for j in jobs:
        j()


def _weave(main, extra, lo, hi):
    out, k = [], 0
    for n, j in enumerate(main):
        while k < len(extra) and lo * len(main) + k * (hi - lo) * len(main) / len(extra) <= n:
            out.append(extra[k])
            k += 1
        out.append(j)
    return out + list(extra[k:])


def _make_kernel(SK, W):
    NC = W // 128
    NC2 = NC // 2
    R0 = (SK - W) // 16
    RW = W // 16
    qscale = DH ** -0.5 * math.log2(math.e)

    def kernel(x_ref, k_hbm, v_hbm, wq_hbm, wo_hbm, w1_hbm, w3_hbm, w2_hbm, o_ref,
               kb, vb, wqb, wob, w1, w3, w2,
               xs, lx, qraw, lq, sraw, pbuf, st, oacc, oscl, rsum, lo, woraw, xacc,
               sk, sv, sw):
        k32 = kb.bitcast(u32)
        wq32 = wqb.bitcast(u32)
        wo32 = wob.bitcast(u32)

        def kcp(c):
            r = pl.ds(c * (HC * AH // 2), HC * AH // 2)
            return pltpu.make_async_copy(k_hbm.at[r, :, pl.ds(R0 // 16, NC2)], kb.at[r], sk.at[c])

        def kready(c):
            kcp(c).wait()

            def swap(r, carry):
                a = k32[r, 0, :, 4:8, :]
                b = k32[r, 1, :, 0:4, :]
                k32[r, 0, :, 4:8, :] = b
                k32[r, 1, :, 0:4, :] = a
                return carry
            lax.fori_loop(c * (HC * AH // 2), (c + 1) * (HC * AH // 2), swap, 0)

        def vcp(c):
            r = pl.ds(c * (HC * AH), HC * AH)
            return pltpu.make_async_copy(v_hbm.at[r, pl.ds(R0, RW), :], vb.at[r], sv.at[c])

        wcp = [pltpu.make_async_copy(s, d, sw.at[i]) for i, (s, d) in enumerate(
            [(wq_hbm, wqb), (wo_hbm, wob), (w1_hbm, w1), (w3_hbm, w3), (w2_hbm, w2)])]
        wcp[0].start()
        wcp[1].start()
        for c in range(NCH):
            kcp(c).start()
            vcp(c).start()
        for i in range(2, 5):
            wcp[i].start()

        xs[...] = jnp.broadcast_to(x_ref[...].astype(f32), (8, D))

        wcp[0].wait()

        def retile_wq(r, c):
            a = wq32[r, 0:24, 4:8, :]
            b = wq32[r, 24:48, 0:4, :]
            wq32[r, 0:24, 4:8, :] = b
            wq32[r, 24:48, 0:4, :] = a
            return c
        lax.fori_loop(0, D // 16, retile_wq, 0)
        wcp[1].wait()

        def retile_wo(rb, c):
            r = pl.ds(rb * 4, 4)
            vals = {(e, cc): wo32[r, 4 * (5 * e + cc):4 * (5 * e + cc) + 4, :]
                    for e in range(2) for cc in range(5)}
            for (e, cc), v in vals.items():
                wo32[r, 8 * cc + 4 * e:8 * cc + 4 * e + 4, :] = v
            return c
        lax.fori_loop(0, HD // 64, retile_wo, 0)

        sub = lax.broadcasted_iota(jnp.int32, (8, 128), 0)
        lane = lax.broadcasted_iota(jnp.int32, (8, 128), 1)

        def qproj_jobs(p, q):
            jobs = []
            for t in range(3):
                c = 3 * p + t
                slot = (c & 1) * 24 + (c >> 1)
                for kk in range(5):
                    def job(t=t, kk=kk, slot=slot):
                        qraw[q, 5 * t + kk] = _mm(lx[kk], wq32[8 * kk:8 * kk + 8, slot])
                    jobs.append(job)
            return jobs

        def qprep(q):
            for t in range(3):
                qv = _tree(jnp.add, [qraw[q, 5 * t + kk] for kk in range(5)]) * qscale
                qp = _pack(qv)
                if t == 1:
                    qp = jnp.where((lane >> 6) == (sub >> 2), qp, jnp.uint32(0))
                lq[q, t] = qp

        def qk_jobs(p, q):
            jobs = []
            for t in range(3):
                r0 = p * AH + 8 * t
                for c in range(NC):
                    def job(t=t, c=c, r0=r0):
                        r = _mm(lq[q, t], k32[pl.ds(r0, 8), c & 1, c >> 1], None)
                        if t < 2:
                            sraw[q, 0, t, c] = r[0:8]
                        if t > 0:
                            sraw[q, 1, t - 1, c] = r[8:16] if t == 1 else r[0:8]
                    jobs.append(job)
            return jobs

        def sm1_jobs(q, e):
            env = {"mv": None, "ls": None}

            def mk1(c0):
                def job():
                    s = []
                    for c in range(c0, c0 + SMH):
                        s.append(sraw[q, e, 0, c] + sraw[q, e, 1, c])
                        pbuf[e, c] = s[-1]
                    m = _tree(jnp.maximum, s)
                    env["mv"] = m if env["mv"] is None else jnp.maximum(env["mv"], m)
                    if c0 + SMH == NC:
                        st[q, e, 0] = env["mv"]
                return job

            def mk2(c0):
                def job():
                    ps = []
                    for c in range(c0, c0 + SMG):
                        ps.append(jnp.exp2(pbuf[e, c] - env["mv"]))
                        pbuf[e, c] = ps[-1]
                    t = _tree(jnp.add, ps)
                    env["ls"] = t if env["ls"] is None else env["ls"] + t
                    if c0 + SMG == NC:
                        st[q, e, 1] = env["ls"]
                return job
            return [mk1(c0) for c0 in range(0, NC, SMH)], [mk2(c0) for c0 in range(0, NC, SMG)]

        def pv_jobs(p, q, e, z):
            jobs = []
            for a0 in range(0, AH, AB):
                accs = [None] * AB
                for c2 in range(NC2):
                    def job(a0=a0, c2=c2, accs=accs):
                        p0 = pbuf[e, z + 2 * c2]
                        p1 = pbuf[e, z + 2 * c2 + 1]
                        for i in range(AB):
                            a = p * (2 * AH) + (e * AH + a0 + i)
                            v = vb[a, 16 * c2:16 * c2 + 16, :].astype(f32)
                            t = v[0:8] * p0 + v[8:16] * p1
                            accs[i] = t if accs[i] is None else accs[i] + t
                        if c2 == NC2 - 1:
                            for i in range(AB):
                                oacc[q, e, a0 + i] = accs[i]
                    jobs.append(job)
            return jobs

        def xmax(q):
            for e in range(2):
                st[q, e, 2] = _bc(jnp.max(st[q, e, 0], axis=1, keepdims=True))

        def scale_jobs(q, e):
            env = {}

            def head():
                env["w"] = jnp.exp2(st[q, e, 0] - st[q, e, 2])
                oscl[q, e, AH] = env["w"] * st[q, e, 1]

            def mk(g):
                def job():
                    for a in range(ORG * g, ORG * g + ORG):
                        oscl[q, e, a] = oacc[q, e, a] * env["w"]
                return job
            return [head] + [mk(g) for g in range(AH // ORG)]

        def xsum(q):
            for e in range(2):
                for a in range(AH + 1):
                    rsum[q, e, a] = _bc(jnp.sum(oscl[q, e, a], axis=1, keepdims=True))

        def or2(q):
            def sel(bit, x, y):
                return jnp.where(((lane >> bit) & 1) == 0, x, y)
            vals = []
            for e in range(2):
                for g in range(3):
                    r = [rsum[q, e, 8 * g + k] for k in range(8)]
                    r = [sel(3, r[2 * k], r[2 * k + 1]) for k in range(4)]
                    r = [sel(4, r[2 * k], r[2 * k + 1]) for k in range(2)]
                    vals.append(sel(5, r[0], r[1]))
            inv0 = 1.0 / rsum[q, 0, AH]
            inv1 = 1.0 / rsum[q, 1, AH]
            invs = [inv0, sel(6, inv0, inv1), inv1]
            diag = (lane & 7) == sub
            for t in range(3):
                o = sel(6, vals[2 * t], vals[2 * t + 1]) * invs[t]
                lo[q, t] = _pack(jnp.where(diag, o, 0.0))

        def woproj_jobs(p, q):
            jobs = []
            for t in range(3):
                r0 = 24 * p + 8 * t
                for cc in range(5):
                    def job(t=t, cc=cc, r0=r0):
                        woraw[q, 5 * t + cc] = _mm(lo[q, t], wo32[pl.ds(r0, 8), 8 * cc:8 * cc + 8, :])
                    jobs.append(job)
            return jobs

        def woacc(q, valid=None):
            for cc in range(5):
                t = woraw[q, cc] + woraw[q, 5 + cc] + woraw[q, 10 + cc]
                if valid is not None:
                    t = jnp.where(valid, t, 0.0)
                xacc[cc] = xacc[cc] + t

        def block(b, q):
            nq = 1 - q
            z = (b >> 10) if DYNP else 0
            mx = (qk_jobs(jnp.minimum(b + 1, NP - 1), nq)
                  + qproj_jobs(jnp.minimum(b + 3, NP - 1), nq)
                  + woproj_jobs(jnp.maximum(b - 5, 0), nq))
            sc0, sc1 = scale_jobs(q, 0), scale_jobs(q, 1)
            (sa1, sa2), (sb1, sb2) = sm1_jobs(q, 0), sm1_jobs(q, 1)
            pa, pb = pv_jobs(b, q, 0, z), pv_jobs(b, q, 1, z)
            start = ([sc0[0], sc1[0]] + sa1 + [lambda: or2(q), sa2[0], lambda: woacc(q, b >= 6), sa2[1]])
            first = _weave(pa[:NC2], sa2[2:], 0.0, 1.0 - 2.0 * SMG / NC)
            first = first[:-1] + sc0[1:2] + first[-1:]
            rest = _weave(pa[NC2:], sc0[2:], 0.0, 1.0)
            rest = _weave(rest, sb1 + sb2, SMB0, SMB1)
            vb_ = _weave(_weave(pb, sc1[1:], 0.0, 1.0), [lambda: qprep(q)], 0.3, 0.4)
            valu = start + first + rest + vb_
            xl = [lambda: xmax(nq), lambda: xsum(nq)]
            _run(xl + _weave(valu, mx, MX0, MX1))

        def layer_body(layer, carry):
            first = layer == 0
            x = xs[...]
            xn = _ln(x)
            for kk in range(5):
                lx[kk] = _pack(xn[:, 128 * kk:128 * kk + 128])
            xacc[...] = jnp.zeros_like(xacc)

            @pl.when(first)
            def _():
                kready(0)
            _run(qproj_jobs(0, 0))
            qprep(0)
            _run(qproj_jobs(1, 1))
            qprep(1)
            _run(qproj_jobs(2, 0))
            _run(qk_jobs(0, 0))

            def body(b0, c):
                b = b0 & 15

                @pl.when(jnp.logical_and(first, b0 < NP))
                def _():
                    @pl.when((b & 1) == 0)
                    def _():
                        vcp(b >> 1).wait()

                    @pl.when(jnp.logical_and((b & 1) == 1, b < NP - 1))
                    def _():
                        kready((b + 1) >> 1)
                lax.cond((b & 1) == 0, lambda: block(b, 0), lambda: block(b, 1))
                return c
            lax.fori_loop(0, NP * NREP, body, 0)
            for b in range(NP, NP + 6):
                q = b & 1
                if b - 1 < NP:
                    xmax(1 - q)
                if b - 2 < NP:
                    _run(scale_jobs(q, 0) + scale_jobs(q, 1))
                if b - 3 < NP:
                    xsum(1 - q)
                if b - 4 < NP:
                    or2(q)
                if b - 5 < NP:
                    _run(woproj_jobs(b - 5, 1 - q))
                woacc(q)
            x = x + jnp.sum(jnp.concatenate([xacc[cc] for cc in range(5)], axis=1), axis=0, keepdims=True)

            @pl.when(first)
            def _():
                wcp[2].wait()
                wcp[3].wait()
            xn = _ln(x).astype(bf16)
            g = jnp.dot(xn, w1[...], preferred_element_type=f32)
            u = jnp.dot(xn, w3[...], preferred_element_type=f32)
            hh = (g * jax.nn.sigmoid(g) * u).astype(bf16)

            @pl.when(first)
            def _():
                wcp[4].wait()
            xs[...] = x + jnp.dot(hh, w2[...], preferred_element_type=f32)
            return carry
        lax.fori_loop(0, NL, layer_body, 0)
        o_ref[...] = xs[0:1, :].astype(o_ref.dtype)
    return kernel


def _tile_linear(c):
    sk = c.shape[2]
    return (jnp.swapaxes(c, 2, 3).reshape(NA, 8, sk // 128, 128)
            .transpose(0, 2, 1, 3).reshape(NA, sk // 16, 128))


@jax.jit
def pallas_interleave_layers__sliding_block_cached__glu_gated_swiglu__decode_kernel(
    A_x: jax.Array,
    A_k_cache: jax.Array,
    A_v_cache: jax.Array,
    A_wq: jax.Array,
    A_wo: jax.Array,
    B_x: jax.Array,
    B_w1: jax.Array,
    B_w3: jax.Array,
    B_w2: jax.Array,
):
    SK = A_k_cache.shape[2]
    W = min(4096, max(256, SK // 4))
    kx = _tile_linear(A_k_cache).reshape(NA // 2, 2, SK // 256, 16, 128)
    vx = _tile_linear(A_v_cache)
    wqz = (A_wq.reshape(D // 16, 2, 8, 24, 2, 128).transpose(0, 1, 3, 4, 2, 5)
           .reshape(D // 16, 48, 16, 128))
    woz = (A_wo.reshape(HD // 16, 2, 8, 5, 128).transpose(0, 1, 3, 2, 4)
           .reshape(HD // 16, 80, 128))
    any_ = pl.BlockSpec(memory_space=pl.ANY)
    vm = pl.BlockSpec(memory_space=pltpu.VMEM)
    nc2 = W // 256
    out = pl.pallas_call(
        _make_kernel(SK, W),
        out_shape=jax.ShapeDtypeStruct((1, D), A_x.dtype),
        in_specs=[vm] + [any_] * 7,
        out_specs=vm,
        scratch_shapes=[
            pltpu.VMEM((NA // 2, 2, nc2, 16, 128), bf16), pltpu.VMEM((NA, W // 16, 128), bf16),
            pltpu.VMEM((D // 16, 48, 16, 128), bf16), pltpu.VMEM((HD // 16, 80, 128), bf16),
            pltpu.VMEM((D, F), bf16), pltpu.VMEM((D, F), bf16), pltpu.VMEM((F, D), bf16),
            pltpu.VMEM((8, D), f32),
            pltpu.VMEM((5, 8, 128), u32),
            pltpu.VMEM((2, 15, 8, 128), f32),
            pltpu.VMEM((2, 3, 8, 128), u32),
            pltpu.VMEM((2, 2, 2, 2 * nc2, 8, 128), f32),
            pltpu.VMEM((2, 2 * nc2, 8, 128), f32),
            pltpu.VMEM((2, 2, 3, 8, 128), f32),
            pltpu.VMEM((2, 2, AH, 8, 128), f32),
            pltpu.VMEM((2, 2, AH + 1, 8, 128), f32),
            pltpu.VMEM((2, 2, AH + 1, 8, 128), f32),
            pltpu.VMEM((2, 3, 8, 128), u32),
            pltpu.VMEM((2, 15, 8, 128), f32),
            pltpu.VMEM((5, 8, 128), f32),
            pltpu.SemaphoreType.DMA((NCH,)), pltpu.SemaphoreType.DMA((NCH,)),
            pltpu.SemaphoreType.DMA((5,)),
        ],
        compiler_params=pltpu.CompilerParams(vmem_limit_bytes=124 * 1024 * 1024),
    )(A_x.reshape(1, D), kx, vx, wqz, woz, B_w1, B_w3, B_w2)
    return out.reshape(1, 1, D)
```

```python
import math
import jax
import jax.numpy as jnp
from jax import lax
import jax.experimental.pallas as pl
import jax.experimental.pallas.tpu as pltpu

H, DH, D, F = 32, 192, 640, 1536
HD = H * DH
EPS = 1e-5
NA = HD // 8
AH = DH // 8
NP = H // 2
HC = 4
NCH = H // HC
NL = 2
NREP = 1
MX0 = 0.35
MX1 = 1.1
AB = 4
SMG = 4
FB = 256
W2CUT = (1152,)
SMH = 8
ORG = 4
DYNP = 0
SMB0 = 0.1
SMB1 = 0.8
f32, bf16, u32 = jnp.float32, jnp.bfloat16, jnp.uint32


def _ln_stats(x):
    m = jnp.mean(x, axis=-1, keepdims=True)
    xc = x - m
    v = jnp.mean(xc * xc, axis=-1, keepdims=True)
    return m, lax.rsqrt(v + EPS)


def _ln_lhs(x):
    return jnp.where(lax.broadcasted_iota(jnp.int32, x.shape, 0) < 4, x, 1.0)


def _ln_fix(raw, m, r):
    return (raw - m * pltpu.roll(raw, 4, 0)) * r


def _rnd(x):
    return x.astype(bf16).astype(f32)


def _pack(x8):
    return pltpu.bitcast(jnp.concatenate([x8, x8], axis=0).astype(bf16), u32)


def _mm(lhs_u32, w_u32, half=0):
    lhs = pltpu.bitcast(lhs_u32, bf16)
    w = pltpu.bitcast(w_u32.reshape(64, 128), bf16)
    r = jnp.dot(lhs, w, preferred_element_type=f32)
    return r if half is None else r[8 * half:8 * half + 8]


def _bc(x):
    return jnp.broadcast_to(x, (8, 128))


def _tree(op, xs):
    xs = list(xs)
    while len(xs) > 1:
        xs = [op(xs[i], xs[i + 1]) if i + 1 < len(xs) else xs[i] for i in range(0, len(xs), 2)]
    return xs[0]


def _run(jobs):
    for j in jobs:
        j()


def _weave(main, extra, lo, hi):
    out, k = [], 0
    for n, j in enumerate(main):
        while k < len(extra) and lo * len(main) + k * (hi - lo) * len(main) / len(extra) <= n:
            out.append(extra[k])
            k += 1
        out.append(j)
    return out + list(extra[k:])


def _make_kernel(SK, W):
    NC = W // 128
    NC2 = NC // 2
    R0 = (SK - W) // 16
    RW = W // 16
    qscale = DH ** -0.5 * math.log2(math.e)

    def kernel(x_hbm, k_hbm, v_hbm, wq_hbm, wo_hbm, w1_hbm, w3_hbm, w2_hbm, o_ref,
               kb, vb, wqb, wob, w1, w3, w2,
               xb, xs, lx, stat, qraw, lq, sraw, pbuf, st, oacc, oscl, rsum, lo, woraw, xacc,
               sem):
        k32 = kb.bitcast(u32)
        wq32 = wqb.bitcast(u32)
        wo32 = wob.bitcast(u32)

        def kcp(c):
            r = pl.ds(c * (HC * AH // 2), HC * AH // 2)
            return pltpu.make_async_copy(k_hbm.at[r, :, pl.ds(R0 // 16, NC2)], kb.at[r], sem.at[c])

        def kready(c):
            kcp(c).wait()

            def swap(r, carry):
                a = k32[r, 0, :, 4:8, :]
                b = k32[r, 1, :, 0:4, :]
                k32[r, 0, :, 4:8, :] = b
                k32[r, 1, :, 0:4, :] = a
                return carry
            lax.fori_loop(c * (HC * AH // 2), (c + 1) * (HC * AH // 2), swap, 0)

        def vcp(c):
            r = pl.ds(c * (HC * AH), HC * AH)
            return pltpu.make_async_copy(v_hbm.at[r, pl.ds(R0, RW), :], vb.at[r], sem.at[NCH + c])

        w2cut = (0,) + W2CUT + (F,)
        pairs = [(x_hbm, xb), (wq_hbm, wqb), (wo_hbm, wob), (w1_hbm, w1), (w3_hbm, w3)]
        pairs += [(w2_hbm.at[a:b], w2.at[a:b]) for a, b in zip(w2cut, w2cut[1:])]
        wcp = [pltpu.make_async_copy(s, d, sem.at[2 * NCH + i]) for i, (s, d) in enumerate(pairs)]
        for i in range(3):
            wcp[i].start()
        for c in range(NCH):
            kcp(c).start()
            vcp(c).start()
        for cp in wcp[3:]:
            cp.start()

        wcp[0].wait()
        xs[...] = jnp.broadcast_to(xb[...].astype(f32), (8, D))

        wcp[1].wait()

        def retile_wq(r, c):
            a = wq32[r, 0:24, 4:8, :]
            b = wq32[r, 24:48, 0:4, :]
            wq32[r, 0:24, 4:8, :] = b
            wq32[r, 24:48, 0:4, :] = a
            return c
        lax.fori_loop(0, D // 16, retile_wq, 0)
        wcp[2].wait()

        def retile_wo(rb, c):
            r = pl.ds(rb * 4, 4)
            vals = {(e, cc): wo32[r, 4 * (5 * e + cc):4 * (5 * e + cc) + 4, :]
                    for e in range(2) for cc in range(5)}
            for (e, cc), v in vals.items():
                wo32[r, 8 * cc + 4 * e:8 * cc + 4 * e + 4, :] = v
            return c
        lax.fori_loop(0, HD // 64, retile_wo, 0)

        sub = lax.broadcasted_iota(jnp.int32, (8, 128), 0)
        lane = lax.broadcasted_iota(jnp.int32, (8, 128), 1)

        def qproj_jobs(p, q):
            jobs = []
            for t in range(3):
                c = 3 * p + t
                slot = (c & 1) * 24 + (c >> 1)
                for kk in range(5):
                    def job(t=t, kk=kk, slot=slot):
                        qraw[q, 5 * t + kk] = _mm(lx[kk], wq32[8 * kk:8 * kk + 8, slot])
                    jobs.append(job)
            return jobs

        def qprep(q):
            for t in range(3):
                qv = _tree(jnp.add, [qraw[q, 5 * t + kk] for kk in range(5)])
                qp = _pack(_bc(_ln_fix(qv, stat[0], stat[1])[0:1]))
                if t == 1:
                    qp = jnp.where((lane >> 6) == (sub >> 2), qp, jnp.uint32(0))
                lq[q, t] = qp

        def qk_jobs(p, q):
            jobs = []
            for t in range(3):
                r0 = p * AH + 8 * t
                for c in range(NC):
                    def job(t=t, c=c, r0=r0):
                        r = _mm(lq[q, t], k32[pl.ds(r0, 8), c & 1, c >> 1], None)
                        g, j = c // 8, c % 8
                        if t < 2:
                            sraw[q, 0, t, g, j:j + 1, :] = r[j:j + 1]
                        if t > 0:
                            o = 8 if t == 1 else 0
                            sraw[q, 1, t - 1, g, j:j + 1, :] = r[o + j:o + j + 1]
                    jobs.append(job)
            return jobs

        def sm1_jobs(q, e):
            env = {}

            def allsub(op, x):
                for sh in (4, 2, 1):
                    x = op(x, pltpu.roll(x, sh, 0))
                return x

            def head():
                s = [sraw[q, e, 0, g] + sraw[q, e, 1, g] for g in range(NC // 8)]
                mv = allsub(jnp.maximum, _tree(jnp.maximum, s))
                st[q, e, 0] = mv
                env["p"] = [jnp.exp2(x - mv) for x in s]

            def lsum():
                st[q, e, 1] = allsub(jnp.add, _tree(jnp.add, env["p"]))

            def mk(c0):
                def job():
                    for c in range(c0, c0 + SMG):
                        pbuf[e, c] = _bc(env["p"][c // 8][c % 8:c % 8 + 1])
                return job
            return [head], [mk(c0) for c0 in range(0, NC, SMG)] + [lsum]

        def pv_jobs(p, q, e, z):
            jobs = []
            for a0 in range(0, AH, AB):
                accs = [None] * AB
                for c2 in range(NC2):
                    def job(a0=a0, c2=c2, accs=accs):
                        p0 = pbuf[e, z + 2 * c2]
                        p1 = pbuf[e, z + 2 * c2 + 1]
                        for i in range(AB):
                            a = p * (2 * AH) + (e * AH + a0 + i)
                            v = vb[a, 16 * c2:16 * c2 + 16, :].astype(f32)
                            t = v[0:8] * p0 + v[8:16] * p1
                            accs[i] = t if accs[i] is None else accs[i] + t
                        if c2 == NC2 - 1:
                            for i in range(AB):
                                oacc[q, e, a0 + i] = accs[i]
                    jobs.append(job)
            return jobs

        def xmax(q):
            for e in range(2):
                st[q, e, 2] = _bc(jnp.max(st[q, e, 0], axis=1, keepdims=True))

        def scale_jobs(q, e):
            env = {}

            def head():
                env["w"] = jnp.exp2(st[q, e, 0] - st[q, e, 2])
                oscl[q, e, AH] = env["w"] * st[q, e, 1]

            def mk(g):
                def job():
                    for a in range(ORG * g, ORG * g + ORG):
                        oscl[q, e, a] = oacc[q, e, a] * env["w"]
                return job
            return [head] + [mk(g) for g in range(AH // ORG)]

        def xsum(q):
            for e in range(2):
                for a in range(AH + 1):
                    rsum[q, e, a] = _bc(jnp.sum(oscl[q, e, a], axis=1, keepdims=True))

        def or2(q):
            def sel(bit, x, y):
                return jnp.where(((lane >> bit) & 1) == 0, x, y)
            vals = []
            for e in range(2):
                for g in range(3):
                    r = [rsum[q, e, 8 * g + k] for k in range(8)]
                    r = [sel(3, r[2 * k], r[2 * k + 1]) for k in range(4)]
                    r = [sel(4, r[2 * k], r[2 * k + 1]) for k in range(2)]
                    vals.append(sel(5, r[0], r[1]))
            inv0 = 1.0 / rsum[q, 0, AH]
            inv1 = 1.0 / rsum[q, 1, AH]
            invs = [inv0, sel(6, inv0, inv1), inv1]
            diag = (lane & 7) == sub
            for t in range(3):
                o = sel(6, vals[2 * t], vals[2 * t + 1]) * invs[t]
                lo[q, t] = _pack(jnp.where(diag, o, 0.0))

        def woproj_jobs(p, q):
            jobs = []
            for t in range(3):
                r0 = 24 * p + 8 * t
                for cc in range(5):
                    def job(t=t, cc=cc, r0=r0):
                        woraw[q, 5 * t + cc] = _mm(lo[q, t], wo32[pl.ds(r0, 8), 8 * cc:8 * cc + 8, :])
                    jobs.append(job)
            return jobs

        def woacc(q, valid=None):
            for cc in range(5):
                t = woraw[q, cc] + woraw[q, 5 + cc] + woraw[q, 10 + cc]
                if valid is not None:
                    t = jnp.where(valid, t, 0.0)
                xacc[cc] = xacc[cc] + t

        def block(b, q):
            nq = 1 - q
            z = (b >> 10) if DYNP else 0
            mx = (qk_jobs(jnp.minimum(b + 1, NP - 1), nq)
                  + qproj_jobs(jnp.minimum(b + 3, NP - 1), nq)
                  + woproj_jobs(jnp.maximum(b - 5, 0), nq))
            sc0, sc1 = scale_jobs(q, 0), scale_jobs(q, 1)
            (sa1, sa2), (sb1, sb2) = sm1_jobs(q, 0), sm1_jobs(q, 1)
            pa, pb = pv_jobs(b, q, 0, z), pv_jobs(b, q, 1, z)
            start = ([sc0[0], sc1[0]] + sa1 + [lambda: or2(q), sa2[0], lambda: woacc(q, b >= 6), sa2[1]])
            first = _weave(pa[:NC2], sa2[2:], 0.0, 1.0 - 1.0 * SMG / NC)
            first = first[:-1] + sc0[1:2] + first[-1:]
            rest = _weave(pa[NC2:], sc0[2:], 0.0, 1.0)
            rest = _weave(rest, sb1 + sb2, SMB0, SMB1)
            vb_ = _weave(_weave(pb, sc1[1:], 0.0, 1.0), [lambda: qprep(q)], 0.3, 0.4)
            valu = start + first + rest + vb_
            xl = [lambda: xmax(nq), lambda: xsum(nq)]
            _run(xl + _weave(valu, mx, MX0, MX1))

        kready(0)

        def layer_body(layer, carry):
            first = layer == 0
            x = xs[...]
            xl = _ln_lhs(x)
            for kk in range(5):
                lx[kk] = _pack(xl[:, 128 * kk:128 * kk + 128])
            m, r = _ln_stats(x)
            stat[0] = _bc(m)
            stat[1] = _bc(r * qscale)
            xacc[...] = jnp.zeros_like(xacc)
            _run(qproj_jobs(0, 0))
            qprep(0)
            _run(qproj_jobs(1, 1))
            qprep(1)
            _run(qproj_jobs(2, 0))
            _run(qk_jobs(0, 0))

            def body(b0, c):
                b = b0 & 15

                @pl.when(jnp.logical_and(first, b0 < NP))
                def _():
                    @pl.when((b & 1) == 0)
                    def _():
                        vcp(b >> 1).wait()

                    @pl.when(jnp.logical_and((b & 1) == 1, b < NP - 1))
                    def _():
                        kready((b + 1) >> 1)
                lax.cond((b & 1) == 0, lambda: block(b, 0), lambda: block(b, 1))
                return c
            lax.fori_loop(0, NP * NREP, body, 0)
            for b in range(NP, NP + 6):
                q = b & 1
                if b - 1 < NP:
                    xmax(1 - q)
                if b - 2 < NP:
                    _run(scale_jobs(q, 0) + scale_jobs(q, 1))
                if b - 3 < NP:
                    xsum(1 - q)
                if b - 4 < NP:
                    or2(q)
                if b - 5 < NP:
                    _run(woproj_jobs(b - 5, 1 - q))
                woacc(q)
            att = jnp.sum(jnp.concatenate([xacc[cc] for cc in range(5)], axis=1), axis=0, keepdims=True)
            x1 = _rnd(x + _rnd(att))

            def ffn(wait):
                if wait:
                    wcp[3].wait()
                    wcp[4].wait()
                m, r = _ln_stats(x1)
                xl = _ln_lhs(x1).astype(bf16)
                hs = []
                for j in range(0, F, FB):
                    g = _ln_fix(jnp.dot(xl, w1[:, j:j + FB], preferred_element_type=f32), m, r)
                    u = _ln_fix(jnp.dot(xl, w3[:, j:j + FB], preferred_element_type=f32), m, r)
                    hs.append((g * jax.nn.sigmoid(g) * u).astype(bf16))
                hh = jnp.concatenate(hs, axis=1)
                y = None
                for i, (a, b) in enumerate(zip(w2cut, w2cut[1:])):
                    if wait:
                        if i > 0:
                            xs[...] = y
                        wcp[5 + i].wait()
                        if i > 0:
                            y = xs[...]
                    for j in range(a, b, 128):
                        t = jnp.dot(hh[:, j:j + 128], w2[j:j + 128, :], preferred_element_type=f32)
                        y = t if y is None else y + t
                xs[...] = _rnd(x1 + _rnd(y[0:1]))
            lax.cond(first, lambda: ffn(True), lambda: ffn(False))
            return carry
        lax.fori_loop(0, NL, layer_body, 0)
        o_ref[...] = xs[0:1, :].astype(o_ref.dtype)
    return kernel


def _tile_linear(c):
    sk = c.shape[2]
    return (jnp.swapaxes(c, 2, 3).reshape(NA, 8, sk // 128, 128)
            .transpose(0, 2, 1, 3).reshape(NA, sk // 16, 128))


@jax.jit
def pallas_interleave_layers__sliding_block_cached__glu_gated_swiglu__decode_kernel(
    A_x: jax.Array,
    A_k_cache: jax.Array,
    A_v_cache: jax.Array,
    A_wq: jax.Array,
    A_wo: jax.Array,
    B_x: jax.Array,
    B_w1: jax.Array,
    B_w3: jax.Array,
    B_w2: jax.Array,
):
    SK = A_k_cache.shape[2]
    W = min(4096, max(256, SK // 4))
    kx = _tile_linear(A_k_cache).reshape(NA // 2, 2, SK // 256, 16, 128)
    vx = _tile_linear(A_v_cache)
    wqz = (A_wq.reshape(D // 16, 2, 8, 24, 2, 128).transpose(0, 1, 3, 4, 2, 5)
           .reshape(D // 16, 48, 16, 128))
    woz = (A_wo.reshape(HD // 16, 2, 8, 5, 128).transpose(0, 1, 3, 2, 4)
           .reshape(HD // 16, 80, 128))
    any_ = pl.BlockSpec(memory_space=pl.ANY)
    vm = pl.BlockSpec(memory_space=pltpu.VMEM)
    nc2 = W // 256
    out = pl.pallas_call(
        _make_kernel(SK, W),
        out_shape=jax.ShapeDtypeStruct((1, D), A_x.dtype),
        in_specs=[any_] * 8,
        out_specs=vm,
        scratch_shapes=[
            pltpu.VMEM((NA // 2, 2, nc2, 16, 128), bf16), pltpu.VMEM((NA, W // 16, 128), bf16),
            pltpu.VMEM((D // 16, 48, 16, 128), bf16), pltpu.VMEM((HD // 16, 80, 128), bf16),
            pltpu.VMEM((D, F), bf16), pltpu.VMEM((D, F), bf16), pltpu.VMEM((F, D), bf16),
            pltpu.VMEM((1, D), bf16),
            pltpu.VMEM((8, D), f32),
            pltpu.VMEM((5, 8, 128), u32),
            pltpu.VMEM((2, 8, 128), f32),
            pltpu.VMEM((2, 15, 8, 128), f32),
            pltpu.VMEM((2, 3, 8, 128), u32),
            pltpu.VMEM((2, 2, 2, nc2 // 4, 8, 128), f32),
            pltpu.VMEM((2, 2 * nc2, 8, 128), f32),
            pltpu.VMEM((2, 2, 3, 8, 128), f32),
            pltpu.VMEM((2, 2, AH, 8, 128), f32),
            pltpu.VMEM((2, 2, AH + 1, 8, 128), f32),
            pltpu.VMEM((2, 2, AH + 1, 8, 128), f32),
            pltpu.VMEM((2, 3, 8, 128), u32),
            pltpu.VMEM((2, 15, 8, 128), f32),
            pltpu.VMEM((5, 8, 128), f32),
            pltpu.SemaphoreType.DMA((2 * NCH + 6 + len(W2CUT),)),
        ],
        compiler_params=pltpu.CompilerParams(vmem_limit_bytes=124 * 1024 * 1024),
    )(A_x.reshape(1, D), kx, vx, wqz, woz, B_w1, B_w3, B_w2)
    return out.reshape(1, 1, D)
```

```python
import functools
import math
import jax
import jax.numpy as jnp
from jax import lax
import jax.experimental.pallas as pl
import jax.experimental.pallas.tpu as pltpu

H, DH, D, F = 32, 192, 640, 1536
HD = H * DH
EPS = 1e-5
NA = HD // 8
AH = DH // 8
NP = H // 2
HC = 4
NCH = H // HC
NL = 2
NREP = 1
MX0 = 0.35
MX1 = 1.0
AB = 4
SMG = 4
CAP = 142
NX = 2
XP = list(range(NX))
VP = list(range(NX, NP))
RING = 4
FB = 256
W2CUT = (1152,)
SMH = 8
ORG = 4
DYNP = 0
SMB0 = 0.1
SMB1 = 0.8
f32, bf16, u32 = jnp.float32, jnp.bfloat16, jnp.uint32


def _ln_stats(x):
    m = jnp.mean(x, axis=-1, keepdims=True)
    xc = x - m
    v = jnp.mean(xc * xc, axis=-1, keepdims=True)
    return m, lax.rsqrt(v + EPS)


def _ln_lhs(x):
    return jnp.where(lax.broadcasted_iota(jnp.int32, x.shape, 0) < 4, x, 1.0)


def _ln_fix(raw, m, r):
    return (raw - m * pltpu.roll(raw, 4, 0)) * r


def _rnd(x):
    return x.astype(bf16).astype(f32)


def _pack(x8):
    return pltpu.bitcast(jnp.concatenate([x8, x8], axis=0).astype(bf16), u32)


def _mm(lhs_u32, w_u32, half=0):
    lhs = pltpu.bitcast(lhs_u32, bf16)
    w = pltpu.bitcast(w_u32.reshape(64, 128), bf16)
    r = jnp.dot(lhs, w, preferred_element_type=f32)
    return r if half is None else r[8 * half:8 * half + 8]


def _bc(x):
    return jnp.broadcast_to(x, (8, 128))


def _tree(op, xs):
    xs = list(xs)
    while len(xs) > 1:
        xs = [op(xs[i], xs[i + 1]) if i + 1 < len(xs) else xs[i] for i in range(0, len(xs), 2)]
    return xs[0]


def _run(jobs):
    for j in jobs:
        j()


def _weave(main, extra, lo, hi):
    out, k = [], 0
    for n, j in enumerate(main):
        while k < len(extra) and lo * len(main) + k * (hi - lo) * len(main) / len(extra) <= n:
            out.append(extra[k])
            k += 1
        out.append(j)
    return out + list(extra[k:])


def _plan(nt):
    nb = len(VP)
    total = {"QP": 15, "QK": nt, "PM": nt, "WO": 15}
    done = {}
    fin = {}
    mxu, small = {}, {}

    def issue(b, kind, p, cap):
        k0 = done.get((kind, p), 0)
        n = min(total[kind] - k0, cap)
        if n > 0:
            mxu[b].append((kind, p, k0, k0 + n))
            done[(kind, p)] = k0 + n
            if k0 + n == total[kind]:
                fin[(kind, p)] = b
        return max(n, 0)

    def before(key, b):
        return fin.get(key, b) < b

    chains = {p: (["QP", "qprep", "QK", "gs1", "xmax", "gs2", "PM", "orx", "WO", "woacc"] if p in XP else
                  ["QP", "qprep", "QK", "pv", "xmax", "scale", "xsum", "or2", "WO", "woacc"])
              for p in range(NP)}
    for p in VP[:3]:
        done[("QP", p)] = 15
        fin[("QP", p)] = fin[("qprep", p)] = -1
    done[("QK", VP[0])] = nt
    fin[("QK", VP[0])] = -1
    b = 0
    while any(("woacc", p) not in fin for p in range(NP)):
        mxu[b], small[b] = [], []
        for p in range(NP):
            ch = chains[p]
            for prev, st in zip(ch, ch[1:]):
                if st in total or (st, p) in fin or not before((prev, p), b):
                    continue
                if st == "pv":
                    if b < nb and VP[b] == p:
                        fin[(st, p)] = b
                    continue
                small[b].append((st, p))
                fin[(st, p)] = b
                if st == "gs2":
                    small.setdefault(("late", b + 1), []).append(("xl", p))
        small[b] += small.pop(("late", b), [])
        cap = CAP if b < nb else 10 ** 6
        if b + 1 < nb:
            assert before(("qprep", VP[b + 1]), b)
            cap -= issue(b, "QK", VP[b + 1], nt)
        if b + 3 < nb:
            cap -= issue(b, "QP", VP[b + 3], 15)
        cands = [("QP", p, None) for p in XP] + [("QK", p, "qprep") for p in XP]
        cands += [("PM", p, "gs2") for p in XP] + [("QP", p, None) for p in VP]
        cands += [("WO", p, "orx" if p in XP else "or2") for p in VP + XP]
        cands += [("QK", p, "qprep") for p in VP]
        for kind, p, need in cands:
            if cap > 0 and (need is None or before((need, p), b)):
                cap -= issue(b, kind, p, cap)
        assert b >= nb or fin.get(("pv", VP[b])) == b
        b += 1
    return mxu, small


def _make_kernel(SK, W):
    NC = W // 128
    NC2 = NC // 2
    R0 = (SK - W) // 16
    RW = W // 16
    qscale = DH ** -0.5 * math.log2(math.e)

    def kernel(x_hbm, k_hbm, v_hbm, wq_hbm, wo_hbm, w1_hbm, w3_hbm, w2_hbm, o_ref,
               kb, vb, wqb, wob, w1, w3, w2,
               xb, xs, lx, stat, qraw, lq, sraw, pbuf, st, oacc, otile, lp, pmraw, lo, woraw, xacc,
               sem):
        k32 = kb.bitcast(u32)
        v32 = vb.bitcast(u32)
        wq32 = wqb.bitcast(u32)
        wo32 = wob.bitcast(u32)

        def kcp(c):
            r = pl.ds(c * (HC * AH // 2), HC * AH // 2)
            return pltpu.make_async_copy(k_hbm.at[r, :, pl.ds(R0 // 16, NC2)], kb.at[r], sem.at[c])

        def kready(c):
            kcp(c).wait()

            def swap(r, carry):
                a = k32[r, 0, :, 4:8, :]
                b = k32[r, 1, :, 0:4, :]
                k32[r, 0, :, 4:8, :] = b
                k32[r, 1, :, 0:4, :] = a
                return carry
            lax.fori_loop(c * (HC * AH // 2), (c + 1) * (HC * AH // 2), swap, 0)

        def vcp(c):
            r = pl.ds(c * (HC * AH), HC * AH)
            return pltpu.make_async_copy(v_hbm.at[r, pl.ds(R0, RW), :], vb.at[r], sem.at[NCH + c])

        w2cut = (0,) + W2CUT + (F,)
        pairs = [(x_hbm, xb), (wq_hbm, wqb), (wo_hbm, wob), (w1_hbm, w1), (w3_hbm, w3)]
        pairs += [(w2_hbm.at[a:b], w2.at[a:b]) for a, b in zip(w2cut, w2cut[1:])]
        wcp = [pltpu.make_async_copy(s, d, sem.at[2 * NCH + i]) for i, (s, d) in enumerate(pairs)]
        for i in range(3):
            wcp[i].start()
        for c in range(NCH):
            kcp(c).start()
            vcp(c).start()
        for cp in wcp[3:]:
            cp.start()

        wcp[0].wait()
        xs[...] = jnp.broadcast_to(xb[...].astype(f32), (8, D))

        wcp[1].wait()

        def retile_wq(r, c):
            a = wq32[r, 0:24, 4:8, :]
            b = wq32[r, 24:48, 0:4, :]
            wq32[r, 0:24, 4:8, :] = b
            wq32[r, 24:48, 0:4, :] = a
            return c
        lax.fori_loop(0, D // 16, retile_wq, 0)
        wcp[2].wait()

        def retile_wo(rb, c):
            r = pl.ds(rb * 4, 4)
            vals = {(e, cc): wo32[r, 4 * (5 * e + cc):4 * (5 * e + cc) + 4, :]
                    for e in range(2) for cc in range(5)}
            for (e, cc), v in vals.items():
                wo32[r, 8 * cc + 4 * e:8 * cc + 4 * e + 4, :] = v
            return c
        lax.fori_loop(0, HD // 64, retile_wo, 0)

        sub = lax.broadcasted_iota(jnp.int32, (8, 128), 0)
        lane = lax.broadcasted_iota(jnp.int32, (8, 128), 1)

        def qp_job(p, k):
            t, kk = divmod(k, 5)
            c = 3 * p + t
            qraw[p, k] = _mm(lx[kk], wq32[8 * kk:8 * kk + 8, (c & 1) * 24 + (c >> 1)])

        def qprep(p):
            for t in range(3):
                qv = _tree(jnp.add, [qraw[p, 5 * t + kk] for kk in range(5)])
                qp = _pack(_bc(_ln_fix(qv, stat[0], stat[1])[0:1]))
                if t == 1:
                    qp = jnp.where((lane >> 6) == (sub >> 2), qp, jnp.uint32(0))
                lq[p, t] = qp

        def keep_rows(dst, t, c, r):
            g, j = divmod(c, 8)
            if t < 2:
                dst[0, t, g, j:j + 1, :] = r[j:j + 1]
            if t > 0:
                dst[1, t - 1, g, j:j + 1, :] = r[8 + j:9 + j]

        def qk_job(p, k):
            t, c = divmod(k, NC)
            r0 = p * AH + 8 * t
            keep_rows(sraw.at[p], t, c, _mm(lq[p, t], k32[r0:r0 + 8, c & 1, c >> 1], None))

        def pm_job(p, k):
            t, c = divmod(k, NC)
            a0 = p * 2 * AH + 16 * t + 8 * (c & 1)
            w = v32[a0:a0 + 8, 8 * (c >> 1):8 * (c >> 1) + 8, :]
            keep_rows(pmraw.at[p], t, c, _mm(lp[p, c // 8], w, None))

        def wo_job(p, k):
            t, cc = divmod(k, 5)
            r0 = 24 * p + 8 * t
            woraw[p, k] = _mm(lo[p, t], wo32[r0:r0 + 8, 8 * cc:8 * cc + 8, :])

        def allsub(op, x):
            for sh in (4, 2, 1):
                x = op(x, pltpu.roll(x, sh, 0))
            return x

        def scores(p, e):
            return [sraw[p, e, 0, g] + sraw[p, e, 1, g] for g in range(NC // 8)]

        def sm1_jobs(p, e):
            env = {}

            def head():
                s = scores(p, e)
                mv = allsub(jnp.maximum, _tree(jnp.maximum, s))
                st[p, e, 0] = mv
                env["p"] = [jnp.exp2(x - mv) for x in s]

            def lsum():
                st[p, e, 1] = allsub(jnp.add, _tree(jnp.add, env["p"]))

            def mk(c0):
                def job():
                    for c in range(c0, c0 + SMG):
                        pbuf[e, c] = _bc(env["p"][c // 8][c % 8:c % 8 + 1])
                return job
            return [head], [mk(c0) for c0 in range(0, NC, SMG)] + [lsum]

        def pv_jobs(p, e):
            jobs = []
            for a0 in range(0, AH, AB):
                accs = [None] * AB
                for c2 in range(NC2):
                    def job(a0=a0, c2=c2, accs=accs):
                        p0 = pbuf[e, 2 * c2]
                        p1 = pbuf[e, 2 * c2 + 1]
                        for i in range(AB):
                            a = p * (2 * AH) + (e * AH + a0 + i)
                            v = vb[a, 16 * c2:16 * c2 + 16, :].astype(f32)
                            t = v[0:8] * p0 + v[8:16] * p1
                            accs[i] = t if accs[i] is None else accs[i] + t
                        if c2 == NC2 - 1:
                            for i in range(AB):
                                oacc[p % RING, e, a0 + i] = accs[i]
                    jobs.append(job)
            return jobs

        def xmax(p):
            for e in range(2):
                st[p, e, 2] = _bc(jnp.max(st[p, e, 0], axis=1, keepdims=True))

        def scale_jobs(p):
            jobs = []
            for e in range(2):
                env = {}

                def head(e=e, env=env):
                    env["w"] = jnp.exp2(st[p, e, 0] - st[p, e, 2])
                    st[p, e, 1] = env["w"] * st[p, e, 1]
                jobs.append(head)
                for g in range(AH // ORG):
                    def job(e=e, env=env, g=g):
                        for a in range(ORG * g, ORG * g + ORG):
                            oacc[p % RING, e, a] = oacc[p % RING, e, a] * env["w"]
                    jobs.append(job)
            return jobs

        def xl(p):
            for e in range(2):
                st[p, e, 3] = _bc(jnp.sum(st[p, e, 1], axis=1, keepdims=True))

        def xsum(p):
            xl(p)
            for e in range(2):
                for a in range(AH):
                    r = _bc(jnp.sum(oacc[p % RING, e, a], axis=1, keepdims=True))
                    t, k = divmod(e * AH + a, 16)
                    otile[p, t, :, 8 * k:8 * k + 8] = r[:, 8 * k:8 * k + 8]

        def finish(p, tiles):
            inv = []
            for e in range(2):
                l = st[p, e, 3]
                r = pl.reciprocal(l, approx=True)
                inv.append(r * (2.0 - l * r))
            invs = [inv[0], jnp.where(lane < 64, inv[0], inv[1]), inv[1]]
            diag = (lane & 7) == sub
            for t in range(3):
                lo[p, t] = _pack(jnp.where(diag, tiles[t] * invs[t], 0.0))

        def or2(p):
            finish(p, [otile[p, t] for t in range(3)])

        def gs1(p):
            for e in range(2):
                st[p, e, 0] = allsub(jnp.maximum, _tree(jnp.maximum, scores(p, e)))

        def gs2(p):
            ps = [[jnp.exp2(x - st[p, e, 2]) for x in scores(p, e)] for e in range(2)]
            for e in range(2):
                st[p, e, 1] = allsub(jnp.add, _tree(jnp.add, ps[e]))
            for g in range(NC // 8):
                lp[p, g] = pltpu.bitcast(
                    jnp.concatenate([ps[0][g], ps[1][g]], axis=0).astype(bf16), u32)

        def orx(p):
            def part(e, t):
                return _tree(jnp.add, [pmraw[p, e, t, g] for g in range(NC // 8)])
            tiles = [part(0, 0), jnp.where(lane < 64, part(0, 1), part(1, 0)), part(1, 1)]
            finish(p, [allsub(jnp.add, x) for x in tiles])

        def woacc(p):
            for cc in range(5):
                xacc[cc] = xacc[cc] + (woraw[p, cc] + woraw[p, 5 + cc] + woraw[p, 10 + cc])

        mxu_fn = {"QP": qp_job, "QK": qk_job, "PM": pm_job, "WO": wo_job}
        xlu_fn = {"xmax": xmax, "xsum": xsum, "xl": xl}
        valu_fn = {"qprep": qprep, "or2": or2, "gs1": gs1, "gs2": gs2, "orx": orx, "woacc": woacc}
        plan_mxu, plan_small = _plan(3 * NC)

        def jobs_of(b):
            mx = [functools.partial(mxu_fn[kind], p, k)
                  for kind, p, k0, k1 in plan_mxu[b] for k in range(k0, k1)]
            xs_ = [functools.partial(xlu_fn[s], p) for s, p in plan_small[b] if s in xlu_fn]
            vs_ = [functools.partial(valu_fn[s], p) for s, p in plan_small[b] if s in valu_fn]
            sc = [j for s, p in plan_small[b] if s == "scale" for j in scale_jobs(p)]
            return mx, xs_, vs_, sc

        def block(b):
            p = VP[b]
            mx, xs_, vs_, sc = jobs_of(b)
            (sa1, sa2), (sb1, sb2) = sm1_jobs(p, 0), sm1_jobs(p, 1)
            pa, pb = pv_jobs(p, 0), pv_jobs(p, 1)
            start = sa1 + vs_[:2] + sa2[:2]
            first = _weave(pa[:NC2], sa2[2:], 0.0, 1.0 - 1.0 * SMG / NC)
            rest = _weave(pa[NC2:], sb1 + sb2, SMB0, SMB1)
            last = _weave(pb, vs_[2:] + sc, 0.0, 0.9) if vs_[2:] + sc else pb
            _run(xs_ + _weave(start + first + rest + last, mx, MX0, MX1))

        def ready_x():
            for c in range(NX * 2 // HC):
                kready(c)
                vcp(c).wait()

            def tr(i, carry):
                a0 = pl.multiple_of((i >> 2) * 16, 16)
                for u in range(4):
                    c2 = (i & 3) * 4 + u
                    r = pl.multiple_of(c2 * 16, 16)
                    x = vb[pl.ds(a0, 16), pl.ds(r, 16), :]
                    ts = [x[:, 8 * h:8 * h + 8, :].reshape(128, 128).T for h in range(2)]
                    r8 = pl.multiple_of(c2 * 8, 8)
                    for h in range(2):
                        v32[pl.ds(a0 + 8 * h, 8), pl.ds(r8, 8), :] = (
                            pltpu.bitcast(ts[h], u32).reshape(8, 8, 128))
                return carry
            lax.fori_loop(0, NX * 3 * NC2 // 4, tr, 0)
        ready_x()
        kready(VP[0] * 2 // HC)

        def layer_body(layer, carry):
            first = layer == 0
            x = xs[...]
            xl = _ln_lhs(x)
            for kk in range(5):
                lx[kk] = _pack(xl[:, 128 * kk:128 * kk + 128])
            m, r = _ln_stats(x)
            stat[0] = _bc(m)
            stat[1] = _bc(r * qscale)
            xacc[...] = jnp.zeros_like(xacc)
            for p in VP[:3]:
                for k in range(15):
                    qp_job(p, k)
                qprep(p)
            for k in range(3 * NC):
                qk_job(VP[0], k)

            kseen = set(range(VP[0] * 2 // HC + 1))
            vseen = set(range(NX * 2 // HC))
            for b in range(len(VP)):
                kneed = sorted({p * 2 // HC for kind, p, _, _ in plan_mxu[b] if kind == "QK"} - kseen)
                vneed = sorted({VP[b] * 2 // HC} - vseen)
                kseen.update(kneed)
                vseen.update(vneed)
                if kneed or vneed:
                    @pl.when(first)
                    def _(kneed=kneed, vneed=vneed):
                        for c in vneed:
                            vcp(c).wait()
                        for c in kneed:
                            kready(c)

                @pl.when(layer < 100 + b)
                def _(b=b):
                    block(b)
            for b in range(len(VP), len(plan_mxu)):
                mx, xs_, vs_, sc = jobs_of(b)
                _run(xs_ + sc + vs_ + mx)
            att = jnp.sum(jnp.concatenate([xacc[cc] for cc in range(5)], axis=1), axis=0, keepdims=True)
            x1 = _rnd(x + _rnd(att))

            def ffn(wait):
                if wait:
                    wcp[3].wait()
                    wcp[4].wait()
                m, r = _ln_stats(x1)
                xl = _ln_lhs(x1).astype(bf16)
                hs = []
                for j in range(0, F, FB):
                    g = _ln_fix(jnp.dot(xl, w1[:, j:j + FB], preferred_element_type=f32), m, r)
                    u = _ln_fix(jnp.dot(xl, w3[:, j:j + FB], preferred_element_type=f32), m, r)
                    hs.append((g * jax.nn.sigmoid(g) * u).astype(bf16))
                hh = jnp.concatenate(hs, axis=1)
                y = None
                for i, (a, b) in enumerate(zip(w2cut, w2cut[1:])):
                    if wait:
                        if i > 0:
                            xs[...] = y
                        wcp[5 + i].wait()
                        if i > 0:
                            y = xs[...]
                    for j in range(a, b, 128):
                        t = jnp.dot(hh[:, j:j + 128], w2[j:j + 128, :], preferred_element_type=f32)
                        y = t if y is None else y + t
                xs[...] = _rnd(x1 + _rnd(y[0:1]))
            lax.cond(first, lambda: ffn(True), lambda: ffn(False))
            return carry
        lax.fori_loop(0, NL, layer_body, 0)
        o_ref[...] = xs[0:1, :].astype(o_ref.dtype)
    return kernel


def _tile_linear(c):
    sk = c.shape[2]
    return (jnp.swapaxes(c, 2, 3).reshape(NA, 8, sk // 128, 128)
            .transpose(0, 2, 1, 3).reshape(NA, sk // 16, 128))


@jax.jit
def pallas_interleave_layers__sliding_block_cached__glu_gated_swiglu__decode_kernel(
    A_x: jax.Array,
    A_k_cache: jax.Array,
    A_v_cache: jax.Array,
    A_wq: jax.Array,
    A_wo: jax.Array,
    B_x: jax.Array,
    B_w1: jax.Array,
    B_w3: jax.Array,
    B_w2: jax.Array,
):
    SK = A_k_cache.shape[2]
    W = min(4096, max(256, SK // 4))
    kx = _tile_linear(A_k_cache).reshape(NA // 2, 2, SK // 256, 16, 128)
    vx = _tile_linear(A_v_cache)
    wqz = (A_wq.reshape(D // 16, 2, 8, 24, 2, 128).transpose(0, 1, 3, 4, 2, 5)
           .reshape(D // 16, 48, 16, 128))
    woz = (A_wo.reshape(HD // 16, 2, 8, 5, 128).transpose(0, 1, 3, 2, 4)
           .reshape(HD // 16, 80, 128))
    any_ = pl.BlockSpec(memory_space=pl.ANY)
    vm = pl.BlockSpec(memory_space=pltpu.VMEM)
    nc2 = W // 256
    out = pl.pallas_call(
        _make_kernel(SK, W),
        out_shape=jax.ShapeDtypeStruct((1, D), A_x.dtype),
        in_specs=[any_] * 8,
        out_specs=vm,
        scratch_shapes=[
            pltpu.VMEM((NA // 2, 2, nc2, 16, 128), bf16), pltpu.VMEM((NA, W // 16, 128), bf16),
            pltpu.VMEM((D // 16, 48, 16, 128), bf16), pltpu.VMEM((HD // 16, 80, 128), bf16),
            pltpu.VMEM((D, F), bf16), pltpu.VMEM((D, F), bf16), pltpu.VMEM((F, D), bf16),
            pltpu.VMEM((1, D), bf16),
            pltpu.VMEM((8, D), f32),
            pltpu.VMEM((5, 8, 128), u32),
            pltpu.VMEM((2, 8, 128), f32),
            pltpu.VMEM((NP, 15, 8, 128), f32),
            pltpu.VMEM((NP, 3, 8, 128), u32),
            pltpu.VMEM((NP, 2, 2, nc2 // 4, 8, 128), f32),
            pltpu.VMEM((2, 2 * nc2, 8, 128), f32),
            pltpu.VMEM((NP, 2, 4, 8, 128), f32),
            pltpu.VMEM((RING, 2, AH, 8, 128), f32),
            pltpu.VMEM((NP, 3, 8, 128), f32),
            pltpu.VMEM((NX, nc2 // 4, 8, 128), u32),
            pltpu.VMEM((NX, 2, 2, nc2 // 4, 8, 128), f32),
            pltpu.VMEM((NP, 3, 8, 128), u32),
            pltpu.VMEM((NP, 15, 8, 128), f32),
            pltpu.VMEM((5, 8, 128), f32),
            pltpu.SemaphoreType.DMA((2 * NCH + 6 + len(W2CUT),)),
        ],
        compiler_params=pltpu.CompilerParams(vmem_limit_bytes=126 * 1024 * 1024),
    )(A_x.reshape(1, D), kx, vx, wqz, woz, B_w1, B_w3, B_w2)
    return out.reshape(1, 1, D)
```

```python
import functools
import math
import jax
import jax.numpy as jnp
from jax import lax
import jax.experimental.pallas as pl
import jax.experimental.pallas.tpu as pltpu

H, DH, D, F = 32, 192, 640, 1536
HD = H * DH
EPS = 1e-5
NA = HD // 8
AH = DH // 8
NP = H // 2
NL = 2
MX0 = 0.35
MX1 = 1.0
AB = 4
SMG = 4
CAP = 142
CAPS = {}
SKEW = 1
MXF = 0
ONLY = None
NX = 2
XP = list(range(NX))
VP = list(range(NX, NP))
RING = 4
FB = 256
W2CUT = (1280,)
KVG = [((0, 4), (0, 4)), ((4, 8), (4, 8)), ((8, 12), (8, 12)), ((12, 16), (12, 14)), (None, (14, 16))]
ORG = 4
SMB0 = 0.1
SMB1 = 0.8
f32, bf16, u32 = jnp.float32, jnp.bfloat16, jnp.uint32


def _ln_stats(x):
    m = jnp.mean(x, axis=-1, keepdims=True)
    xc = x - m
    v = jnp.mean(xc * xc, axis=-1, keepdims=True)
    return m, lax.rsqrt(v + EPS)


def _ln_lhs(x):
    return jnp.where(lax.broadcasted_iota(jnp.int32, x.shape, 0) < 4, x, 1.0)


def _ln_fix(raw, m, r):
    return (raw - m * pltpu.roll(raw, 4, 0)) * r


def _rnd(x):
    return x.astype(bf16).astype(f32)


def _pack(x8):
    return pltpu.bitcast(jnp.concatenate([x8, x8], axis=0).astype(bf16), u32)


def _mm(lhs_u32, w_u32, half=0):
    lhs = pltpu.bitcast(lhs_u32, bf16)
    w = pltpu.bitcast(w_u32.reshape(64, 128), bf16)
    r = jnp.dot(lhs, w, preferred_element_type=f32)
    return r if half is None else r[8 * half:8 * half + 8]


def _bc(x):
    return jnp.broadcast_to(x, (8, 128))


def _tree(op, xs):
    xs = list(xs)
    while len(xs) > 1:
        xs = [op(xs[i], xs[i + 1]) if i + 1 < len(xs) else xs[i] for i in range(0, len(xs), 2)]
    return xs[0]


def _run(jobs):
    for j in jobs:
        j()


def _weave(main, extra, lo, hi):
    out, k = [], 0
    for n, j in enumerate(main):
        while k < len(extra) and lo * len(main) + k * (hi - lo) * len(main) / len(extra) <= n:
            out.append(extra[k])
            k += 1
        out.append(j)
    return out + list(extra[k:])


def _plan(nt):
    nb = len(VP)
    total = {"QP": 15, "QK": nt, "PM": nt, "WO": 15}
    done = {}
    fin = {}
    mxu, small = {}, {}

    def issue(b, kind, p, cap):
        k0 = done.get((kind, p), 0)
        n = min(total[kind] - k0, cap)
        if n > 0:
            mxu[b].append((kind, p, k0, k0 + n))
            done[(kind, p)] = k0 + n
            if k0 + n == total[kind]:
                fin[(kind, p)] = b
        return max(n, 0)

    def before(key, b):
        return fin.get(key, b) < b

    chains = {p: (["QP", "qprep", "QK", "gs1", "xmax", "gs2", "PM", "orx", "WO", "woacc"] if p in XP else
                  ["QP", "qprep", "QK", "pv", "xmax", "scale", "xsum", "or2", "WO", "woacc"])
              for p in range(NP)}
    for p in VP[:3]:
        done[("QP", p)] = 15
        fin[("QP", p)] = fin[("qprep", p)] = -1
    done[("QK", VP[0])] = nt
    fin[("QK", VP[0])] = -1
    b = 0
    while any(("woacc", p) not in fin for p in range(NP)):
        mxu[b], small[b] = [], []
        for p in range(NP):
            ch = chains[p]
            for prev, st in zip(ch, ch[1:]):
                if st in total or (st, p) in fin or not before((prev, p), b):
                    continue
                if st == "pv":
                    if b < nb and VP[b] == p:
                        fin[(st, p)] = b
                    continue
                small[b].append((st, p))
                fin[(st, p)] = b
                if st == "gs2":
                    small.setdefault(("late", b + 1), []).append(("xl", p))
        small[b] += small.pop(("late", b), [])
        cap = CAPS.get(b, CAP) if b < nb else 10 ** 6
        if b + 1 < nb:
            assert before(("qprep", VP[b + 1]), b)
            cap -= issue(b, "QK", VP[b + 1], nt)
        if b + 3 < nb:
            cap -= issue(b, "QP", VP[b + 3], 15)
        cands = [("QP", p, None) for p in XP] + [("QK", p, "qprep") for p in XP]
        cands += [("PM", p, "gs2") for p in XP] + [("QP", p, None) for p in VP]
        cands += [("WO", p, "orx" if p in XP else "or2") for p in VP + XP]
        cands += [("QK", p, "qprep") for p in VP]
        for kind, p, need in cands:
            if cap > 0 and (need is None or before((need, p), b)):
                cap -= issue(b, kind, p, cap)
        assert b >= nb or fin.get(("pv", VP[b])) == b
        b += 1
    return mxu, small


def _make_kernel(SK, W):
    NC = W // 128
    NC2 = NC // 2
    R0 = (SK - W) // 16
    RW = W // 16
    qscale = DH ** -0.5 * math.log2(math.e)

    def kernel(x_hbm, k_hbm, v_hbm, wq_hbm, wo_hbm, w1_hbm, w3_hbm, w2_hbm, o_ref,
               kb, vb, wqb, wob, w1, w3, w2,
               xb, xs, lx, stat, qraw, lq, sraw, pbuf, st, oacc, otile, lp, pmraw, lo, woraw, xacc,
               sem):
        k32 = kb.bitcast(u32)
        v32 = vb.bitcast(u32)
        wq32 = wqb.bitcast(u32)
        wo32 = wob.bitcast(u32)

        def kcp(p0, p1, g):
            r = pl.ds(p0 * AH, (p1 - p0) * AH)
            return pltpu.make_async_copy(k_hbm.at[r, :, pl.ds(R0 // 16, NC2)], kb.at[r], sem.at[g])

        def vcp(p0, p1, g):
            r = pl.ds(p0 * 2 * AH, (p1 - p0) * 2 * AH)
            return pltpu.make_async_copy(v_hbm.at[r, pl.ds(R0, RW), :], vb.at[r], sem.at[g])

        w2cut = (0,) + W2CUT + (F,)
        groups = [[pltpu.make_async_copy(s_, d, sem.at[0])
                   for s_, d in [(x_hbm, xb), (wq_hbm, wqb), (wo_hbm, wob)]]]
        for kr, vr in KVG:
            g = len(groups)
            groups.append(([kcp(*kr, g)] if kr else []) + [vcp(*vr, g)])
        gffn = len(groups)
        groups.append([pltpu.make_async_copy(w1_hbm, w1, sem.at[gffn]),
                       pltpu.make_async_copy(w3_hbm, w3, sem.at[gffn])])
        for a_, b_ in zip(w2cut, w2cut[1:]):
            groups.append([pltpu.make_async_copy(w2_hbm.at[a_:b_], w2.at[a_:b_], sem.at[len(groups)])])
        for grp in groups:
            for cp in grp:
                cp.start()

        def gwait(g):
            for cp in groups[g]:
                cp.wait()

        def kvready(i):
            gwait(1 + i)
            kr = KVG[i][0]
            if kr:
                def swap(r, carry):
                    a = k32[r, 0, :, 4:8, :]
                    b = k32[r, 1, :, 0:4, :]
                    k32[r, 0, :, 4:8, :] = b
                    k32[r, 1, :, 0:4, :] = a
                    return carry
                lax.fori_loop(kr[0] * AH, kr[1] * AH, swap, 0)

        gwait(0)
        xs[...] = jnp.broadcast_to(xb[...].astype(f32), (8, D))


        def retile_wq(r, c):
            a = wq32[r, 0:24, 4:8, :]
            b = wq32[r, 24:48, 0:4, :]
            wq32[r, 0:24, 4:8, :] = b
            wq32[r, 24:48, 0:4, :] = a
            return c
        lax.fori_loop(0, D // 16, retile_wq, 0)

        def retile_wo(rb, c):
            r = pl.ds(rb * 4, 4)
            vals = {(e, cc): wo32[r, 4 * (5 * e + cc):4 * (5 * e + cc) + 4, :]
                    for e in range(2) for cc in range(5)}
            for (e, cc), v in vals.items():
                wo32[r, 8 * cc + 4 * e:8 * cc + 4 * e + 4, :] = v
            return c
        lax.fori_loop(0, HD // 64, retile_wo, 0)

        sub = lax.broadcasted_iota(jnp.int32, (8, 128), 0)
        lane = lax.broadcasted_iota(jnp.int32, (8, 128), 1)

        def qp_job(p, k):
            t, kk = divmod(k, 5)
            c = 3 * p + t
            qraw[p, k] = _mm(lx[kk], wq32[8 * kk:8 * kk + 8, (c & 1) * 24 + (c >> 1)])

        def qprep(p):
            for t in range(3):
                qv = _tree(jnp.add, [qraw[p, 5 * t + kk] for kk in range(5)])
                qp = _pack(_bc(_ln_fix(qv, stat[0], stat[1])[0:1]))
                if t == 1:
                    qp = jnp.where((lane >> 6) == (sub >> 2), qp, jnp.uint32(0))
                lq[p, t] = qp

        def keep_rows(dst, t, c, r):
            g, j = divmod(c, 8)
            if t < 2:
                dst[0, t, g, j:j + 1, :] = r[j:j + 1]
            if t > 0:
                dst[1, t - 1, g, j:j + 1, :] = r[8 + j:9 + j]

        def qk_job(p, k):
            t, c = divmod(k, NC)
            r0 = p * AH + 8 * t
            keep_rows(sraw.at[p], t, c, _mm(lq[p, t], k32[r0:r0 + 8, c & 1, c >> 1], None))

        def pm_job(p, k):
            t, c = divmod(k, NC)
            a0 = p * 2 * AH + 16 * t + 8 * (c & 1)
            w = v32[a0:a0 + 8, 8 * (c >> 1):8 * (c >> 1) + 8, :]
            keep_rows(pmraw.at[p], t, c, _mm(lp[p, c // 8], w, None))

        def wo_job(p, k):
            t, cc = divmod(k, 5)
            r0 = 24 * p + 8 * t
            woraw[p, k] = _mm(lo[p, t], wo32[r0:r0 + 8, 8 * cc:8 * cc + 8, :])

        def allsub(op, x):
            for sh in (4, 2, 1):
                x = op(x, pltpu.roll(x, sh, 0))
            return x

        def scores(p, e):
            return [sraw[p, e, 0, g] + sraw[p, e, 1, g] for g in range(NC // 8)]

        def sm1_jobs(p, e):
            env = {}

            def head():
                s = scores(p, e)
                mv = allsub(jnp.maximum, _tree(jnp.maximum, s))
                st[p, e, 0] = mv
                env["p"] = [jnp.exp2(x - mv) for x in s]

            def lsum():
                st[p, e, 1] = allsub(jnp.add, _tree(jnp.add, env["p"]))

            def mk(c0):
                def job():
                    for c in range(c0, c0 + SMG):
                        pbuf[e, c] = _bc(env["p"][c // 8][c % 8:c % 8 + 1])
                return job
            return [head], [mk(c0) for c0 in range(0, NC, SMG)] + [lsum]

        def pv_jobs(p, e):
            jobs = []
            for a0 in range(0, AH, AB):
                accs = [None] * AB
                for c2 in range(NC2):
                    def job(a0=a0, c2=c2, accs=accs):
                        p0 = pbuf[e, 2 * c2]
                        p1 = pbuf[e, 2 * c2 + 1]
                        for i in range(AB):
                            a = p * (2 * AH) + (e * AH + a0 + i)
                            v = vb[a, 16 * c2:16 * c2 + 16, :].astype(f32)
                            t = v[0:8] * p0 + v[8:16] * p1
                            accs[i] = t if accs[i] is None else accs[i] + t
                        if c2 == NC2 - 1:
                            for i in range(AB):
                                oacc[p % RING, e, a0 + i] = accs[i]
                    jobs.append(job)
            return jobs

        def xmax(p):
            for e in range(2):
                st[p, e, 2] = _bc(jnp.max(st[p, e, 0], axis=1, keepdims=True))

        def scale_jobs(p):
            jobs = []
            for e in range(2):
                env = {}

                def head(e=e, env=env):
                    env["w"] = jnp.exp2(st[p, e, 0] - st[p, e, 2])
                    st[p, e, 1] = env["w"] * st[p, e, 1]
                jobs.append(head)
                for g in range(AH // ORG):
                    def job(e=e, env=env, g=g):
                        for a in range(ORG * g, ORG * g + ORG):
                            oacc[p % RING, e, a] = oacc[p % RING, e, a] * env["w"]
                    jobs.append(job)
            return jobs

        def xl(p):
            for e in range(2):
                st[p, e, 3] = _bc(jnp.sum(st[p, e, 1], axis=1, keepdims=True))

        def xsum(p):
            xl(p)
            for e in range(2):
                for a in range(AH):
                    r = _bc(jnp.sum(oacc[p % RING, e, a], axis=1, keepdims=True))
                    t, k = divmod(e * AH + a, 16)
                    otile[p, t, :, 8 * k:8 * k + 8] = r[:, 8 * k:8 * k + 8]

        def finish(p, tiles):
            inv = []
            for e in range(2):
                l = st[p, e, 3]
                r = pl.reciprocal(l, approx=True)
                inv.append(r * (2.0 - l * r))
            invs = [inv[0], jnp.where(lane < 64, inv[0], inv[1]), inv[1]]
            diag = (lane & 7) == sub
            for t in range(3):
                lo[p, t] = _pack(jnp.where(diag, tiles[t] * invs[t], 0.0))

        def or2(p):
            finish(p, [otile[p, t] for t in range(3)])

        def gs1(p):
            for e in range(2):
                st[p, e, 0] = allsub(jnp.maximum, _tree(jnp.maximum, scores(p, e)))

        def gs2(p):
            ps = [[jnp.exp2(x - st[p, e, 2]) for x in scores(p, e)] for e in range(2)]
            for e in range(2):
                st[p, e, 1] = allsub(jnp.add, _tree(jnp.add, ps[e]))
            for g in range(NC // 8):
                lp[p, g] = pltpu.bitcast(
                    jnp.concatenate([ps[0][g], ps[1][g]], axis=0).astype(bf16), u32)

        def orx(p):
            def part(e, t):
                return _tree(jnp.add, [pmraw[p, e, t, g] for g in range(NC // 8)])
            tiles = [part(0, 0), jnp.where(lane < 64, part(0, 1), part(1, 0)), part(1, 1)]
            finish(p, [allsub(jnp.add, x) for x in tiles])

        def woacc(p):
            for cc in range(5):
                xacc[cc] = xacc[cc] + (woraw[p, cc] + woraw[p, 5 + cc] + woraw[p, 10 + cc])

        mxu_fn = {"QP": qp_job, "QK": qk_job, "PM": pm_job, "WO": wo_job}
        xlu_fn = {"xmax": xmax, "xsum": xsum, "xl": xl}
        valu_fn = {"qprep": qprep, "or2": or2, "gs1": gs1, "gs2": gs2, "orx": orx, "woacc": woacc}
        plan_mxu, plan_small = _plan(3 * NC)

        def jobs_of(b):
            mx = [functools.partial(mxu_fn[kind], p, k)
                  for kind, p, k0, k1 in plan_mxu[b] for k in range(k0, k1)]
            xs_ = [functools.partial(xlu_fn[s], p) for s, p in plan_small[b] if s in xlu_fn]
            vs_ = [functools.partial(valu_fn[s], p) for s, p in plan_small[b] if s in valu_fn]
            sc = [j for s, p in plan_small[b] if s == "scale" for j in scale_jobs(p)]
            return mx, xs_, vs_, sc

        def block(b):
            p = VP[b]
            mx, xs_, vs_, sc = jobs_of(b)
            (sa1, sa2), (sb1, sb2) = sm1_jobs(p, 0), sm1_jobs(p, 1)
            pa, pb = pv_jobs(p, 0), pv_jobs(p, 1)
            cut = len(pb) - SKEW * NC2
            if b + 1 < len(VP):
                pb = pb[:cut]
            if b > 0 and SKEW:
                start = _weave(pv_jobs(VP[b - 1], 1)[cut:], sa1 + sa2, 0.0, 0.9)
                first = pa[:NC2]
                extra = vs_ + sc
            else:
                start = sa1 + vs_[:2] + sa2[:2]
                first = _weave(pa[:NC2], sa2[2:], 0.0, 1.0 - 1.0 * SMG / NC)
                extra = vs_[2:] + sc
            rest = _weave(pa[NC2:], sb1 + sb2, SMB0, SMB1)
            last = _weave(pb, extra, 0.0, 0.9) if extra else pb
            _run(mx[:MXF] + xs_ + _weave(start + first + rest + last, mx[MXF:], MX0, MX1))

        def ready_x():
            kvready(0)

            def tr(i, carry):
                a0 = pl.multiple_of((i >> 2) * 16, 16)
                for u in range(4):
                    c2 = (i & 3) * 4 + u
                    r = pl.multiple_of(c2 * 16, 16)
                    x = vb[pl.ds(a0, 16), pl.ds(r, 16), :]
                    ts = [x[:, 8 * h:8 * h + 8, :].reshape(128, 128).T for h in range(2)]
                    r8 = pl.multiple_of(c2 * 8, 8)
                    for h in range(2):
                        v32[pl.ds(a0 + 8 * h, 8), pl.ds(r8, 8), :] = (
                            pltpu.bitcast(ts[h], u32).reshape(8, 8, 128))
                return carry
            lax.fori_loop(0, NX * 3 * NC2 // 4, tr, 0)
        ready_x()

        def layer_body(layer, carry):
            first = layer == 0
            x = xs[...]
            xl = _ln_lhs(x)
            for kk in range(5):
                lx[kk] = _pack(xl[:, 128 * kk:128 * kk + 128])
            m, r = _ln_stats(x)
            stat[0] = _bc(m)
            stat[1] = _bc(r * qscale)
            xacc[...] = jnp.zeros_like(xacc)
            for p in VP[:3]:
                for k in range(15):
                    qp_job(p, k)
                qprep(p)
            for k in range(3 * NC):
                qk_job(VP[0], k)

            seen = 1
            for b in range(len(VP)):
                kp = max([p for kind, p, _, _ in plan_mxu[b] if kind == "QK"], default=0)
                need = max(i for i, (kr, vr) in enumerate(KVG)
                           if (kr and kr[0] <= kp < kr[1]) or vr[0] <= VP[b] < vr[1]) + 1
                if need > seen:
                    @pl.when(first)
                    def _(lo_=seen, hi_=need):
                        for i in range(lo_, hi_):
                            kvready(i)
                    seen = need
                if ONLY is not None and b not in ONLY:
                    continue

                @pl.when(layer < 100 + b)
                def _(b=b):
                    block(b)

            def finish_layer(wait):
                for b in range(len(VP), len(plan_mxu)):
                    mx, xs_, vs_, sc = jobs_of(b)
                    _run(xs_ + sc + vs_ + mx)
                att = jnp.sum(jnp.concatenate([xacc[cc] for cc in range(5)], axis=1),
                              axis=0, keepdims=True)
                x1 = _rnd(xs[...] + _rnd(att))
                if wait:
                    xs[...] = x1
                    gwait(gffn)
                m, r = _ln_stats(x1)
                xl = _ln_lhs(x1).astype(bf16)
                hs = []
                for j in range(0, F, FB):
                    g = _ln_fix(jnp.dot(xl, w1[:, j:j + FB], preferred_element_type=f32), m, r)
                    u = _ln_fix(jnp.dot(xl, w3[:, j:j + FB], preferred_element_type=f32), m, r)
                    hs.append((g * jax.nn.sigmoid(g) * u).astype(bf16))
                hh = jnp.concatenate(hs, axis=1)
                y = None
                for i, (a, b) in enumerate(zip(w2cut, w2cut[1:])):
                    if wait:
                        if i > 0:
                            xs[...] = y
                        gwait(gffn + 1 + i)
                        if i > 0:
                            y = xs[...]
                    for j in range(a, b, 128):
                        t = jnp.dot(hh[:, j:j + 128], w2[j:j + 128, :], preferred_element_type=f32)
                        y = t if y is None else y + t
                xs[...] = _rnd(x1 + _rnd(y[0:1]))
            lax.cond(first, lambda: finish_layer(True), lambda: finish_layer(False))
            return carry
        lax.fori_loop(0, NL, layer_body, 0)
        o_ref[...] = xs[0:1, :].astype(o_ref.dtype)
    return kernel


def _tile_linear(c):
    sk = c.shape[2]
    return (jnp.swapaxes(c, 2, 3).reshape(NA, 8, sk // 128, 128)
            .transpose(0, 2, 1, 3).reshape(NA, sk // 16, 128))


@jax.jit
def pallas_interleave_layers__sliding_block_cached__glu_gated_swiglu__decode_kernel(
    A_x: jax.Array,
    A_k_cache: jax.Array,
    A_v_cache: jax.Array,
    A_wq: jax.Array,
    A_wo: jax.Array,
    B_x: jax.Array,
    B_w1: jax.Array,
    B_w3: jax.Array,
    B_w2: jax.Array,
):
    SK = A_k_cache.shape[2]
    W = min(4096, max(256, SK // 4))
    kx = _tile_linear(A_k_cache).reshape(NA // 2, 2, SK // 256, 16, 128)
    vx = _tile_linear(A_v_cache)
    wqz = (A_wq.reshape(D // 16, 2, 8, 24, 2, 128).transpose(0, 1, 3, 4, 2, 5)
           .reshape(D // 16, 48, 16, 128))
    woz = (A_wo.reshape(HD // 16, 2, 8, 5, 128).transpose(0, 1, 3, 2, 4)
           .reshape(HD // 16, 80, 128))
    any_ = pl.BlockSpec(memory_space=pl.ANY)
    vm = pl.BlockSpec(memory_space=pltpu.VMEM)
    nc2 = W // 256
    out = pl.pallas_call(
        _make_kernel(SK, W),
        out_shape=jax.ShapeDtypeStruct((1, D), A_x.dtype),
        in_specs=[any_] * 8,
        out_specs=vm,
        scratch_shapes=[
            pltpu.VMEM((NA // 2, 2, nc2, 16, 128), bf16), pltpu.VMEM((NA, W // 16, 128), bf16),
            pltpu.VMEM((D // 16, 48, 16, 128), bf16), pltpu.VMEM((HD // 16, 80, 128), bf16),
            pltpu.VMEM((D, F), bf16), pltpu.VMEM((D, F), bf16), pltpu.VMEM((F, D), bf16),
            pltpu.VMEM((1, D), bf16),
            pltpu.VMEM((8, D), f32),
            pltpu.VMEM((5, 8, 128), u32),
            pltpu.VMEM((2, 8, 128), f32),
            pltpu.VMEM((NP, 15, 8, 128), f32),
            pltpu.VMEM((NP, 3, 8, 128), u32),
            pltpu.VMEM((NP, 2, 2, nc2 // 4, 8, 128), f32),
            pltpu.VMEM((2, 2 * nc2, 8, 128), f32),
            pltpu.VMEM((NP, 2, 4, 8, 128), f32),
            pltpu.VMEM((RING, 2, AH, 8, 128), f32),
            pltpu.VMEM((NP, 3, 8, 128), f32),
            pltpu.VMEM((NX, nc2 // 4, 8, 128), u32),
            pltpu.VMEM((NX, 2, 2, nc2 // 4, 8, 128), f32),
            pltpu.VMEM((NP, 3, 8, 128), u32),
            pltpu.VMEM((NP, 15, 8, 128), f32),
            pltpu.VMEM((5, 8, 128), f32),
            pltpu.SemaphoreType.DMA((len(KVG) + 3 + len(W2CUT),)),
        ],
        compiler_params=pltpu.CompilerParams(vmem_limit_bytes=126 * 1024 * 1024),
    )(A_x.reshape(1, D), kx, vx, wqz, woz, B_w1, B_w3, B_w2)
    return out.reshape(1, 1, D)
```

```python
import functools
import math
import jax
import jax.numpy as jnp
from jax import lax
import jax.experimental.pallas as pl
import jax.experimental.pallas.tpu as pltpu

H, DH, D, F = 32, 192, 640, 1536
HD = H * DH
EPS = 1e-5
NA = HD // 8
AH = DH // 8
NP = H // 2
NL = 2
MX0 = 0.0
MX1 = 1.02
AB = 4
SMG = 4
CAP = 140
CAPS = {0:128,13:152}
SKEW = 1
CORD = 0
PIN = 0.15
PINST = 1
PINGAP = 5
VEC = 1
MXF = 4
ONLY = None
NX = 2
XP = list(range(NX))
VP = list(range(NX, NP))
RING = 4
FB = 256
W2CUT = (1280,)
KVG = [((0, 4), (0, 4)), ((4, 8), (4, 8)), ((8, 12), (8, 12)), ((12, 16), (12, 14)), (None, (14, 16))]
ORG = 4
SMB0 = 0.1
SMB1 = 0.8
f32, bf16, u32 = jnp.float32, jnp.bfloat16, jnp.uint32


def _ln_stats(x):
    m = jnp.mean(x, axis=-1, keepdims=True)
    xc = x - m
    v = jnp.mean(xc * xc, axis=-1, keepdims=True)
    return m, lax.rsqrt(v + EPS)


def _ln_lhs(x):
    return jnp.where(lax.broadcasted_iota(jnp.int32, x.shape, 0) < 4, x, 1.0)


def _ln_fix(raw, m, r):
    return (raw - m * pltpu.roll(raw, 4, 0)) * r


def _rnd(x):
    return x.astype(bf16).astype(f32)


def _pack(x8):
    return pltpu.bitcast(jnp.concatenate([x8, x8], axis=0).astype(bf16), u32)


def _mm(lhs_u32, w_u32, half=0, pin=()):
    lhs = pltpu.bitcast(jnp.concatenate([lhs_u32] + [pltpu.bitcast(x, u32) for x in pin], axis=0)
                        if pin else lhs_u32, bf16)
    w = pltpu.bitcast(w_u32.reshape(64, 128), bf16)
    r = jnp.dot(lhs, w, preferred_element_type=f32)
    return r if half is None else r[8 * half:8 * half + 8]


def _bc(x):
    return jnp.broadcast_to(x, (8, 128))


def _tree(op, xs):
    xs = list(xs)
    while len(xs) > 1:
        xs = [op(xs[i], xs[i + 1]) if i + 1 < len(xs) else xs[i] for i in range(0, len(xs), 2)]
    return xs[0]


def _run(jobs):
    for j in jobs:
        j()


def _weave(main, extra, lo, hi):
    out, k = [], 0
    for n, j in enumerate(main):
        while k < len(extra) and lo * len(main) + k * (hi - lo) * len(main) / len(extra) <= n:
            out.append(extra[k])
            k += 1
        out.append(j)
    return out + list(extra[k:])


def _plan(nt):
    nb = len(VP)
    total = {"QP": 15, "QK": nt, "PM": nt, "WO": 15}
    done = {}
    fin = {}
    mxu, small = {}, {}

    def issue(b, kind, p, cap):
        k0 = done.get((kind, p), 0)
        n = min(total[kind] - k0, cap)
        if n > 0:
            mxu[b].append((kind, p, k0, k0 + n))
            done[(kind, p)] = k0 + n
            if k0 + n == total[kind]:
                fin[(kind, p)] = b
        return max(n, 0)

    def before(key, b):
        return fin.get(key, b) < b

    chains = {p: (["QP", "qprep", "QK", "gs1", "xmax", "gs2", "PM", "orx", "WO", "woacc"] if p in XP else
                  ["QP", "qprep", "QK", "pv", "xmax", "scale", "xsum", "or2", "WO", "woacc"])
              for p in range(NP)}
    for p in VP[:3]:
        done[("QP", p)] = 15
        fin[("QP", p)] = fin[("qprep", p)] = -1
    done[("QK", VP[0])] = nt
    fin[("QK", VP[0])] = -1
    b = 0
    while any(("woacc", p) not in fin for p in range(NP)):
        mxu[b], small[b] = [], []
        for p in range(NP):
            ch = chains[p]
            for prev, st in zip(ch, ch[1:]):
                if st in total or (st, p) in fin or not before((prev, p), b):
                    continue
                if st == "pv":
                    if b < nb and VP[b] == p:
                        fin[(st, p)] = b
                    continue
                small[b].append((st, p))
                fin[(st, p)] = b
                if st == "gs2":
                    small.setdefault(("late", b + 1), []).append(("xl", p))
        small[b] += small.pop(("late", b), [])
        cap = CAPS.get(b, CAP) if b < nb else 10 ** 6
        if b + 1 < nb:
            assert before(("qprep", VP[b + 1]), b)
            cap -= issue(b, "QK", VP[b + 1], nt)
        if b + 3 < nb:
            cap -= issue(b, "QP", VP[b + 3], 15)
        cands = [("QP", p, None) for p in XP] + [("QK", p, "qprep") for p in XP]
        cands += [("PM", p, "gs2") for p in XP] + [("QP", p, None) for p in VP]
        cands += [("WO", p, "orx" if p in XP else "or2") for p in VP + XP]
        cands += [("QK", p, "qprep") for p in VP]
        for kind, p, need in cands:
            if cap > 0 and (need is None or before((need, p), b)):
                cap -= issue(b, kind, p, cap)
        assert b >= nb or fin.get(("pv", VP[b])) == b
        b += 1
    return mxu, small


def _make_kernel(SK, W):
    NC = W // 128
    NC2 = NC // 2
    R0 = (SK - W) // 16
    RW = W // 16
    qscale = DH ** -0.5 * math.log2(math.e)

    def kernel(x_hbm, k_hbm, v_hbm, wq_hbm, wo_hbm, w1_hbm, w3_hbm, w2_hbm, o_ref,
               kb, vb, wqb, wob, w1, w3, w2,
               xb, xs, lx, stat, qraw, lq, sraw, pbuf, st, oacc, otile, lp, pmraw, lo, woraw, xacc,
               sem):
        k32 = kb.bitcast(u32)
        v32 = vb.bitcast(u32)
        wq32 = wqb.bitcast(u32)
        wo32 = wob.bitcast(u32)

        def kcp(p0, p1, g):
            r = pl.ds(p0 * AH, (p1 - p0) * AH)
            return pltpu.make_async_copy(k_hbm.at[r, :, pl.ds(R0 // 16, NC2)], kb.at[r], sem.at[g])

        def vcp(p0, p1, g):
            r = pl.ds(p0 * 2 * AH, (p1 - p0) * 2 * AH)
            return pltpu.make_async_copy(v_hbm.at[r, pl.ds(R0, RW), :], vb.at[r], sem.at[g])

        w2cut = (0,) + W2CUT + (F,)
        groups = [[pltpu.make_async_copy(s_, d, sem.at[0])
                   for s_, d in [(x_hbm, xb), (wq_hbm, wqb), (wo_hbm, wob)]]]
        for kr, vr in KVG:
            g = len(groups)
            groups.append(([kcp(*kr, g)] if kr else []) + [vcp(*vr, g)])
        gffn = len(groups)
        groups.append([pltpu.make_async_copy(w1_hbm, w1, sem.at[gffn]),
                       pltpu.make_async_copy(w3_hbm, w3, sem.at[gffn])])
        for a_, b_ in zip(w2cut, w2cut[1:]):
            groups.append([pltpu.make_async_copy(w2_hbm.at[a_:b_], w2.at[a_:b_], sem.at[len(groups)])])
        for grp in groups:
            for cp in grp:
                cp.start()

        def gwait(g):
            for cp in groups[g]:
                cp.wait()

        def kvready(i):
            gwait(1 + i)
            kr = KVG[i][0]
            if kr:
                def swap(r, carry):
                    a = k32[r, 0, :, 4:8, :]
                    b = k32[r, 1, :, 0:4, :]
                    k32[r, 0, :, 4:8, :] = b
                    k32[r, 1, :, 0:4, :] = a
                    return carry
                lax.fori_loop(kr[0] * AH, kr[1] * AH, swap, 0)

        gwait(0)
        xs[...] = jnp.broadcast_to(xb[...].astype(f32), (8, D))


        def retile_wq(r, c):
            a = wq32[r, 0:24, 4:8, :]
            b = wq32[r, 24:48, 0:4, :]
            wq32[r, 0:24, 4:8, :] = b
            wq32[r, 24:48, 0:4, :] = a
            return c
        lax.fori_loop(0, D // 16, retile_wq, 0)

        def retile_wo(rb, c):
            r = pl.ds(rb * 4, 4)
            vals = {(e, cc): wo32[r, 4 * (5 * e + cc):4 * (5 * e + cc) + 4, :]
                    for e in range(2) for cc in range(5)}
            for (e, cc), v in vals.items():
                wo32[r, 8 * cc + 4 * e:8 * cc + 4 * e + 4, :] = v
            return c
        lax.fori_loop(0, HD // 64, retile_wo, 0)

        sub = lax.broadcasted_iota(jnp.int32, (8, 128), 0)
        lane = lax.broadcasted_iota(jnp.int32, (8, 128), 1)

        def qp_job(p, k, pin=lambda: ()):
            kk, t = divmod(k, 3)
            c = 3 * p + t
            qraw[p, 5 * t + kk] = _mm(lx[kk], wq32[8 * kk:8 * kk + 8, (c & 1) * 24 + (c >> 1)], 0, pin())

        def qprep(p):
            for t in range(3):
                qv = _tree(jnp.add, [qraw[p, 5 * t + kk] for kk in range(5)])
                qp = _pack(_bc(_ln_fix(qv, stat[0], stat[1])[0:1]))
                if t == 1:
                    qp = jnp.where((lane >> 6) == (sub >> 2), qp, jnp.uint32(0))
                lq[p, t] = qp

        def keep_rows(dst, t, c, r):
            g, j = divmod(c, 8)
            if t < 2:
                dst[0, t, g, j:j + 1, :] = r[j:j + 1]
            if t > 0:
                dst[1, t - 1, g, j:j + 1, :] = r[8 + j:9 + j]

        def qk_job(p, k, pin=lambda: ()):
            t, c = divmod(k, NC)
            if CORD & 1:
                c = (c & ~7) | ((c & 3) << 1) | ((c >> 2) & 1)
            r0 = p * AH + 8 * t
            keep_rows(sraw.at[p], t, c, _mm(lq[p, t], k32[r0:r0 + 8, c & 1, c >> 1], None, pin()))

        def pm_job(p, k, pin=lambda: ()):
            t, c = divmod(k, NC)
            if CORD & 2:
                c = (c & ~7) | ((c & 3) << 1) | ((c >> 2) & 1)
            a0 = p * 2 * AH + 16 * t + 8 * (c & 1)
            w = v32[a0:a0 + 8, 8 * (c >> 1):8 * (c >> 1) + 8, :]
            keep_rows(pmraw.at[p], t, c, _mm(lp[p, c // 8], w, None, pin()))

        def wo_job(p, k, pin=lambda: ()):
            t, cc = divmod(k, 5)
            r0 = 24 * p + 8 * t
            woraw[p, k] = _mm(lo[p, t], wo32[r0:r0 + 8, 8 * cc:8 * cc + 8, :], 0, pin())

        def allsub(op, x):
            for sh in (4, 2, 1):
                x = op(x, pltpu.roll(x, sh, 0))
            return x

        def scores(p, e):
            return [sraw[p, e, 0, g] + sraw[p, e, 1, g] for g in range(NC // 8)]

        def sm1_jobs(p, e):
            env = {}

            def head():
                s = scores(p, e)
                mv = allsub(jnp.maximum, _tree(jnp.maximum, s))
                st[p, e, 0] = mv
                env["p"] = [jnp.exp2(x - mv) for x in s]

            def lsum():
                st[p, e, 1] = allsub(jnp.add, _tree(jnp.add, env["p"]))

            def mk(c0):
                def job():
                    for c in range(c0, c0 + SMG):
                        pbuf[e, c] = _bc(env["p"][c // 8][c % 8:c % 8 + 1])
                return job
            return [head], [mk(c0) for c0 in range(0, NC, SMG)] + [lsum]

        def pv_jobs(p, e):
            jobs = []
            for a0 in range(0, AH, AB):
                accs = [None] * AB
                for c2 in range(NC2):
                    def job(a0=a0, c2=c2, accs=accs):
                        p0 = pbuf[e, 2 * c2]
                        p1 = pbuf[e, 2 * c2 + 1]
                        a = p * (2 * AH) + (e * AH + a0)
                        if VEC:
                            v = vb[a:a + AB, 16 * c2:16 * c2 + 16, :].astype(f32)
                            t = v[:, 0:8] * p0 + v[:, 8:16] * p1
                            accs[0] = t if accs[0] is None else accs[0] + t
                            if c2 == NC2 - 1:
                                oacc[p % RING, e, a0:a0 + AB] = accs[0]
                            return
                        for i in range(AB):
                            v = vb[a + i, 16 * c2:16 * c2 + 16, :].astype(f32)
                            t = v[0:8] * p0 + v[8:16] * p1
                            accs[i] = t if accs[i] is None else accs[i] + t
                        if c2 == NC2 - 1:
                            for i in range(AB):
                                oacc[p % RING, e, a0 + i] = accs[i]
                    jobs.append(job)
            return jobs

        def xmax(p):
            for e in range(2):
                st[p, e, 2] = _bc(jnp.max(st[p, e, 0], axis=1, keepdims=True))

        def scale_jobs(p):
            jobs = []
            for e in range(2):
                env = {}

                def head(e=e, env=env):
                    env["w"] = jnp.exp2(st[p, e, 0] - st[p, e, 2])
                    st[p, e, 1] = env["w"] * st[p, e, 1]
                jobs.append(head)
                for g in range(AH // ORG):
                    def job(e=e, env=env, g=g):
                        for a in range(ORG * g, ORG * g + ORG):
                            oacc[p % RING, e, a] = oacc[p % RING, e, a] * env["w"]
                    jobs.append(job)
            return jobs

        def xl(p):
            for e in range(2):
                st[p, e, 3] = _bc(jnp.sum(st[p, e, 1], axis=1, keepdims=True))

        def xsum(p):
            xl(p)
            for e in range(2):
                for a in range(AH):
                    r = _bc(jnp.sum(oacc[p % RING, e, a], axis=1, keepdims=True))
                    t, k = divmod(e * AH + a, 16)
                    otile[p, t, :, 8 * k:8 * k + 8] = r[:, 8 * k:8 * k + 8]

        def finish(p, tiles):
            inv = []
            for e in range(2):
                l = st[p, e, 3]
                r = pl.reciprocal(l, approx=True)
                inv.append(r * (2.0 - l * r))
            invs = [inv[0], jnp.where(lane < 64, inv[0], inv[1]), inv[1]]
            diag = (lane & 7) == sub
            for t in range(3):
                lo[p, t] = _pack(jnp.where(diag, tiles[t] * invs[t], 0.0))

        def or2(p):
            finish(p, [otile[p, t] for t in range(3)])

        def gs1(p):
            for e in range(2):
                st[p, e, 0] = allsub(jnp.maximum, _tree(jnp.maximum, scores(p, e)))

        def gs2(p):
            ps = [[jnp.exp2(x - st[p, e, 2]) for x in scores(p, e)] for e in range(2)]
            for e in range(2):
                st[p, e, 1] = allsub(jnp.add, _tree(jnp.add, ps[e]))
            for g in range(NC // 8):
                lp[p, g] = pltpu.bitcast(
                    jnp.concatenate([ps[0][g], ps[1][g]], axis=0).astype(bf16), u32)

        def orx(p):
            def part(e, t):
                return _tree(jnp.add, [pmraw[p, e, t, g] for g in range(NC // 8)])
            tiles = [part(0, 0), jnp.where(lane < 64, part(0, 1), part(1, 0)), part(1, 1)]
            finish(p, [allsub(jnp.add, x) for x in tiles])

        def woacc(p):
            for cc in range(5):
                xacc[cc] = xacc[cc] + (woraw[p, cc] + woraw[p, 5 + cc] + woraw[p, 10 + cc])

        mxu_fn = {"QP": qp_job, "QK": qk_job, "PM": pm_job, "WO": wo_job}
        xlu_fn = {"xmax": xmax, "xsum": xsum, "xl": xl}
        valu_fn = {"qprep": qprep, "or2": or2, "gs1": gs1, "gs2": gs2, "orx": orx, "woacc": woacc}
        plan_mxu, plan_small = _plan(3 * NC)

        def jobs_of(b):
            mx = [functools.partial(mxu_fn[kind], p, k)
                  for kind, p, k0, k1 in plan_mxu[b] for k in range(k0, k1)]
            xs_ = [functools.partial(xlu_fn[s], p) for s, p in plan_small[b] if s in xlu_fn]
            vs_ = [functools.partial(valu_fn[s], p) for s, p in plan_small[b] if s in valu_fn]
            sc = [j for s, p in plan_small[b] if s == "scale" for j in scale_jobs(p)]
            return mx, xs_, vs_, sc

        def block(b):
            p = VP[b]
            mx, xs_, vs_, sc = jobs_of(b)
            (sa1, sa2), (sb1, sb2) = sm1_jobs(p, 0), sm1_jobs(p, 1)
            pa, pb = pv_jobs(p, 0), pv_jobs(p, 1)
            cut = len(pb) - SKEW * NC2
            if b + 1 < len(VP):
                pb = pb[:cut]
            if b > 0 and SKEW:
                start = _weave(pv_jobs(VP[b - 1], 1)[cut:], sa1 + sa2, 0.0, 0.9)
                first = pa[:NC2]
                extra = vs_ + sc
            else:
                start = sa1 + vs_[:2] + sa2[:2]
                first = _weave(pa[:NC2], sa2[2:], 0.0, 1.0 - 1.0 * SMG / NC)
                extra = vs_[2:] + sc
            rest = _weave(pa[NC2:], sb1 + sb2, SMB0, SMB1)
            last = _weave(pb, extra, 0.0, 0.9) if extra else pb
            if PIN:
                outs = []
                for s_, q in plan_small[b]:
                    if s_ == "xsum":
                        outs += [otile.at[q, t] for t in range(3)]
                    if PINST and s_ in ("xsum", "xl", "xmax"):
                        outs += [st.at[q, e, 2 if s_ == "xmax" else 3] for e in range(2)]
                for n, ref in enumerate(outs):
                    k = int(len(mx) * PIN) + PINGAP * n
                    mx[k] = functools.partial(mx[k], pin=lambda ref=ref: (ref[...],))
            _run(mx[:MXF] + xs_ + _weave(start + first + rest + last, mx[MXF:], MX0, MX1))

        def ready_x():
            kvready(0)

            def tr(i, carry):
                a0 = pl.multiple_of((i >> 2) * 16, 16)
                for u in range(4):
                    c2 = (i & 3) * 4 + u
                    r = pl.multiple_of(c2 * 16, 16)
                    x = vb[pl.ds(a0, 16), pl.ds(r, 16), :]
                    ts = [x[:, 8 * h:8 * h + 8, :].reshape(128, 128).T for h in range(2)]
                    r8 = pl.multiple_of(c2 * 8, 8)
                    for h in range(2):
                        v32[pl.ds(a0 + 8 * h, 8), pl.ds(r8, 8), :] = (
                            pltpu.bitcast(ts[h], u32).reshape(8, 8, 128))
                return carry
            lax.fori_loop(0, NX * 3 * NC2 // 4, tr, 0)
        ready_x()

        def layer_body(layer, carry):
            first = layer == 0
            x = xs[...]
            xl = _ln_lhs(x)
            for kk in range(5):
                lx[kk] = _pack(xl[:, 128 * kk:128 * kk + 128])
            m, r = _ln_stats(x)
            stat[0] = _bc(m)
            stat[1] = _bc(r * qscale)
            xacc[...] = jnp.zeros_like(xacc)
            for p in VP[:3]:
                for k in range(15):
                    qp_job(p, k)
                qprep(p)
            for k in range(3 * NC):
                qk_job(VP[0], k)

            seen = 1
            for b in range(len(VP)):
                kp = max([p for kind, p, _, _ in plan_mxu[b] if kind == "QK"], default=0)
                need = max(i for i, (kr, vr) in enumerate(KVG)
                           if (kr and kr[0] <= kp < kr[1]) or vr[0] <= VP[b] < vr[1]) + 1
                if need > seen:
                    @pl.when(first)
                    def _(lo_=seen, hi_=need):
                        for i in range(lo_, hi_):
                            kvready(i)
                    seen = need
                if ONLY is not None and b not in ONLY:
                    continue

                @pl.when(layer < 100 + b)
                def _(b=b):
                    block(b)

            def finish_layer(wait):
                for b in range(len(VP), len(plan_mxu)):
                    mx, xs_, vs_, sc = jobs_of(b)
                    _run(xs_ + sc + vs_ + mx)
                att = jnp.sum(jnp.concatenate([xacc[cc] for cc in range(5)], axis=1),
                              axis=0, keepdims=True)
                x1 = _rnd(xs[...] + _rnd(att))
                if wait:
                    xs[...] = x1
                    gwait(gffn)
                m, r = _ln_stats(x1)
                xl = _ln_lhs(x1).astype(bf16)
                hs = []
                for j in range(0, F, FB):
                    g = _ln_fix(jnp.dot(xl, w1[:, j:j + FB], preferred_element_type=f32), m, r)
                    u = _ln_fix(jnp.dot(xl, w3[:, j:j + FB], preferred_element_type=f32), m, r)
                    hs.append((g * jax.nn.sigmoid(g) * u).astype(bf16))
                hh = jnp.concatenate(hs, axis=1)
                y = None
                for i, (a, b) in enumerate(zip(w2cut, w2cut[1:])):
                    if wait:
                        if i > 0:
                            xs[...] = y
                        gwait(gffn + 1 + i)
                        if i > 0:
                            y = xs[...]
                    for j in range(a, b, 128):
                        t = jnp.dot(hh[:, j:j + 128], w2[j:j + 128, :], preferred_element_type=f32)
                        y = t if y is None else y + t
                xs[...] = _rnd(x1 + _rnd(y[0:1]))
            lax.cond(first, lambda: finish_layer(True), lambda: finish_layer(False))
            return carry
        lax.fori_loop(0, NL, layer_body, 0)
        o_ref[...] = xs[0:1, :].astype(o_ref.dtype)
    return kernel


def _tile_linear(c):
    sk = c.shape[2]
    return (jnp.swapaxes(c, 2, 3).reshape(NA, 8, sk // 128, 128)
            .transpose(0, 2, 1, 3).reshape(NA, sk // 16, 128))


@jax.jit
def pallas_interleave_layers__sliding_block_cached__glu_gated_swiglu__decode_kernel(
    A_x: jax.Array,
    A_k_cache: jax.Array,
    A_v_cache: jax.Array,
    A_wq: jax.Array,
    A_wo: jax.Array,
    B_x: jax.Array,
    B_w1: jax.Array,
    B_w3: jax.Array,
    B_w2: jax.Array,
):
    SK = A_k_cache.shape[2]
    W = min(4096, max(256, SK // 4))
    kx = _tile_linear(A_k_cache).reshape(NA // 2, 2, SK // 256, 16, 128)
    vx = _tile_linear(A_v_cache)
    wqz = (A_wq.reshape(D // 16, 2, 8, 24, 2, 128).transpose(0, 1, 3, 4, 2, 5)
           .reshape(D // 16, 48, 16, 128))
    woz = (A_wo.reshape(HD // 16, 2, 8, 5, 128).transpose(0, 1, 3, 2, 4)
           .reshape(HD // 16, 80, 128))
    any_ = pl.BlockSpec(memory_space=pl.ANY)
    vm = pl.BlockSpec(memory_space=pltpu.VMEM)
    nc2 = W // 256
    out = pl.pallas_call(
        _make_kernel(SK, W),
        out_shape=jax.ShapeDtypeStruct((1, D), A_x.dtype),
        in_specs=[any_] * 8,
        out_specs=vm,
        scratch_shapes=[
            pltpu.VMEM((NA // 2, 2, nc2, 16, 128), bf16), pltpu.VMEM((NA, W // 16, 128), bf16),
            pltpu.VMEM((D // 16, 48, 16, 128), bf16), pltpu.VMEM((HD // 16, 80, 128), bf16),
            pltpu.VMEM((D, F), bf16), pltpu.VMEM((D, F), bf16), pltpu.VMEM((F, D), bf16),
            pltpu.VMEM((1, D), bf16),
            pltpu.VMEM((8, D), f32),
            pltpu.VMEM((5, 8, 128), u32),
            pltpu.VMEM((2, 8, 128), f32),
            pltpu.VMEM((NP, 15, 8, 128), f32),
            pltpu.VMEM((NP, 3, 8, 128), u32),
            pltpu.VMEM((NP, 2, 2, nc2 // 4, 8, 128), f32),
            pltpu.VMEM((2, 2 * nc2, 8, 128), f32),
            pltpu.VMEM((NP, 2, 4, 8, 128), f32),
            pltpu.VMEM((RING, 2, AH, 8, 128), f32),
            pltpu.VMEM((NP, 3, 8, 128), f32),
            pltpu.VMEM((NX, nc2 // 4, 8, 128), u32),
            pltpu.VMEM((NX, 2, 2, nc2 // 4, 8, 128), f32),
            pltpu.VMEM((NP, 3, 8, 128), u32),
            pltpu.VMEM((NP, 15, 8, 128), f32),
            pltpu.VMEM((5, 8, 128), f32),
            pltpu.SemaphoreType.DMA((len(KVG) + 3 + len(W2CUT),)),
        ],
        compiler_params=pltpu.CompilerParams(vmem_limit_bytes=126 * 1024 * 1024),
    )(A_x.reshape(1, D), kx, vx, wqz, woz, B_w1, B_w3, B_w2)
    return out.reshape(1, 1, D)
```

```python
import functools
import math
import jax
import jax.numpy as jnp
from jax import lax
import jax.experimental.pallas as pl
import jax.experimental.pallas.tpu as pltpu

H, DH, D, F = 32, 192, 640, 1536
HD = H * DH
EPS = 1e-5
NA = HD // 8
AH = DH // 8
NP = H // 2
MX0 = 0.0
MX1 = 1.02
AB = 4
SMG = 4
CAP = 140
CAPS = {0:128,13:152,7:144,11:144,12:144}
SKEW = 1
CORD = 0
PIN = 0.15
PINST = 1
PINGAP = 5
VEC = 1
MXF = 4
ONLY = None
NX = 2
XP = list(range(NX))
VP = list(range(NX, NP))
RING = 4
FB = 256
W2CUT = (1024,1408)
KVG = [((0, 4), (0, 4)), ((4, 8), (4, 8)), ((8, 12), (8, 12)), ((12, 16), (12, 14)), (None, (14, 16))]
ORG = 4
SMB0 = 0.1
SMB1 = 0.8
f32, bf16, u32 = jnp.float32, jnp.bfloat16, jnp.uint32


def _ln_stats(x):
    m = jnp.mean(x, axis=-1, keepdims=True)
    xc = x - m
    v = jnp.mean(xc * xc, axis=-1, keepdims=True)
    return m, lax.rsqrt(v + EPS)


def _ln_lhs(x):
    return jnp.where(lax.broadcasted_iota(jnp.int32, x.shape, 0) < 4, x, 1.0)


def _ln_fix(raw, m, r):
    return (raw - m * pltpu.roll(raw, 4, 0)) * r


def _rnd(x):
    return x.astype(bf16).astype(f32)


def _pack(x8):
    return pltpu.bitcast(jnp.concatenate([x8, x8], axis=0).astype(bf16), u32)


def _mm(lhs_u32, w_u32, half=0, pin=()):
    lhs = pltpu.bitcast(jnp.concatenate([lhs_u32] + [pltpu.bitcast(x, u32) for x in pin], axis=0)
                        if pin else lhs_u32, bf16)
    w = pltpu.bitcast(w_u32.reshape(64, 128), bf16)
    r = jnp.dot(lhs, w, preferred_element_type=f32)
    return r if half is None else r[8 * half:8 * half + 8]


def _bc(x):
    return jnp.broadcast_to(x, (8, 128))


def _tree(op, xs):
    xs = list(xs)
    while len(xs) > 1:
        xs = [op(xs[i], xs[i + 1]) if i + 1 < len(xs) else xs[i] for i in range(0, len(xs), 2)]
    return xs[0]


def _run(jobs):
    for j in jobs:
        j()


def _weave(main, extra, lo, hi):
    out, k = [], 0
    for n, j in enumerate(main):
        while k < len(extra) and lo * len(main) + k * (hi - lo) * len(main) / len(extra) <= n:
            out.append(extra[k])
            k += 1
        out.append(j)
    return out + list(extra[k:])


def _plan(nt):
    nb = len(VP)
    total = {"QP": 15, "QK": nt, "PM": nt, "WO": 15}
    done = {}
    fin = {}
    mxu, small = {}, {}

    def issue(b, kind, p, cap):
        k0 = done.get((kind, p), 0)
        n = min(total[kind] - k0, cap)
        if n > 0:
            mxu[b].append((kind, p, k0, k0 + n))
            done[(kind, p)] = k0 + n
            if k0 + n == total[kind]:
                fin[(kind, p)] = b
        return max(n, 0)

    def before(key, b):
        return fin.get(key, b) < b

    chains = {p: (["QP", "qprep", "QK", "gs1", "xmax", "gs2", "PM", "orx", "WO", "woacc"] if p in XP else
                  ["QP", "qprep", "QK", "pv", "xmax", "scale", "xsum", "or2", "WO", "woacc"])
              for p in range(NP)}
    for p in VP[:3]:
        done[("QP", p)] = 15
        fin[("QP", p)] = fin[("qprep", p)] = -1
    done[("QK", VP[0])] = nt
    fin[("QK", VP[0])] = -1
    b = 0
    while any(("woacc", p) not in fin for p in range(NP)):
        mxu[b], small[b] = [], []
        for p in range(NP):
            ch = chains[p]
            for prev, st in zip(ch, ch[1:]):
                if st in total or (st, p) in fin or not before((prev, p), b):
                    continue
                if st == "pv":
                    if b < nb and VP[b] == p:
                        fin[(st, p)] = b
                    continue
                small[b].append((st, p))
                fin[(st, p)] = b
                if st == "gs2":
                    small.setdefault(("late", b + 1), []).append(("xl", p))
        small[b] += small.pop(("late", b), [])
        cap = CAPS.get(b, CAP) if b < nb else 10 ** 6
        if b + 1 < nb:
            assert before(("qprep", VP[b + 1]), b)
            cap -= issue(b, "QK", VP[b + 1], nt)
        if b + 3 < nb:
            cap -= issue(b, "QP", VP[b + 3], 15)
        cands = [("QP", p, None) for p in XP] + [("QK", p, "qprep") for p in XP]
        cands += [("PM", p, "gs2") for p in XP] + [("QP", p, None) for p in VP]
        cands += [("WO", p, "orx" if p in XP else "or2") for p in VP + XP]
        cands += [("QK", p, "qprep") for p in VP]
        for kind, p, need in cands:
            if cap > 0 and (need is None or before((need, p), b)):
                cap -= issue(b, kind, p, cap)
        assert b >= nb or fin.get(("pv", VP[b])) == b
        b += 1
    return mxu, small


def _make_kernel(SK, W):
    NC = W // 128
    NC2 = NC // 2
    R0 = (SK - W) // 16
    RW = W // 16
    qscale = DH ** -0.5 * math.log2(math.e)

    def kernel(x_hbm, k_hbm, v_hbm, wq_hbm, wo_hbm, w1_hbm, w3_hbm, w2_hbm, o_ref,
               kb, vb, wqb, wob, w1, w3, w2,
               xb, xs, lx, stat, qraw, lq, sraw, pbuf, st, oacc, otile, lp, pmraw, lo, woraw, xacc,
               sem):
        k32 = kb.bitcast(u32)
        v32 = vb.bitcast(u32)
        wq32 = wqb.bitcast(u32)
        wo32 = wob.bitcast(u32)

        def kcp(p0, p1, g):
            r = pl.ds(p0 * AH, (p1 - p0) * AH)
            return pltpu.make_async_copy(k_hbm.at[r, :, pl.ds(R0 // 16, NC2)], kb.at[r], sem.at[g])

        def vcp(p0, p1, g):
            r = pl.ds(p0 * 2 * AH, (p1 - p0) * 2 * AH)
            return pltpu.make_async_copy(v_hbm.at[r, pl.ds(R0, RW), :], vb.at[r], sem.at[g])

        w2cut = (0,) + W2CUT + (F,)
        groups = [[pltpu.make_async_copy(s_, d, sem.at[0])
                   for s_, d in [(x_hbm, xb), (wq_hbm, wqb), (wo_hbm, wob)]]]
        for kr, vr in KVG:
            g = len(groups)
            groups.append(([kcp(*kr, g)] if kr else []) + [vcp(*vr, g)])
        gffn = len(groups)
        groups.append([pltpu.make_async_copy(w1_hbm, w1, sem.at[gffn]),
                       pltpu.make_async_copy(w3_hbm, w3, sem.at[gffn])])
        for a_, b_ in zip(w2cut, w2cut[1:]):
            groups.append([pltpu.make_async_copy(w2_hbm.at[a_:b_], w2.at[a_:b_], sem.at[len(groups)])])
        for grp in groups:
            for cp in grp:
                cp.start()

        def gwait(g):
            for cp in groups[g]:
                cp.wait()

        def kvready(i):
            gwait(1 + i)
            kr = KVG[i][0]
            if kr:
                def swap(r, carry):
                    a = k32[r, 0, :, 4:8, :]
                    b = k32[r, 1, :, 0:4, :]
                    k32[r, 0, :, 4:8, :] = b
                    k32[r, 1, :, 0:4, :] = a
                    return carry
                lax.fori_loop(kr[0] * AH, kr[1] * AH, swap, 0)

        gwait(0)


        def retile_wq(r, c):
            a = wq32[r, 0:24, 4:8, :]
            b = wq32[r, 24:48, 0:4, :]
            wq32[r, 0:24, 4:8, :] = b
            wq32[r, 24:48, 0:4, :] = a
            return c
        lax.fori_loop(0, D // 16, retile_wq, 0)

        def retile_wo(rb, c):
            r = pl.ds(rb * 4, 4)
            vals = {(e, cc): wo32[r, 4 * (5 * e + cc):4 * (5 * e + cc) + 4, :]
                    for e in range(2) for cc in range(5)}
            for (e, cc), v in vals.items():
                wo32[r, 8 * cc + 4 * e:8 * cc + 4 * e + 4, :] = v
            return c
        lax.fori_loop(0, HD // 64, retile_wo, 0)

        sub = lax.broadcasted_iota(jnp.int32, (8, 128), 0)
        lane = lax.broadcasted_iota(jnp.int32, (8, 128), 1)

        def qp_job(p, k, pin=lambda: ()):
            kk, t = divmod(k, 3)
            c = 3 * p + t
            qraw[p, 5 * t + kk] = _mm(lx[kk], wq32[8 * kk:8 * kk + 8, (c & 1) * 24 + (c >> 1)], 0, pin())

        def qprep(p):
            for t in range(3):
                qv = _tree(jnp.add, [qraw[p, 5 * t + kk] for kk in range(5)])
                qp = _pack(_bc(_ln_fix(qv, stat[0], stat[1])[0:1]))
                if t == 1:
                    qp = jnp.where((lane >> 6) == (sub >> 2), qp, jnp.uint32(0))
                lq[p, t] = qp

        def keep_rows(dst, t, c, r):
            g, j = divmod(c, 8)
            if t < 2:
                dst[0, t, g, j:j + 1, :] = r[j:j + 1]
            if t > 0:
                dst[1, t - 1, g, j:j + 1, :] = r[8 + j:9 + j]

        def qk_job(p, k, pin=lambda: ()):
            t, c = divmod(k, NC)
            if CORD & 1:
                c = (c & ~7) | ((c & 3) << 1) | ((c >> 2) & 1)
            r0 = p * AH + 8 * t
            keep_rows(sraw.at[p], t, c, _mm(lq[p, t], k32[r0:r0 + 8, c & 1, c >> 1], None, pin()))

        def pm_job(p, k, pin=lambda: ()):
            t, c = divmod(k, NC)
            if CORD & 2:
                c = (c & ~7) | ((c & 3) << 1) | ((c >> 2) & 1)
            a0 = p * 2 * AH + 16 * t + 8 * (c & 1)
            w = v32[a0:a0 + 8, 8 * (c >> 1):8 * (c >> 1) + 8, :]
            keep_rows(pmraw.at[p], t, c, _mm(lp[p, c // 8], w, None, pin()))

        def wo_job(p, k, pin=lambda: ()):
            t, cc = divmod(k, 5)
            r0 = 24 * p + 8 * t
            woraw[p, k] = _mm(lo[p, t], wo32[r0:r0 + 8, 8 * cc:8 * cc + 8, :], 0, pin())

        def allsub(op, x):
            for sh in (4, 2, 1):
                x = op(x, pltpu.roll(x, sh, 0))
            return x

        def scores(p, e):
            return [sraw[p, e, 0, g] + sraw[p, e, 1, g] for g in range(NC // 8)]

        def sm1_jobs(p, e):
            env = {}

            def head():
                s = scores(p, e)
                mv = allsub(jnp.maximum, _tree(jnp.maximum, s))
                st[p, e, 0] = mv
                env["p"] = [jnp.exp2(x - mv) for x in s]

            def lsum():
                st[p, e, 1] = allsub(jnp.add, _tree(jnp.add, env["p"]))

            def mk(c0):
                def job():
                    for c in range(c0, c0 + SMG):
                        pbuf[e, c] = _bc(env["p"][c // 8][c % 8:c % 8 + 1])
                return job
            return [head], [mk(c0) for c0 in range(0, NC, SMG)] + [lsum]

        def pv_jobs(p, e):
            jobs = []
            for a0 in range(0, AH, AB):
                accs = [None] * AB
                for c2 in range(NC2):
                    def job(a0=a0, c2=c2, accs=accs):
                        p0 = pbuf[e, 2 * c2]
                        p1 = pbuf[e, 2 * c2 + 1]
                        a = p * (2 * AH) + (e * AH + a0)
                        if VEC:
                            v = vb[a:a + AB, 16 * c2:16 * c2 + 16, :].astype(f32)
                            t = v[:, 0:8] * p0 + v[:, 8:16] * p1
                            accs[0] = t if accs[0] is None else accs[0] + t
                            if c2 == NC2 - 1:
                                oacc[p % RING, e, a0:a0 + AB] = accs[0]
                            return
                        for i in range(AB):
                            v = vb[a + i, 16 * c2:16 * c2 + 16, :].astype(f32)
                            t = v[0:8] * p0 + v[8:16] * p1
                            accs[i] = t if accs[i] is None else accs[i] + t
                        if c2 == NC2 - 1:
                            for i in range(AB):
                                oacc[p % RING, e, a0 + i] = accs[i]
                    jobs.append(job)
            return jobs

        def xmax(p):
            for e in range(2):
                st[p, e, 2] = _bc(jnp.max(st[p, e, 0], axis=1, keepdims=True))

        def scale_jobs(p):
            jobs = []
            for e in range(2):
                env = {}

                def head(e=e, env=env):
                    env["w"] = jnp.exp2(st[p, e, 0] - st[p, e, 2])
                    st[p, e, 1] = env["w"] * st[p, e, 1]
                jobs.append(head)
                for g in range(AH // ORG):
                    def job(e=e, env=env, g=g):
                        for a in range(ORG * g, ORG * g + ORG):
                            oacc[p % RING, e, a] = oacc[p % RING, e, a] * env["w"]
                    jobs.append(job)
            return jobs

        def xl(p):
            for e in range(2):
                st[p, e, 3] = _bc(jnp.sum(st[p, e, 1], axis=1, keepdims=True))

        def xsum(p):
            xl(p)
            for e in range(2):
                for a in range(AH):
                    r = _bc(jnp.sum(oacc[p % RING, e, a], axis=1, keepdims=True))
                    t, k = divmod(e * AH + a, 16)
                    otile[p, t, :, 8 * k:8 * k + 8] = r[:, 8 * k:8 * k + 8]

        def finish(p, tiles):
            inv = []
            for e in range(2):
                l = st[p, e, 3]
                r = pl.reciprocal(l, approx=True)
                inv.append(r * (2.0 - l * r))
            invs = [inv[0], jnp.where(lane < 64, inv[0], inv[1]), inv[1]]
            diag = (lane & 7) == sub
            for t in range(3):
                lo[p, t] = _pack(jnp.where(diag, tiles[t] * invs[t], 0.0))

        def or2(p):
            finish(p, [otile[p, t] for t in range(3)])

        def gs1(p):
            for e in range(2):
                st[p, e, 0] = allsub(jnp.maximum, _tree(jnp.maximum, scores(p, e)))

        def gs2(p):
            ps = [[jnp.exp2(x - st[p, e, 2]) for x in scores(p, e)] for e in range(2)]
            for e in range(2):
                st[p, e, 1] = allsub(jnp.add, _tree(jnp.add, ps[e]))
            for g in range(NC // 8):
                lp[p, g] = pltpu.bitcast(
                    jnp.concatenate([ps[0][g], ps[1][g]], axis=0).astype(bf16), u32)

        def orx(p):
            def part(e, t):
                return _tree(jnp.add, [pmraw[p, e, t, g] for g in range(NC // 8)])
            tiles = [part(0, 0), jnp.where(lane < 64, part(0, 1), part(1, 0)), part(1, 1)]
            finish(p, [allsub(jnp.add, x) for x in tiles])

        def woacc(p):
            for cc in range(5):
                xacc[cc] = xacc[cc] + (woraw[p, cc] + woraw[p, 5 + cc] + woraw[p, 10 + cc])

        mxu_fn = {"QP": qp_job, "QK": qk_job, "PM": pm_job, "WO": wo_job}
        xlu_fn = {"xmax": xmax, "xsum": xsum, "xl": xl}
        valu_fn = {"qprep": qprep, "or2": or2, "gs1": gs1, "gs2": gs2, "orx": orx, "woacc": woacc}
        plan_mxu, plan_small = _plan(3 * NC)

        def jobs_of(b):
            mx = [functools.partial(mxu_fn[kind], p, k)
                  for kind, p, k0, k1 in plan_mxu[b] for k in range(k0, k1)]
            xs_ = [functools.partial(xlu_fn[s], p) for s, p in plan_small[b] if s in xlu_fn]
            vs_ = [functools.partial(valu_fn[s], p) for s, p in plan_small[b] if s in valu_fn]
            sc = [j for s, p in plan_small[b] if s == "scale" for j in scale_jobs(p)]
            return mx, xs_, vs_, sc

        def block(b):
            p = VP[b]
            mx, xs_, vs_, sc = jobs_of(b)
            (sa1, sa2), (sb1, sb2) = sm1_jobs(p, 0), sm1_jobs(p, 1)
            pa, pb = pv_jobs(p, 0), pv_jobs(p, 1)
            cut = len(pb) - SKEW * NC2
            if b + 1 < len(VP):
                pb = pb[:cut]
            if b > 0 and SKEW:
                start = _weave(pv_jobs(VP[b - 1], 1)[cut:], sa1 + sa2, 0.0, 0.9)
                first = pa[:NC2]
                extra = vs_ + sc
            else:
                start = sa1 + vs_[:2] + sa2[:2]
                first = _weave(pa[:NC2], sa2[2:], 0.0, 1.0 - 1.0 * SMG / NC)
                extra = vs_[2:] + sc
            rest = _weave(pa[NC2:], sb1 + sb2, SMB0, SMB1)
            last = _weave(pb, extra, 0.0, 0.9) if extra else pb
            if PIN:
                outs = []
                for s_, q in plan_small[b]:
                    if s_ == "xsum":
                        outs += [otile.at[q, t] for t in range(3)]
                    if PINST and s_ in ("xsum", "xl", "xmax"):
                        outs += [st.at[q, e, 2 if s_ == "xmax" else 3] for e in range(2)]
                for n, ref in enumerate(outs):
                    k = int(len(mx) * PIN) + PINGAP * n
                    mx[k] = functools.partial(mx[k], pin=lambda ref=ref: (ref[...],))
            _run(mx[:MXF] + xs_ + _weave(start + first + rest + last, mx[MXF:], MX0, MX1))

        def ready_x():
            kvready(0)

            def tr(i, carry):
                a0 = pl.multiple_of((i >> 2) * 16, 16)
                for u in range(4):
                    c2 = (i & 3) * 4 + u
                    r = pl.multiple_of(c2 * 16, 16)
                    x = vb[pl.ds(a0, 16), pl.ds(r, 16), :]
                    ts = [x[:, 8 * h:8 * h + 8, :].reshape(128, 128).T for h in range(2)]
                    r8 = pl.multiple_of(c2 * 8, 8)
                    for h in range(2):
                        v32[pl.ds(a0 + 8 * h, 8), pl.ds(r8, 8), :] = (
                            pltpu.bitcast(ts[h], u32).reshape(8, 8, 128))
                return carry
            lax.fori_loop(0, NX * 3 * NC2 // 4, tr, 0)
        ready_x()

        def start_layer(x):
            xs[...] = x
            xl = _ln_lhs(x)
            for kk in range(5):
                lx[kk] = _pack(xl[:, 128 * kk:128 * kk + 128])
            m, r = _ln_stats(x)
            stat[0] = _bc(m)
            stat[1] = _bc(r * qscale)
            xacc[...] = jnp.zeros_like(xacc)
            for p in VP[:3]:
                for k in range(15):
                    qp_job(p, k)
                qprep(p)
            for k in range(3 * NC):
                qk_job(VP[0], k)

        start_layer(jnp.broadcast_to(xb[...].astype(f32), (8, D)))

        def layer_body(layer, carry):
            first = layer == 0
            seen = 1
            for b in range(len(VP)):
                kp = max([p for kind, p, _, _ in plan_mxu[b] if kind == "QK"], default=0)
                need = max(i for i, (kr, vr) in enumerate(KVG)
                           if (kr and kr[0] <= kp < kr[1]) or vr[0] <= VP[b] < vr[1]) + 1
                if need > seen:
                    @pl.when(first)
                    def _(lo_=seen, hi_=need):
                        for i in range(lo_, hi_):
                            kvready(i)
                    seen = need
                if ONLY is not None and b not in ONLY:
                    continue

                @pl.when(layer < 100 + b)
                def _(b=b):
                    block(b)

            def finish_layer(wait):
                for b in range(len(VP), len(plan_mxu)):
                    mx, xs_, vs_, sc = jobs_of(b)
                    _run(xs_ + sc + vs_ + mx)
                att = jnp.sum(jnp.concatenate([xacc[cc] for cc in range(5)], axis=1),
                              axis=0, keepdims=True)
                x1 = _rnd(xs[...] + _rnd(att))
                if wait:
                    xs[...] = x1
                    gwait(gffn)
                m, r = _ln_stats(x1)
                xl = _ln_lhs(x1).astype(bf16)
                hs = []
                for j in range(0, F, FB):
                    g = _ln_fix(jnp.dot(xl, w1[:, j:j + FB], preferred_element_type=f32), m, r)
                    u = _ln_fix(jnp.dot(xl, w3[:, j:j + FB], preferred_element_type=f32), m, r)
                    hs.append((g * jax.nn.sigmoid(g) * u).astype(bf16))
                hh = jnp.concatenate(hs, axis=1)
                y = None
                for i, (a, b) in enumerate(zip(w2cut, w2cut[1:])):
                    if wait:
                        if i > 0:
                            xs[...] = y
                        gwait(gffn + 1 + i)
                        if i > 0:
                            y = xs[...]
                    for j in range(a, b, 128):
                        t = jnp.dot(hh[:, j:j + 128], w2[j:j + 128, :], preferred_element_type=f32)
                        y = t if y is None else y + t
                if wait:
                    start_layer(_rnd(x1 + _rnd(y[0:1])))
                else:
                    o_ref[...] = (x1[0:1] + _rnd(y[0:1])).astype(o_ref.dtype)
            lax.cond(first, lambda: finish_layer(True), lambda: finish_layer(False))
            return carry
        lax.fori_loop(0, 2, layer_body, 0)
    return kernel


def _tile_linear(c):
    sk = c.shape[2]
    return (jnp.swapaxes(c, 2, 3).reshape(NA, 8, sk // 128, 128)
            .transpose(0, 2, 1, 3).reshape(NA, sk // 16, 128))


@jax.jit
def pallas_interleave_layers__sliding_block_cached__glu_gated_swiglu__decode_kernel(
    A_x: jax.Array,
    A_k_cache: jax.Array,
    A_v_cache: jax.Array,
    A_wq: jax.Array,
    A_wo: jax.Array,
    B_x: jax.Array,
    B_w1: jax.Array,
    B_w3: jax.Array,
    B_w2: jax.Array,
):
    SK = A_k_cache.shape[2]
    W = min(4096, max(256, SK // 4))
    kx = _tile_linear(A_k_cache).reshape(NA // 2, 2, SK // 256, 16, 128)
    vx = _tile_linear(A_v_cache)
    wqz = (A_wq.reshape(D // 16, 2, 8, 24, 2, 128).transpose(0, 1, 3, 4, 2, 5)
           .reshape(D // 16, 48, 16, 128))
    woz = (A_wo.reshape(HD // 16, 2, 8, 5, 128).transpose(0, 1, 3, 2, 4)
           .reshape(HD // 16, 80, 128))
    any_ = pl.BlockSpec(memory_space=pl.ANY)
    vm = pl.BlockSpec(memory_space=pltpu.VMEM)
    nc2 = W // 256
    out = pl.pallas_call(
        _make_kernel(SK, W),
        out_shape=jax.ShapeDtypeStruct((1, D), A_x.dtype),
        in_specs=[any_] * 8,
        out_specs=vm,
        scratch_shapes=[
            pltpu.VMEM((NA // 2, 2, nc2, 16, 128), bf16), pltpu.VMEM((NA, W // 16, 128), bf16),
            pltpu.VMEM((D // 16, 48, 16, 128), bf16), pltpu.VMEM((HD // 16, 80, 128), bf16),
            pltpu.VMEM((D, F), bf16), pltpu.VMEM((D, F), bf16), pltpu.VMEM((F, D), bf16),
            pltpu.VMEM((1, D), bf16),
            pltpu.VMEM((8, D), f32),
            pltpu.VMEM((5, 8, 128), u32),
            pltpu.VMEM((2, 8, 128), f32),
            pltpu.VMEM((NP, 15, 8, 128), f32),
            pltpu.VMEM((NP, 3, 8, 128), u32),
            pltpu.VMEM((NP, 2, 2, nc2 // 4, 8, 128), f32),
            pltpu.VMEM((2, 2 * nc2, 8, 128), f32),
            pltpu.VMEM((NP, 2, 4, 8, 128), f32),
            pltpu.VMEM((RING, 2, AH, 8, 128), f32),
            pltpu.VMEM((NP, 3, 8, 128), f32),
            pltpu.VMEM((NX, nc2 // 4, 8, 128), u32),
            pltpu.VMEM((NX, 2, 2, nc2 // 4, 8, 128), f32),
            pltpu.VMEM((NP, 3, 8, 128), u32),
            pltpu.VMEM((NP, 15, 8, 128), f32),
            pltpu.VMEM((5, 8, 128), f32),
            pltpu.SemaphoreType.DMA((len(KVG) + 3 + len(W2CUT),)),
        ],
        compiler_params=pltpu.CompilerParams(vmem_limit_bytes=126 * 1024 * 1024,
                                             disable_semaphore_checks=True),
    )(A_x.reshape(1, D), kx, vx, wqz, woz, B_w1, B_w3, B_w2)
    return out.reshape(1, 1, D)
```

```python
import functools
import math

import jax
import jax.numpy as jnp
from jax import lax
import jax.experimental.pallas as pl
import jax.experimental.pallas.tpu as pltpu

H, DH, D, F = 32, 192, 640, 1536
HD = H * DH
EPS = 1e-5
NA = HD // 8
AH = DH // 8
NP = H // 2
NX = 3
XP = list(range(NX))
VP = list(range(NX, NP))
NVQ = 6
VQ = (XP + VP[3:])[:NVQ]
VW = [3,4,5,6,15]
RING = 5
KVG = [((0, 5), (0, 4)), ((5, 8), (4, 8)), ((8, 12), (8, 12)), ((12, 16), (12, 14)), (None, (14, 16))]
W2CUT = (0, 1024, 1408, 1536)
AB = 4
SKEW = 1
VOFF = 55
VCOST = {"qprep": 10, "qprepv": 14, "scale": 14, "or2": 8, "woacc": 4, "gs1": 7, "gs2": 16,
         "orx": 18, "vwo": 186, "xsum": 4, "xq": 4}
CAPS = {}
XQMAX = 3
MXF = 4
MX1 = 1.02
MXP = 0.97
PIN = 0.15
PINGAP = 5
PINL = 36
SMG = 4
ORG = 4
FB = 256
ONLY = None
f32, bf16, u32 = jnp.float32, jnp.bfloat16, jnp.uint32


def _ln_stats(x):
    m = jnp.mean(x, axis=-1, keepdims=True)
    xc = x - m
    v = jnp.mean(xc * xc, axis=-1, keepdims=True)
    return m, lax.rsqrt(v + EPS)


def _ln_lhs(x):
    return jnp.where(lax.broadcasted_iota(jnp.int32, x.shape, 0) < 4, x, 1.0)


def _ln_fix(raw, m, r):
    return (raw - m * pltpu.roll(raw, 4, 0)) * r


def _rnd(x):
    return x.astype(bf16).astype(f32)


def _pack(lo, hi=None):
    return pltpu.bitcast(jnp.concatenate([lo, lo if hi is None else hi], axis=0).astype(bf16), u32)


def _tile(w_u32):
    return pltpu.bitcast(w_u32.reshape(64, 128), bf16)


def _mm(lhs_u32, w_u32, pin=()):
    if pin:
        lhs_u32 = jnp.concatenate([lhs_u32] + [pltpu.bitcast(x, u32) for x in pin], axis=0)
    return jnp.dot(pltpu.bitcast(lhs_u32, bf16), _tile(w_u32), preferred_element_type=f32)[0:16]


def _bc(x):
    return jnp.broadcast_to(x, (8, 128))


def _tree(op, xs):
    xs = list(xs)
    while len(xs) > 1:
        xs = [op(xs[i], xs[i + 1]) if i + 1 < len(xs) else xs[i] for i in range(0, len(xs), 2)]
    return xs[0]


def _allsub(op, x):
    for sh in (4, 2, 1):
        x = op(x, pltpu.roll(x, sh, 0))
    return x


def _recip(l):
    r = pl.reciprocal(l, approx=True)
    return r * (2.0 - l * r)


def _run(jobs):
    for j in jobs:
        j()


def _weave(main, extra, lo, hi):
    out, k = [], 0
    for n, j in enumerate(main):
        while k < len(extra) and lo * len(main) + k * (hi - lo) * len(main) / len(extra) <= n:
            out.append(extra[k])
            k += 1
        out.append(j)
    return out + list(extra[k:])


def _plan(nt):
    nb = len(VP)
    total = {"QP": 15, "QK": nt, "PM": nt, "WO": 15}
    done, fin, mxu, small = {}, {}, {}, {}

    def issue(b, kind, p, cap):
        k0 = done.get((kind, p), 0)
        n = max(min(total[kind] - k0, cap), 0)
        if n:
            mxu[b].append((kind, p, k0, k0 + n))
            done[(kind, p)] = k0 + n
            if k0 + n == total[kind]:
                fin[(kind, p)] = b
        return n

    def before(key, b):
        return fin.get(key, b) < b

    chains, qlast = {}, {}
    for p in range(NP):
        ch = ["vqp", "xq", "qprepv"] if p in VQ else ["QP", "qprep"]
        qlast[p] = ch[-1]
        if p in XP:
            ch += ["QK", "gs1", "xmax", "gs2", "PM", "orx", "WO", "woacc"]
        else:
            ch += ["QK", "pv", "xmax", "scale"]
            ch += ["xcol", "vwo"] if p in VW else ["xsum", "or2", "WO", "woacc"]
        chains[p] = ch
    for p in VQ:
        fin[("vqp", p)] = -1
    for p in VP[:3]:
        done[("QP", p)] = 15
        fin[("QP", p)] = fin[("qprep", p)] = -1
    done[("QK", VP[0])] = nt
    fin[("QK", VP[0])] = -1
    xq_order = sorted(VQ, key=lambda p: 2 * XP.index(p) + 1 if p in XP else 2 * (VP.index(p) - 3))
    late = []
    b = 0
    while any((chains[p][-1], p) not in fin for p in range(NP)):
        mxu[b], small[b], late = [], late, []
        for p in range(NP):
            for prev, st in zip(chains[p], chains[p][1:]):
                if st in total or (st, p) in fin or not before((prev, p), b):
                    continue
                if st == "xq" and xq_order.index(p) // XQMAX > b:
                    continue
                if st == "pv":
                    if b < nb and VP[b] == p:
                        fin[(st, p)] = b
                    continue
                small[b].append((st, p))
                fin[(st, p)] = b
                if st == "gs2":
                    late.append(("xl", p))
        cap = 10 ** 6
        if b < nb:
            nab = 12 - (SKEW if b == 0 else 0) + (SKEW if b == nb - 1 else 0)
            vload = 95 * nab + 31 + VOFF + sum(VCOST.get(s, 0) for s, _ in small[b])
            cap = CAPS.get(b, 4 * int(round((vload - 147) / 32.0)))
            assert fin.get(("pv", VP[b])) == b
        if b + 1 < nb:
            assert before((qlast[VP[b + 1]], VP[b + 1]), b)
            cap -= issue(b, "QK", VP[b + 1], nt)
        if b + 3 < nb and VP[b + 3] not in VQ:
            cap -= issue(b, "QP", VP[b + 3], 15)
        cands = [("QP", p, None) for p in XP if p not in VQ] + [("QK", p, qlast[p]) for p in XP]
        cands += [("PM", p, "gs2") for p in XP] + [("QP", p, None) for p in VP if p not in VQ]
        cands += [("WO", p, "orx" if p in XP else "or2") for p in VP + XP if p not in VW]
        cands += [("QK", p, qlast[p]) for p in VP]
        for kind, p, need in cands:
            if need is None or before((need, p), b):
                cap -= issue(b, kind, p, cap)
        b += 1
    return mxu, small


def _group_of(p, which):
    return next(i for i, g in enumerate(KVG) if g[which] and g[which][0] <= p < g[which][1])


def _make_kernel(SK, W):
    NC = W // 128
    NC2, NG = NC // 2, NC // 8
    qscale = DH ** -0.5 * math.log2(math.e)
    nk = sum(1 for kr, _ in KVG if kr)
    nv, nw2 = len(KVG), len(W2CUT) - 1

    def kernel(x_hbm, k_hbm, v_hbm, wq_hbm, wo_hbm, w1_hbm, w3_hbm, w2_hbm, o_ref, *scratch):
        kbs, vbs = scratch[:nk], scratch[nk:nk + nv]
        w2s = scratch[nk + nv:nk + nv + nw2]
        (wqb, wob, w1, w3, xb, xs, xrow, lx, stat, csum, qacc, qraw, lq, sraw, pbuf, st, oacc,
         otile, lp, pmraw, lo, woraw, xacc, sem) = scratch[nk + nv + nw2:]
        k32s = [r.bitcast(u32) for r in kbs]
        v32 = vbs[0].bitcast(u32)
        wq32 = wqb.bitcast(u32)
        wo32 = wob.bitcast(u32)

        groups = [[(x_hbm, xb), (wq_hbm, wqb), (wo_hbm, wob)]]
        for i, (kr, vr) in enumerate(KVG):
            grp = []
            if kr:
                grp.append((k_hbm.at[kr[0] * AH:kr[1] * AH, :, pl.ds((SK - W) // 256, NC2)], kbs[i]))
            grp.append((v_hbm.at[vr[0] * 2 * AH:vr[1] * 2 * AH, pl.ds((SK - W) // 16, W // 16), :], vbs[i]))
            groups.append(grp)
        gffn = len(groups)
        groups.append([(w1_hbm, w1), (w3_hbm, w3)])
        for i in range(nw2):
            groups.append([(w2_hbm.at[W2CUT[i]:W2CUT[i + 1]], w2s[i])])
        groups = [[pltpu.make_async_copy(s, d, sem.at[g]) for s, d in grp]
                  for g, grp in enumerate(groups)]
        for grp in groups:
            for cp in grp:
                cp.start()

        def gwait(g):
            for cp in groups[g]:
                cp.wait()

        sub = lax.broadcasted_iota(jnp.int32, (8, 128), 0)
        lane = lax.broadcasted_iota(jnp.int32, (8, 128), 1)

        def kvready(i):
            gwait(1 + i)
            if KVG[i][0]:
                k32 = k32s[i]

                def swap(r, carry):
                    a = k32[r, 0, :, 4:8, :]
                    b = k32[r, 1, :, 0:4, :]
                    k32[r, 0, :, 4:8, :] = b
                    k32[r, 1, :, 0:4, :] = a
                    return carry
                lax.fori_loop(0, k32.shape[0], swap, 0)

        def retile_wq(r, carry):
            a = wq32[r, 0:24, 4:8, :]
            b = wq32[r, 24:48, 0:4, :]
            wq32[r, 0:24, 4:8, :] = b
            wq32[r, 24:48, 0:4, :] = a
            return carry

        def retile_wo(rb, carry):
            r = pl.ds(rb * 4, 4)
            vals = {(e, cc): wo32[r, 4 * (5 * e + cc):4 * (5 * e + cc) + 4, :]
                    for e in range(2) for cc in range(5)}
            for (e, cc), v in vals.items():
                wo32[r, 8 * cc + 4 * e:8 * cc + 4 * e + 4, :] = v
            return carry

        def transpose_wq(i, carry):
            c = i + jnp.where(i >= 3 * NX, 9, 0)
            slot = (c & 1) * 24 + (c >> 1)
            ones = jnp.ones((16, 128), bf16)
            tiles = [_tile(wq32[8 * kk:8 * kk + 8, slot]) for kk in range(5)]
            csum[i] = _tree(jnp.add, [jnp.dot(ones, t, preferred_element_type=f32)[0:8] for t in tiles])
            for kk in range(5):
                wq32[8 * kk:8 * kk + 8, slot] = pltpu.bitcast(tiles[kk].T, u32).reshape(8, 8, 128)
            return carry

        def transpose_v(i, carry):
            a0 = pl.multiple_of((i >> 2) * 16, 16)
            for u in range(4):
                c2 = (i & 3) * 4 + u
                x = vbs[0][pl.ds(a0, 16), pl.ds(pl.multiple_of(c2 * 16, 16), 16), :]
                ts = [x[:, 8 * h:8 * h + 8, :].reshape(128, 128).T for h in range(2)]
                for h in range(2):
                    v32[pl.ds(a0 + 8 * h, 8), pl.ds(pl.multiple_of(c2 * 8, 8), 8), :] = (
                        pltpu.bitcast(ts[h], u32).reshape(8, 8, 128))
            return carry

        gwait(0)
        lax.fori_loop(0, D // 16, retile_wq, 0)
        lax.fori_loop(0, HD // 64, retile_wo, 0)
        if NVQ:
            lax.fori_loop(0, 3 * NVQ, transpose_wq, 0)
        kvready(0)
        lax.fori_loop(0, NX * 3 * NC2 // 4, transpose_v, 0)

        def wq_slot(p, t):
            c = 3 * p + t
            return (c & 1) * 24 + (c >> 1)

        def qp_job(p, k, pin=tuple):
            kk, t = divmod(k, 3)
            qraw[p, 5 * t + kk] = _mm(lx[kk], wq32[8 * kk:8 * kk + 8, wq_slot(p, t)], pin())[0:8]

        def keep_rows(dst, t, c, r):
            g, j = divmod(c, 8)
            if t < 2:
                dst[0, t, g, j:j + 1, :] = r[j:j + 1]
            if t > 0:
                dst[1, t - 1, g, j:j + 1, :] = r[8 + j:9 + j]

        def qk_job(p, k, pin=tuple):
            t, c = divmod(k, NC)
            g = _group_of(p, 0)
            r0 = (p - KVG[g][0][0]) * AH + 8 * t
            keep_rows(sraw.at[p], t, c, _mm(lq[p, t], k32s[g][r0:r0 + 8, c & 1, c >> 1], pin()))

        def pm_job(p, k, pin=tuple):
            t, c = divmod(k, NC)
            a0 = p * 2 * AH + 16 * t + 8 * (c & 1)
            w = v32[a0:a0 + 8, 8 * (c >> 1):8 * (c >> 1) + 8, :]
            keep_rows(pmraw.at[p], t, c, _mm(lp[p, c // 8], w, pin()))

        def wo_job(p, k, pin=tuple):
            t, cc = divmod(k, 5)
            r0 = 24 * p + 8 * t
            woraw[p, k] = _mm(lo[p, t], wo32[r0:r0 + 8, 8 * cc:8 * cc + 8, :], pin())[0:8]

        def lane_sums(p, src):
            for a in range(2 * AH):
                r = _bc(jnp.sum(src(a), axis=1, keepdims=True))
                t, k = divmod(a, 16)
                otile[p, t, :, 8 * k:8 * k + 8] = r[:, 8 * k:8 * k + 8]

        def xq(p):
            lane_sums(p, lambda a: qacc[VQ.index(p), a])

        def xmax(p):
            for e in range(2):
                st[p, e, 2] = _bc(jnp.max(st[p, e, 0], axis=1, keepdims=True))

        def xl(p):
            for e in range(2):
                st[p, e, 3] = _bc(jnp.sum(st[p, e, 1], axis=1, keepdims=True))

        def xsum(p):
            xl(p)
            lane_sums(p, lambda a: oacc[p % RING, a])

        def xcol(p):
            xl(p)
            for a in range(2 * AH):
                oacc[p % RING, a] = _bc(jnp.sum(oacc[p % RING, a], axis=1, keepdims=True))

        def store_lq(p, t, q):
            qp = _pack(q)
            if t == 1:
                qp = jnp.where((lane >> 6) == (sub >> 2), qp, jnp.uint32(0))
            lq[p, t] = qp

        def qprep(p):
            for t in range(3):
                qv = _tree(jnp.add, [qraw[p, 5 * t + kk] for kk in range(5)])
                store_lq(p, t, _bc(_ln_fix(qv, stat[0], stat[1])[0:1]))

        def vqp_jobs(p):
            def job(t, i):
                w = jnp.stack([wq32[8 * kk + i, wq_slot(p, t)] for kk in range(5)])
                w = pltpu.bitcast(w.reshape(40, 128), bf16).astype(f32).reshape(5, 2, 8, 128)
                acc = _tree(jnp.add, [w[kk] * xrow[kk] for kk in range(5)])
                qacc[VQ.index(p), 16 * t + 2 * i:16 * t + 2 * i + 2] = acc
            return [functools.partial(job, t, i) for t in range(3) for i in range(8)]

        def qprepv(p):
            for t in range(3):
                raw = _allsub(jnp.add, jnp.where((lane & 7) == sub, otile[p, t], 0.0))
                store_lq(p, t, (raw - stat[0] * csum[3 * VQ.index(p) + t]) * stat[1])

        def scores(p, e):
            return [sraw[p, e, 0, g] + sraw[p, e, 1, g] for g in range(NG)]

        def sm_jobs(p, e):
            env = {}

            def head():
                s = scores(p, e)
                mv = _allsub(jnp.maximum, _tree(jnp.maximum, s))
                st[p, e, 0] = mv
                env["p"] = [jnp.exp2(x - mv) for x in s]

            def spread(c0):
                for c in range(c0, c0 + SMG):
                    pbuf[e, c] = _bc(env["p"][c // 8][c % 8:c % 8 + 1])

            def lsum():
                st[p, e, 1] = _allsub(jnp.add, _tree(jnp.add, env["p"]))
            return [head] + [functools.partial(spread, c0) for c0 in range(0, NC, SMG)] + [lsum]

        def pv_jobs(p, e):
            g = _group_of(p, 1)

            def job(a0, c2, env):
                a = (p - KVG[g][1][0]) * 2 * AH + e * AH + a0
                v = vbs[g][a:a + AB, 16 * c2:16 * c2 + 16, :].astype(f32)
                t = v[:, 0:8] * pbuf[e, 2 * c2] + v[:, 8:16] * pbuf[e, 2 * c2 + 1]
                env["acc"] = t if c2 == 0 else env["acc"] + t
                if c2 == NC2 - 1:
                    oacc[p % RING, e * AH + a0:e * AH + a0 + AB] = env["acc"]
            jobs = []
            for a0 in range(0, AH, AB):
                env = {}
                jobs += [functools.partial(job, a0, c2, env) for c2 in range(NC2)]
            return jobs

        def scale_jobs(p):
            def head(e, env):
                env["w"] = jnp.exp2(st[p, e, 0] - st[p, e, 2])
                st[p, e, 1] = env["w"] * st[p, e, 1]

            def job(a, env):
                oacc[p % RING, a:a + ORG] = oacc[p % RING, a:a + ORG] * env["w"]
            jobs = []
            for e in range(2):
                env = {}
                jobs.append(functools.partial(head, e, env))
                jobs += [functools.partial(job, e * AH + a, env) for a in range(0, AH, ORG)]
            return jobs

        def store_lo(p, tiles):
            inv = [_recip(st[p, e, 3]) for e in range(2)]
            invs = [inv[0], jnp.where(lane < 64, inv[0], inv[1]), inv[1]]
            for t in range(3):
                lo[p, t] = _pack(jnp.where((lane & 7) == sub, tiles[t] * invs[t], 0.0))

        def or2(p):
            store_lo(p, [otile[p, t] for t in range(3)])

        def gs1(p):
            for e in range(2):
                st[p, e, 0] = _allsub(jnp.maximum, _tree(jnp.maximum, scores(p, e)))

        def gs2(p):
            ps = [[jnp.exp2(x - st[p, e, 2]) for x in scores(p, e)] for e in range(2)]
            for e in range(2):
                st[p, e, 1] = _allsub(jnp.add, _tree(jnp.add, ps[e]))
            for g in range(NG):
                lp[p, g] = _pack(ps[0][g], ps[1][g])

        def orx(p):
            def part(e, t):
                return _tree(jnp.add, [pmraw[p, e, t, g] for g in range(NG)])
            tiles = [part(0, 0), jnp.where(lane < 64, part(0, 1), part(1, 0)), part(1, 1)]
            store_lo(p, [_allsub(jnp.add, x) for x in tiles])

        def woacc(p):
            xacc[...] = xacc[...] + (woraw[p, 0:5] + woraw[p, 5:10] + woraw[p, 10:15])

        def vwo_jobs(p):
            def job(e, r, env):
                w = pltpu.bitcast(wo32[24 * p + 12 * e + r], bf16).astype(f32).reshape(5, 16, 128)
                a = e * AH + 2 * r
                t = w[:, 0:8] * oacc[p % RING, a] + w[:, 8:16] * oacc[p % RING, a + 1]
                env["acc"] = t if r == 0 else env["acc"] + t
                if r == AH // 2 - 1:
                    xacc[...] = xacc[...] + env["acc"] * _recip(st[p, e, 3])
            jobs = []
            for e in range(2):
                env = {}
                jobs += [functools.partial(job, e, r, env) for r in range(AH // 2)]
            return jobs

        mxu_fn = {"QP": qp_job, "QK": qk_job, "PM": pm_job, "WO": wo_job}
        xlu_fn = {"xq": xq, "xmax": xmax, "xl": xl, "xsum": xsum, "xcol": xcol}
        valu_fn = {"qprep": qprep, "qprepv": qprepv, "or2": or2, "gs1": gs1, "gs2": gs2, "orx": orx,
                   "woacc": woacc}
        plan_mxu, plan_small = _plan(3 * NC)

        def jobs_of(b):
            mx = [functools.partial(mxu_fn[kind], p, k)
                  for kind, p, k0, k1 in plan_mxu[b] for k in range(k0, k1)]
            xj = [functools.partial(xlu_fn[s], p) for s, p in plan_small[b] if s in xlu_fn]
            vj = [functools.partial(valu_fn[s], p) for s, p in plan_small[b] if s in valu_fn]
            sc = [j for s, p in plan_small[b] if s == "scale" for j in scale_jobs(p)]
            vw = [j for s, p in plan_small[b] if s == "vwo" for j in vwo_jobs(p)]
            return mx, xj, vj, sc, vw

        def block(b):
            p = VP[b]
            mx, xj, vj, sc, vw = jobs_of(b)
            sa, sb = sm_jobs(p, 0), sm_jobs(p, 1)
            pa, pb = pv_jobs(p, 0), pv_jobs(p, 1)
            cut = len(pb) - SKEW * NC2
            if b + 1 < len(VP):
                pb = pb[:cut]
            if b > 0:
                valu = _weave(pv_jobs(VP[b - 1], 1)[cut:], sa, 0.0, 0.9) + pa[:NC2]
            else:
                valu = sa[:3] + _weave(pa[:NC2], sa[3:], 0.0, 1.0 - 1.0 * SMG / NC)
            valu += _weave(pa[NC2:], sb, 0.1, 0.8) + vw
            valu += _weave(pb, vj + sc, 0.0, 0.9) if vj + sc else pb
            k = int(len(mx) * PIN)
            for s, q in plan_small[b]:
                refs = []
                if s in ("xsum", "xl", "xmax", "xcol"):
                    refs += [st.at[q, e, 2 if s == "xmax" else 3] for e in range(2)]
                if s in ("xsum", "xq"):
                    refs += [otile.at[q, t] for t in range(3)]
                for ref in refs:
                    mx[k] = functools.partial(mx[k], pin=lambda ref=ref: (ref[...],))
                    k += PINGAP
                if s == "xcol":
                    k = max(k, PINL)
                    for a in range(2 * AH - 3, 2 * AH):
                        ref = oacc.at[q % RING, a]
                        mx[k] = functools.partial(mx[k], pin=lambda ref=ref: (ref[...],))
                        k += 1
            _run(mx[:MXF] + xj + _weave(valu, mx[MXF:], 0.0, MX1))

        def set_x(x):
            xs[...] = x
            xl_ = _ln_lhs(x)
            for kk in range(5):
                xrow[kk] = x[:, 128 * kk:128 * kk + 128]
                lx[kk] = _pack(xl_[:, 128 * kk:128 * kk + 128])

        def prologue():
            def stats():
                m, r = _ln_stats(xs[...])
                stat[0] = _bc(m)
                stat[1] = _bc(r * qscale)
                xacc[...] = jnp.zeros_like(xacc)
            mx = [stats]
            for p in VP[:3]:
                mx += [functools.partial(qp_job, p, k) for k in range(15)]
                mx.append(functools.partial(qprep, p))
            mx += [functools.partial(qk_job, VP[0], k) for k in range(3 * NC)]
            bulk = [j for p in VQ for j in vqp_jobs(p)]
            _run(mx[:MXF + 1] + _weave(bulk, mx[MXF + 1:], 0.0, MXP) if bulk else mx)

        def finish_layer(first):
            for b in range(len(VP), len(plan_mxu)):
                mx, xj, vj, sc, vw = jobs_of(b)
                _run(xj + sc + vj + vw + mx)
            att = jnp.sum(jnp.concatenate([xacc[cc] for cc in range(5)], axis=1),
                          axis=0, keepdims=True)
            x1 = _rnd(xs[...] + _rnd(att))
            if first:
                xs[...] = x1
                gwait(gffn)
            m, r = _ln_stats(x1)
            xl_ = _ln_lhs(x1).astype(bf16)
            hs = []
            for j in range(0, F, FB):
                g = _ln_fix(jnp.dot(xl_, w1[:, j:j + FB], preferred_element_type=f32), m, r)
                u = _ln_fix(jnp.dot(xl_, w3[:, j:j + FB], preferred_element_type=f32), m, r)
                hs.append((g * jax.nn.sigmoid(g) * u).astype(bf16))
            hh = jnp.concatenate(hs, axis=1)
            y = None
            for i in range(nw2):
                if first:
                    if i:
                        xs[...] = y
                    gwait(gffn + 1 + i)
                    if i:
                        y = xs[...]
                for j in range(W2CUT[i], W2CUT[i + 1], 128):
                    t = jnp.dot(hh[:, j:j + 128], w2s[i][j - W2CUT[i]:j - W2CUT[i] + 128, :],
                                preferred_element_type=f32)
                    y = t if y is None else y + t
            if first:
                set_x(_rnd(x1 + _rnd(y[0:1])))
            else:
                o_ref[...] = (x1[0:1] + _rnd(y[0:1])).astype(o_ref.dtype)

        def layer_body(layer, carry):
            first = layer == 0
            prologue()
            seen = 1
            for b in range(len(VP)):
                need = 1 + max([_group_of(VP[b], 1)] + [_group_of(p, 0) for kind, p, _, _ in plan_mxu[b]
                                                        if kind == "QK"])
                if need > seen:
                    @pl.when(first)
                    def _(lo_=seen, hi_=need):
                        for i in range(lo_, hi_):
                            kvready(i)
                    seen = need
                if ONLY is None or b in ONLY:
                    pl.when(layer < 100 + b)(functools.partial(block, b))
            lax.cond(first, lambda: finish_layer(True), lambda: finish_layer(False))
            return carry

        set_x(jnp.broadcast_to(xb[...].astype(f32), (8, D)))
        lax.fori_loop(0, 2, layer_body, 0)
    return kernel


def _tile_linear(c):
    sk = c.shape[2]
    return (jnp.swapaxes(c, 2, 3).reshape(NA, 8, sk // 128, 128)
            .transpose(0, 2, 1, 3).reshape(NA, sk // 16, 128))


@jax.jit
def pallas_interleave_layers__sliding_block_cached__glu_gated_swiglu__decode_kernel(
    A_x: jax.Array,
    A_k_cache: jax.Array,
    A_v_cache: jax.Array,
    A_wq: jax.Array,
    A_wo: jax.Array,
    B_x: jax.Array,
    B_w1: jax.Array,
    B_w3: jax.Array,
    B_w2: jax.Array,
):
    SK = A_k_cache.shape[2]
    W = min(4096, max(256, SK // 4))
    nc2 = W // 256
    kx = _tile_linear(A_k_cache).reshape(NA // 2, 2, SK // 256, 16, 128)
    vx = _tile_linear(A_v_cache)
    wqz = (A_wq.reshape(D // 16, 2, 8, 24, 2, 128).transpose(0, 1, 3, 4, 2, 5)
           .reshape(D // 16, 48, 16, 128))
    woz = (A_wo.reshape(HD // 16, 2, 8, 5, 128).transpose(0, 1, 3, 2, 4)
           .reshape(HD // 16, 80, 128))
    vreg = lambda *lead, dt=f32: pltpu.VMEM(lead + (8, 128), dt)
    scratch = [pltpu.VMEM(((kr[1] - kr[0]) * AH, 2, nc2, 16, 128), bf16) for kr, _ in KVG if kr]
    scratch += [pltpu.VMEM(((vr[1] - vr[0]) * 2 * AH, W // 16, 128), bf16) for _, vr in KVG]
    scratch += [pltpu.VMEM((b - a, D), bf16) for a, b in zip(W2CUT, W2CUT[1:])]
    scratch += [
        pltpu.VMEM((D // 16, 48, 16, 128), bf16),
        pltpu.VMEM((HD // 16, 80, 128), bf16),
        pltpu.VMEM((D, F), bf16),
        pltpu.VMEM((D, F), bf16),
        pltpu.VMEM((1, D), bf16),
        pltpu.VMEM((8, D), f32),
        vreg(5),
        vreg(5, dt=u32),
        vreg(2),
        vreg(max(3 * NVQ, 1)),
        vreg(max(NVQ, 1), 2 * AH),
        vreg(NP, 15),
        vreg(NP, 3, dt=u32),
        vreg(NP, 2, 2, nc2 // 4),
        vreg(2, 2 * nc2),
        vreg(NP, 2, 4),
        vreg(RING, 2 * AH),
        vreg(NP, 3),
        vreg(NX, nc2 // 4, dt=u32),
        vreg(NX, 2, 2, nc2 // 4),
        vreg(NP, 3, dt=u32),
        vreg(NP, 15),
        vreg(5),
        pltpu.SemaphoreType.DMA((len(KVG) + 1 + len(W2CUT),)),
    ]
    out = pl.pallas_call(
        _make_kernel(SK, W),
        out_shape=jax.ShapeDtypeStruct((1, D), A_x.dtype),
        in_specs=[pl.BlockSpec(memory_space=pl.ANY)] * 8,
        out_specs=pl.BlockSpec(memory_space=pltpu.VMEM),
        scratch_shapes=scratch,
        compiler_params=pltpu.CompilerParams(vmem_limit_bytes=126 * 1024 * 1024,
                                             disable_semaphore_checks=True),
    )(A_x.reshape(1, D), kx, vx, wqz, woz, B_w1, B_w3, B_w2)
    return out.reshape(1, 1, D)
```

```python
import functools
import math

import jax
import jax.numpy as jnp
from jax import lax
import jax.experimental.pallas as pl
import jax.experimental.pallas.tpu as pltpu

H, DH, D, F = 32, 192, 640, 1536
HD = H * DH
EPS = 1e-5
NA = HD // 8
AH = DH // 8
NP = H // 2
NX = 3
XP = list(range(NX))
VP = list(range(NX, NP))
NVQ = 6
VQ = (XP + VP[3:])[:NVQ]
VW = [3,4,5,6,15]
RING = 5
KVG = [((0, 5), (0, 4)), ((5, 8), (4, 8)), ((8, 12), (8, 12)), ((12, 16), (12, 14)), (None, (14, 16))]
W2CUT = (0, 1024, 1408, 1536)
AB = 4
SKEW = 1
VOFF = 55
VCOST = {"qprep": 10, "qprepv": 14, "scale": 14, "or2": 8, "woacc": 4, "gs1": 7, "gs2": 16,
         "orx": 18, "vwo": 186, "xsum": 4, "xq": 4}
CAPS = {0:124,1:144,2:148,3:140,4:164,5:164,6:164,7:164,8:144,9:144,10:144,11:140,12:152}
XQMAX = 3
MXF = 4
MX1 = 1.02
MXP = 0.97
PIN = 0.15
PINGAP = 5
PINL = 36
SMG = 4
ORG = 4
NVH = 7
ONLY = None
f32, bf16, u32 = jnp.float32, jnp.bfloat16, jnp.uint32


def _ln_stats(x):
    m = jnp.mean(x, axis=-1, keepdims=True)
    xc = x - m
    v = jnp.mean(xc * xc, axis=-1, keepdims=True)
    return m, lax.rsqrt(v + EPS)


def _ln_lhs(x):
    return jnp.where(lax.broadcasted_iota(jnp.int32, x.shape, 0) < 4, x, 1.0)


def _ln_fix(raw, m, r):
    return (raw - m * pltpu.roll(raw, 4, 0)) * r


def _rnd(x):
    return x.astype(bf16).astype(f32)


def _pack(lo, hi=None):
    return pltpu.bitcast(jnp.concatenate([lo, lo if hi is None else hi], axis=0).astype(bf16), u32)


def _tile(w_u32):
    return pltpu.bitcast(w_u32.reshape(64, 128), bf16)


def _mm(lhs_u32, w_u32, pin=()):
    if pin:
        lhs_u32 = jnp.concatenate([lhs_u32] + [pltpu.bitcast(x, u32) for x in pin], axis=0)
    return jnp.dot(pltpu.bitcast(lhs_u32, bf16), _tile(w_u32), preferred_element_type=f32)[0:16]


def _bc(x):
    return jnp.broadcast_to(x, (8, 128))


def _tree(op, xs):
    xs = list(xs)
    while len(xs) > 1:
        xs = [op(xs[i], xs[i + 1]) if i + 1 < len(xs) else xs[i] for i in range(0, len(xs), 2)]
    return xs[0]


def _allsub(op, x):
    for sh in (4, 2, 1):
        x = op(x, pltpu.roll(x, sh, 0))
    return x


def _recip(l):
    r = pl.reciprocal(l, approx=True)
    return r * (2.0 - l * r)


def _run(jobs):
    for j in jobs:
        j()


def _weave(main, extra, lo, hi):
    out, k = [], 0
    for n, j in enumerate(main):
        while k < len(extra) and lo * len(main) + k * (hi - lo) * len(main) / len(extra) <= n:
            out.append(extra[k])
            k += 1
        out.append(j)
    return out + list(extra[k:])


def _plan(nt):
    nb = len(VP)
    total = {"QP": 15, "QK": nt, "PM": nt, "WO": 15}
    done, fin, mxu, small = {}, {}, {}, {}

    def issue(b, kind, p, cap):
        k0 = done.get((kind, p), 0)
        n = max(min(total[kind] - k0, cap), 0)
        if n:
            mxu[b].append((kind, p, k0, k0 + n))
            done[(kind, p)] = k0 + n
            if k0 + n == total[kind]:
                fin[(kind, p)] = b
        return n

    def before(key, b):
        return fin.get(key, b) < b

    chains, qlast = {}, {}
    for p in range(NP):
        ch = ["vqp", "xq", "qprepv"] if p in VQ else ["QP", "qprep"]
        qlast[p] = ch[-1]
        if p in XP:
            ch += ["QK", "gs1", "xmax", "gs2", "PM", "orx", "WO", "woacc"]
        else:
            ch += ["QK", "pv", "xmax", "scale"]
            ch += ["xcol", "vwo"] if p in VW else ["xsum", "or2", "WO", "woacc"]
        chains[p] = ch
    for p in VQ:
        fin[("vqp", p)] = -1
    for p in VP[:3]:
        done[("QP", p)] = 15
        fin[("QP", p)] = fin[("qprep", p)] = -1
    done[("QK", VP[0])] = nt
    fin[("QK", VP[0])] = -1
    xq_order = sorted(VQ, key=lambda p: 2 * XP.index(p) + 1 if p in XP else 2 * (VP.index(p) - 3))
    late = []
    b = 0
    while any((chains[p][-1], p) not in fin for p in range(NP)):
        mxu[b], small[b], late = [], late, []
        for p in range(NP):
            for prev, st in zip(chains[p], chains[p][1:]):
                if st in total or (st, p) in fin or not before((prev, p), b):
                    continue
                if st == "xq" and xq_order.index(p) // XQMAX > b:
                    continue
                if st == "pv":
                    if b < nb and VP[b] == p:
                        fin[(st, p)] = b
                    continue
                small[b].append((st, p))
                fin[(st, p)] = b
                if st == "gs2":
                    late.append(("xl", p))
        cap = 10 ** 6
        if b < nb:
            nab = 12 - (SKEW if b == 0 else 0) + (SKEW if b == nb - 1 else 0)
            vload = 95 * nab + 31 + VOFF + sum(VCOST.get(s, 0) for s, _ in small[b])
            cap = CAPS.get(b, 4 * int(round((vload - 147) / 32.0)))
            assert fin.get(("pv", VP[b])) == b
        if b + 1 < nb:
            assert before((qlast[VP[b + 1]], VP[b + 1]), b)
            cap -= issue(b, "QK", VP[b + 1], nt)
        if b + 3 < nb and VP[b + 3] not in VQ:
            cap -= issue(b, "QP", VP[b + 3], 15)
        cands = [("QP", p, None) for p in XP if p not in VQ] + [("QK", p, qlast[p]) for p in XP]
        cands += [("PM", p, "gs2") for p in XP] + [("QP", p, None) for p in VP if p not in VQ]
        cands += [("WO", p, "orx" if p in XP else "or2") for p in VP + XP if p not in VW]
        cands += [("QK", p, qlast[p]) for p in VP]
        for kind, p, need in cands:
            if need is None or before((need, p), b):
                cap -= issue(b, kind, p, cap)
        b += 1
    return mxu, small


def _group_of(p, which):
    return next(i for i, g in enumerate(KVG) if g[which] and g[which][0] <= p < g[which][1])


def _make_kernel(SK, W):
    NC = W // 128
    NC2, NG = NC // 2, NC // 8
    qscale = DH ** -0.5 * math.log2(math.e)
    nk = sum(1 for kr, _ in KVG if kr)
    nv, nw2 = len(KVG), len(W2CUT) - 1

    def kernel(x_hbm, k_hbm, v_hbm, wq_hbm, wo_hbm, w1_hbm, w3_hbm, w2_hbm, o_ref, *scratch):
        kbs, vbs = scratch[:nk], scratch[nk:nk + nv]
        w2s = scratch[nk + nv:nk + nv + nw2]
        (wqb, wob, w1, w3, xb, xs, xrow, lx, stat, csum, qacc, qraw, lq, sraw, pbuf, st, oacc,
         otile, lp, pmraw, lo, woraw, xacc, hcol, sem) = scratch[nk + nv + nw2:]
        k32s = [r.bitcast(u32) for r in kbs]
        v32 = vbs[0].bitcast(u32)
        wq32 = wqb.bitcast(u32)
        wo32 = wob.bitcast(u32)
        wg32 = [w1.bitcast(u32), w3.bitcast(u32)]

        groups = [[(x_hbm, xb), (wq_hbm, wqb), (wo_hbm, wob)]]
        for i, (kr, vr) in enumerate(KVG):
            grp = []
            if kr:
                grp.append((k_hbm.at[kr[0] * AH:kr[1] * AH, :, pl.ds((SK - W) // 256, NC2)], kbs[i]))
            grp.append((v_hbm.at[vr[0] * 2 * AH:vr[1] * 2 * AH, pl.ds((SK - W) // 16, W // 16), :], vbs[i]))
            groups.append(grp)
        gffn = len(groups)
        groups += [[(w1_hbm, w1)], [(w3_hbm, w3)]]
        for i in range(nw2):
            groups.append([(w2_hbm.at[W2CUT[i]:W2CUT[i + 1]], w2s[i])])
        groups = [[pltpu.make_async_copy(s, d, sem.at[g]) for s, d in grp]
                  for g, grp in enumerate(groups)]
        for grp in groups:
            for cp in grp:
                cp.start()

        def gwait(g):
            for cp in groups[g]:
                cp.wait()

        sub = lax.broadcasted_iota(jnp.int32, (8, 128), 0)
        lane = lax.broadcasted_iota(jnp.int32, (8, 128), 1)

        def kvready(i):
            gwait(1 + i)
            if KVG[i][0]:
                k32 = k32s[i]

                def swap(r, carry):
                    a = k32[r, 0, :, 4:8, :]
                    b = k32[r, 1, :, 0:4, :]
                    k32[r, 0, :, 4:8, :] = b
                    k32[r, 1, :, 0:4, :] = a
                    return carry
                lax.fori_loop(0, k32.shape[0], swap, 0)

        def retile(w32, rows):
            n = w32.shape[1] // 2

            def body(rb, carry):
                r = pl.ds(rb * rows, rows)
                a = w32[r, 0:n, 4:8, :]
                b = w32[r, n:2 * n, 0:4, :]
                w32[r, 0:n, 4:8, :] = b
                w32[r, n:2 * n, 0:4, :] = a
                return carry
            lax.fori_loop(0, w32.shape[0] // rows, body, 0)

        def retile_wo(rb, carry):
            r = pl.ds(rb * 4, 4)
            vals = {(e, cc): wo32[r, 4 * (5 * e + cc):4 * (5 * e + cc) + 4, :]
                    for e in range(2) for cc in range(5)}
            for (e, cc), v in vals.items():
                wo32[r, 8 * cc + 4 * e:8 * cc + 4 * e + 4, :] = v
            return carry

        def transpose_wq(i, carry):
            c = i + jnp.where(i >= 3 * NX, 9, 0)
            slot = (c & 1) * 24 + (c >> 1)
            ones = jnp.ones((16, 128), bf16)
            tiles = [_tile(wq32[8 * kk:8 * kk + 8, slot]) for kk in range(5)]
            csum[i] = _tree(jnp.add, [jnp.dot(ones, t, preferred_element_type=f32)[0:8] for t in tiles])
            for kk in range(5):
                wq32[8 * kk:8 * kk + 8, slot] = pltpu.bitcast(tiles[kk].T, u32).reshape(8, 8, 128)
            return carry

        def transpose_v(i, carry):
            a0 = pl.multiple_of((i >> 2) * 16, 16)
            for u in range(4):
                c2 = (i & 3) * 4 + u
                x = vbs[0][pl.ds(a0, 16), pl.ds(pl.multiple_of(c2 * 16, 16), 16), :]
                ts = [x[:, 8 * h:8 * h + 8, :].reshape(128, 128).T for h in range(2)]
                for h in range(2):
                    v32[pl.ds(a0 + 8 * h, 8), pl.ds(pl.multiple_of(c2 * 8, 8), 8), :] = (
                        pltpu.bitcast(ts[h], u32).reshape(8, 8, 128))
            return carry

        gwait(0)
        retile(wq32, 1)
        lax.fori_loop(0, HD // 64, retile_wo, 0)
        if NVQ:
            lax.fori_loop(0, 3 * NVQ, transpose_wq, 0)
        kvready(0)
        lax.fori_loop(0, NX * 3 * NC2 // 4, transpose_v, 0)

        def wq_slot(p, t):
            c = 3 * p + t
            return (c & 1) * 24 + (c >> 1)

        def qp_job(p, k, pin=tuple):
            kk, t = divmod(k, 3)
            qraw[p, 5 * t + kk] = _mm(lx[kk], wq32[8 * kk:8 * kk + 8, wq_slot(p, t)], pin())[0:8]

        def keep_rows(dst, t, c, r):
            g, j = divmod(c, 8)
            if t < 2:
                dst[0, t, g, j:j + 1, :] = r[j:j + 1]
            if t > 0:
                dst[1, t - 1, g, j:j + 1, :] = r[8 + j:9 + j]

        def qk_job(p, k, pin=tuple):
            t, c = divmod(k, NC)
            g = _group_of(p, 0)
            r0 = (p - KVG[g][0][0]) * AH + 8 * t
            keep_rows(sraw.at[p], t, c, _mm(lq[p, t], k32s[g][r0:r0 + 8, c & 1, c >> 1], pin()))

        def pm_job(p, k, pin=tuple):
            t, c = divmod(k, NC)
            a0 = p * 2 * AH + 16 * t + 8 * (c & 1)
            w = v32[a0:a0 + 8, 8 * (c >> 1):8 * (c >> 1) + 8, :]
            keep_rows(pmraw.at[p], t, c, _mm(lp[p, c // 8], w, pin()))

        def wo_job(p, k, pin=tuple):
            t, cc = divmod(k, 5)
            r0 = 24 * p + 8 * t
            woraw[p, k] = _mm(lo[p, t], wo32[r0:r0 + 8, 8 * cc:8 * cc + 8, :], pin())[0:8]

        def lane_sums(p, src):
            for a in range(2 * AH):
                r = _bc(jnp.sum(src(a), axis=1, keepdims=True))
                t, k = divmod(a, 16)
                otile[p, t, :, 8 * k:8 * k + 8] = r[:, 8 * k:8 * k + 8]

        def xq(p):
            lane_sums(p, lambda a: qacc[VQ.index(p), a])

        def xmax(p):
            for e in range(2):
                st[p, e, 2] = _bc(jnp.max(st[p, e, 0], axis=1, keepdims=True))

        def xl(p):
            for e in range(2):
                st[p, e, 3] = _bc(jnp.sum(st[p, e, 1], axis=1, keepdims=True))

        def xsum(p):
            xl(p)
            lane_sums(p, lambda a: oacc[p % RING, a])

        def xcol(p):
            xl(p)
            for a in range(2 * AH):
                oacc[p % RING, a] = _bc(jnp.sum(oacc[p % RING, a], axis=1, keepdims=True))

        def store_lq(p, t, q):
            qp = _pack(q)
            if t == 1:
                qp = jnp.where((lane >> 6) == (sub >> 2), qp, jnp.uint32(0))
            lq[p, t] = qp

        def qprep(p):
            for t in range(3):
                qv = _tree(jnp.add, [qraw[p, 5 * t + kk] for kk in range(5)])
                store_lq(p, t, _bc(_ln_fix(qv, stat[0], stat[1])[0:1]))

        def vqp_jobs(p):
            def job(t, i):
                w = jnp.stack([wq32[8 * kk + i, wq_slot(p, t)] for kk in range(5)])
                w = pltpu.bitcast(w.reshape(40, 128), bf16).astype(f32).reshape(5, 2, 8, 128)
                acc = _tree(jnp.add, [w[kk] * xrow[kk] for kk in range(5)])
                qacc[VQ.index(p), 16 * t + 2 * i:16 * t + 2 * i + 2] = acc
            return [functools.partial(job, t, i) for t in range(3) for i in range(8)]

        def qprepv(p):
            for t in range(3):
                raw = _allsub(jnp.add, jnp.where((lane & 7) == sub, otile[p, t], 0.0))
                store_lq(p, t, (raw - stat[0] * csum[3 * VQ.index(p) + t]) * stat[1])

        def scores(p, e):
            return [sraw[p, e, 0, g] + sraw[p, e, 1, g] for g in range(NG)]

        def sm_jobs(p, e):
            env = {}

            def head():
                s = scores(p, e)
                mv = _allsub(jnp.maximum, _tree(jnp.maximum, s))
                st[p, e, 0] = mv
                env["p"] = [jnp.exp2(x - mv) for x in s]

            def spread(c0):
                for c in range(c0, c0 + SMG):
                    pbuf[e, c] = _bc(env["p"][c // 8][c % 8:c % 8 + 1])

            def lsum():
                st[p, e, 1] = _allsub(jnp.add, _tree(jnp.add, env["p"]))
            return [head] + [functools.partial(spread, c0) for c0 in range(0, NC, SMG)] + [lsum]

        def pv_jobs(p, e):
            g = _group_of(p, 1)

            def job(a0, c2, env):
                a = (p - KVG[g][1][0]) * 2 * AH + e * AH + a0
                v = vbs[g][a:a + AB, 16 * c2:16 * c2 + 16, :].astype(f32)
                t = v[:, 0:8] * pbuf[e, 2 * c2] + v[:, 8:16] * pbuf[e, 2 * c2 + 1]
                env["acc"] = t if c2 == 0 else env["acc"] + t
                if c2 == NC2 - 1:
                    oacc[p % RING, e * AH + a0:e * AH + a0 + AB] = env["acc"]
            jobs = []
            for a0 in range(0, AH, AB):
                env = {}
                jobs += [functools.partial(job, a0, c2, env) for c2 in range(NC2)]
            return jobs

        def scale_jobs(p):
            def head(e, env):
                env["w"] = jnp.exp2(st[p, e, 0] - st[p, e, 2])
                st[p, e, 1] = env["w"] * st[p, e, 1]

            def job(a, env):
                oacc[p % RING, a:a + ORG] = oacc[p % RING, a:a + ORG] * env["w"]
            jobs = []
            for e in range(2):
                env = {}
                jobs.append(functools.partial(head, e, env))
                jobs += [functools.partial(job, e * AH + a, env) for a in range(0, AH, ORG)]
            return jobs

        def store_lo(p, tiles):
            inv = [_recip(st[p, e, 3]) for e in range(2)]
            invs = [inv[0], jnp.where(lane < 64, inv[0], inv[1]), inv[1]]
            for t in range(3):
                lo[p, t] = _pack(jnp.where((lane & 7) == sub, tiles[t] * invs[t], 0.0))

        def or2(p):
            store_lo(p, [otile[p, t] for t in range(3)])

        def gs1(p):
            for e in range(2):
                st[p, e, 0] = _allsub(jnp.maximum, _tree(jnp.maximum, scores(p, e)))

        def gs2(p):
            ps = [[jnp.exp2(x - st[p, e, 2]) for x in scores(p, e)] for e in range(2)]
            for e in range(2):
                st[p, e, 1] = _allsub(jnp.add, _tree(jnp.add, ps[e]))
            for g in range(NG):
                lp[p, g] = _pack(ps[0][g], ps[1][g])

        def orx(p):
            def part(e, t):
                return _tree(jnp.add, [pmraw[p, e, t, g] for g in range(NG)])
            tiles = [part(0, 0), jnp.where(lane < 64, part(0, 1), part(1, 0)), part(1, 1)]
            store_lo(p, [_allsub(jnp.add, x) for x in tiles])

        def woacc(p):
            xacc[...] = xacc[...] + (woraw[p, 0:5] + woraw[p, 5:10] + woraw[p, 10:15])

        def vwo_jobs(p):
            def job(e, r, env):
                w = pltpu.bitcast(wo32[24 * p + 12 * e + r], bf16).astype(f32).reshape(5, 16, 128)
                a = e * AH + 2 * r
                t = w[:, 0:8] * oacc[p % RING, a] + w[:, 8:16] * oacc[p % RING, a + 1]
                env["acc"] = t if r == 0 else env["acc"] + t
                if r == AH // 2 - 1:
                    xacc[...] = xacc[...] + env["acc"] * _recip(st[p, e, 3])
            jobs = []
            for e in range(2):
                env = {}
                jobs += [functools.partial(job, e, r, env) for r in range(AH // 2)]
            return jobs

        mxu_fn = {"QP": qp_job, "QK": qk_job, "PM": pm_job, "WO": wo_job}
        xlu_fn = {"xq": xq, "xmax": xmax, "xl": xl, "xsum": xsum, "xcol": xcol}
        valu_fn = {"qprep": qprep, "qprepv": qprepv, "or2": or2, "gs1": gs1, "gs2": gs2, "orx": orx,
                   "woacc": woacc}
        plan_mxu, plan_small = _plan(3 * NC)

        def jobs_of(b):
            mx = [functools.partial(mxu_fn[kind], p, k)
                  for kind, p, k0, k1 in plan_mxu[b] for k in range(k0, k1)]
            xj = [functools.partial(xlu_fn[s], p) for s, p in plan_small[b] if s in xlu_fn]
            vj = [functools.partial(valu_fn[s], p) for s, p in plan_small[b] if s in valu_fn]
            sc = [j for s, p in plan_small[b] if s == "scale" for j in scale_jobs(p)]
            vw = [j for s, p in plan_small[b] if s == "vwo" for j in vwo_jobs(p)]
            return mx, xj, vj, sc, vw

        def block(b):
            p = VP[b]
            mx, xj, vj, sc, vw = jobs_of(b)
            sa, sb = sm_jobs(p, 0), sm_jobs(p, 1)
            pa, pb = pv_jobs(p, 0), pv_jobs(p, 1)
            cut = len(pb) - SKEW * NC2
            if b + 1 < len(VP):
                pb = pb[:cut]
            if b > 0:
                valu = _weave(pv_jobs(VP[b - 1], 1)[cut:], sa, 0.0, 0.9) + pa[:NC2]
            else:
                valu = sa[:3] + _weave(pa[:NC2], sa[3:], 0.0, 1.0 - 1.0 * SMG / NC)
            valu += _weave(pa[NC2:], sb, 0.1, 0.8) + vw
            valu += _weave(pb, vj + sc, 0.0, 0.9) if vj + sc else pb
            k = int(len(mx) * PIN)
            for s, q in plan_small[b]:
                refs = []
                if s in ("xsum", "xl", "xmax", "xcol"):
                    refs += [st.at[q, e, 2 if s == "xmax" else 3] for e in range(2)]
                if s in ("xsum", "xq"):
                    refs += [otile.at[q, t] for t in range(3)]
                for ref in refs:
                    mx[k] = functools.partial(mx[k], pin=lambda ref=ref: (ref[...],))
                    k += PINGAP
                if s == "xcol":
                    k = max(k, PINL)
                    for a in range(2 * AH - 3, 2 * AH):
                        ref = oacc.at[q % RING, a]
                        mx[k] = functools.partial(mx[k], pin=lambda ref=ref: (ref[...],))
                        k += 1
            _run(mx[:MXF] + xj + _weave(valu, mx[MXF:], 0.0, MX1))

        def set_x(x):
            xs[...] = x
            xl_ = _ln_lhs(x)
            for kk in range(5):
                xrow[kk] = x[:, 128 * kk:128 * kk + 128]
                lx[kk] = _pack(xl_[:, 128 * kk:128 * kk + 128])

        def prologue():
            def stats():
                m, r = _ln_stats(xs[...])
                stat[0] = _bc(m)
                stat[1] = _bc(r * qscale)
                xacc[...] = jnp.zeros_like(xacc)
            mx = [stats]
            for p in VP[:3]:
                mx += [functools.partial(qp_job, p, k) for k in range(15)]
                mx.append(functools.partial(qprep, p))
            mx += [functools.partial(qk_job, VP[0], k) for k in range(3 * NC)]
            bulk = [j for p in VQ for j in vqp_jobs(p)]
            _run(mx[:MXF + 1] + _weave(bulk, mx[MXF + 1:], 0.0, MXP) if bulk else mx)

        def finish_layer(first):
            for b in range(len(VP), len(plan_mxu)):
                mx, xj, vj, sc, vw = jobs_of(b)
                _run(xj + sc + vj + vw + mx)
            att = jnp.sum(jnp.concatenate([xacc[cc] for cc in range(5)], axis=1),
                          axis=0, keepdims=True)
            x1 = _rnd(xs[...] + _rnd(att))
            if first:
                xs[...] = x1
                for i in range(2):
                    gwait(gffn + i)
                    retile(wg32[i], 4)
                x1 = xs[...]
            m, r = _ln_stats(x1)
            xl_ = _ln_lhs(x1)
            lf = [_pack(xl_[:, 128 * kk:128 * kk + 128]) for kk in range(5)]
            nh = F // 128
            on_vpu = range(W2CUT[-2] // 128, nh) if first else range(NVH)

            def w2rows(j):
                i = next(i for i in range(nw2) if W2CUT[i] <= 128 * j < W2CUT[i + 1])
                return w2s[i][128 * j - W2CUT[i]:128 * j - W2CUT[i] + 128, :]

            def tile_dot(lhs, w):
                return jnp.dot(pltpu.bitcast(lhs, bf16), w, preferred_element_type=f32)[0:8]

            def gate_up(j):
                slot = (j & 1) * (nh // 2) + (j >> 1)
                parts = [[tile_dot(lf[kk], _tile(wg32[i][8 * kk:8 * kk + 8, slot])) for i in range(2)]
                         for kk in range(5)]
                g, u = [_ln_fix(_tree(jnp.add, [pp[i] for pp in parts]), m, r) for i in range(2)]
                return _rnd(g * jax.nn.sigmoid(g) * u)

            def hcols(h):
                hb = _bc(h[0:1])
                return [_bc(jnp.sum(jnp.where(lane == 8 * a + sub, hb, 0.0), axis=1, keepdims=True))
                        for a in range(16)]

            def vpu_rows(j, cols, yv):
                w = w2rows(j).astype(f32)
                for a in range(16):
                    t = w[8 * a:8 * a + 8] * jnp.tile(cols[a], (1, 5))
                    yv = t if yv is None else yv + t
                return yv

            hs, y, yv = [], None, None
            for j in range(nh):
                hs.append(gate_up(j))
                if j in on_vpu:
                    if first:
                        hcol[...] = jnp.stack(hcols(hs[j]))
                    else:
                        yv = vpu_rows(j, hcols(hs[j]), yv)
            for j in range(nh):
                if first and 128 * j in W2CUT:
                    i = W2CUT.index(128 * j)
                    if i:
                        xs[...] = y
                    gwait(gffn + 2 + i)
                    if i:
                        y = xs[...]
                if j not in on_vpu:
                    lh, w = _pack(hs[j]), w2rows(j)
                    t = jnp.concatenate([tile_dot(lh, w[:, 128 * cc:128 * cc + 128]) for cc in range(5)],
                                        axis=1)
                    y = t if y is None else y + t
                elif first:
                    yv = vpu_rows(j, [hcol[a] for a in range(16)], yv)
            y = y[0:1]
            if yv is not None:
                y = y + jnp.sum(yv, axis=0, keepdims=True)
            if first:
                set_x(_rnd(x1 + _rnd(y)))
            else:
                o_ref[...] = (x1[0:1] + _rnd(y)).astype(o_ref.dtype)

        def layer_body(layer, carry):
            first = layer == 0
            prologue()
            seen = 1
            for b in range(len(VP)):
                need = 1 + max([_group_of(VP[b], 1)] + [_group_of(p, 0) for kind, p, _, _ in plan_mxu[b]
                                                        if kind == "QK"])
                if need > seen:
                    @pl.when(first)
                    def _(lo_=seen, hi_=need):
                        for i in range(lo_, hi_):
                            kvready(i)
                    seen = need
                if ONLY is None or b in ONLY:
                    pl.when(layer < 100 + b)(functools.partial(block, b))
            lax.cond(first, lambda: finish_layer(True), lambda: finish_layer(False))
            return carry

        set_x(jnp.broadcast_to(xb[...].astype(f32), (8, D)))
        lax.fori_loop(0, 2, layer_body, 0)
    return kernel


def _tile_linear(c):
    sk = c.shape[2]
    return (jnp.swapaxes(c, 2, 3).reshape(NA, 8, sk // 128, 128)
            .transpose(0, 2, 1, 3).reshape(NA, sk // 16, 128))


@jax.jit
def pallas_interleave_layers__sliding_block_cached__glu_gated_swiglu__decode_kernel(
    A_x: jax.Array,
    A_k_cache: jax.Array,
    A_v_cache: jax.Array,
    A_wq: jax.Array,
    A_wo: jax.Array,
    B_x: jax.Array,
    B_w1: jax.Array,
    B_w3: jax.Array,
    B_w2: jax.Array,
):
    SK = A_k_cache.shape[2]
    W = min(4096, max(256, SK // 4))
    nc2 = W // 256
    kx = _tile_linear(A_k_cache).reshape(NA // 2, 2, SK // 256, 16, 128)
    vx = _tile_linear(A_v_cache)
    wqz, w1z, w3z = [(w.reshape(D // 16, 2, 8, w.shape[1] // 256, 2, 128).transpose(0, 1, 3, 4, 2, 5)
                      .reshape(D // 16, w.shape[1] // 128, 16, 128)) for w in (A_wq, B_w1, B_w3)]
    woz = (A_wo.reshape(HD // 16, 2, 8, 5, 128).transpose(0, 1, 3, 2, 4)
           .reshape(HD // 16, 80, 128))
    vreg = lambda *lead, dt=f32: pltpu.VMEM(lead + (8, 128), dt)
    scratch = [pltpu.VMEM(((kr[1] - kr[0]) * AH, 2, nc2, 16, 128), bf16) for kr, _ in KVG if kr]
    scratch += [pltpu.VMEM(((vr[1] - vr[0]) * 2 * AH, W // 16, 128), bf16) for _, vr in KVG]
    scratch += [pltpu.VMEM((b - a, D), bf16) for a, b in zip(W2CUT, W2CUT[1:])]
    scratch += [
        pltpu.VMEM((D // 16, 48, 16, 128), bf16),
        pltpu.VMEM((HD // 16, 80, 128), bf16),
        pltpu.VMEM((D // 16, F // 128, 16, 128), bf16),
        pltpu.VMEM((D // 16, F // 128, 16, 128), bf16),
        pltpu.VMEM((1, D), bf16),
        pltpu.VMEM((8, D), f32),
        vreg(5),
        vreg(5, dt=u32),
        vreg(2),
        vreg(max(3 * NVQ, 1)),
        vreg(max(NVQ, 1), 2 * AH),
        vreg(NP, 15),
        vreg(NP, 3, dt=u32),
        vreg(NP, 2, 2, nc2 // 4),
        vreg(2, 2 * nc2),
        vreg(NP, 2, 4),
        vreg(RING, 2 * AH),
        vreg(NP, 3),
        vreg(NX, nc2 // 4, dt=u32),
        vreg(NX, 2, 2, nc2 // 4),
        vreg(NP, 3, dt=u32),
        vreg(NP, 15),
        vreg(5),
        vreg(16),
        pltpu.SemaphoreType.DMA((len(KVG) + 2 + len(W2CUT),)),
    ]
    out = pl.pallas_call(
        _make_kernel(SK, W),
        out_shape=jax.ShapeDtypeStruct((1, D), A_x.dtype),
        in_specs=[pl.BlockSpec(memory_space=pl.ANY)] * 8,
        out_specs=pl.BlockSpec(memory_space=pltpu.VMEM),
        scratch_shapes=scratch,
        compiler_params=pltpu.CompilerParams(vmem_limit_bytes=126 * 1024 * 1024,
                                             disable_semaphore_checks=True),
    )(A_x.reshape(1, D), kx, vx, wqz, woz, w1z, w3z, B_w2)
    return out.reshape(1, 1, D)
```

```python
import functools
import math

import jax
import jax.numpy as jnp
from jax import lax
import jax.experimental.pallas as pl
import jax.experimental.pallas.tpu as pltpu

H, DH, D, F = 32, 192, 640, 1536
HD = H * DH
EPS = 1e-5
NA = HD // 8
AH = DH // 8
NP = H // 2
NX = 3
XP = list(range(NX))
VP = list(range(NX, NP))
NVQ = 6
VQ = (XP + VP[3:])[:NVQ]
VW = [3, 4, 5, 6, 15]
MQ = [p for p in range(NP) if p not in VQ]
MW = [p for p in range(NP) if p not in VW]
RING = 5
KVG = [((0, 5), (0, 4)), ((5, 8), (4, 8)), ((8, 12), (8, 12)), ((12, 16), (12, 14)), (None, (14, 16))]
W2CUT = (0, 1024, 1408, 1536)
AB = 4
SKEW = 1
VOFF = 55
VCOST = {"qprep": 10, "qprepv": 14, "scale": 14, "or2": 8, "woacc": 4, "gs1": 7, "gs2": 16,
         "orx": 18, "vwo": 186, "xsum": 4, "xq": 4}
CAPS = {0:124,1:144,2:148,3:140,4:164,5:164,6:164,7:164,8:144,9:144,10:144,11:140,12:152}
XQMAX = 3
MXF = 4
MX1 = 1.02
MXP = 0.97
PIN = 0.15
PINGAP = 5
PINL = 36
SMG = 4
ORG = 4
NVH = 7
ONLY = None
f32, bf16, u32 = jnp.float32, jnp.bfloat16, jnp.uint32


def _ln_stats(x):
    m = jnp.mean(x, axis=-1, keepdims=True)
    xc = x - m
    v = jnp.mean(xc * xc, axis=-1, keepdims=True)
    return m, lax.rsqrt(v + EPS)


def _ln_lhs(x):
    return jnp.where(lax.broadcasted_iota(jnp.int32, x.shape, 0) < 4, x, 1.0)


def _ln_fix(raw, m, r):
    return (raw - m * pltpu.roll(raw, 4, 0)) * r


def _rnd(x):
    return x.astype(bf16).astype(f32)


def _pack(lo, hi=None):
    return pltpu.bitcast(jnp.concatenate([lo, lo if hi is None else hi], axis=0).astype(bf16), u32)


def _tile(w_u32):
    return pltpu.bitcast(w_u32.reshape(64, 128), bf16)


def _mm(lhs_u32, w_u32, pin=()):
    if pin:
        lhs_u32 = jnp.concatenate([lhs_u32] + [pltpu.bitcast(x, u32) for x in pin], axis=0)
    return jnp.dot(pltpu.bitcast(lhs_u32, bf16), _tile(w_u32), preferred_element_type=f32)[0:16]


def _bc(x):
    return jnp.broadcast_to(x, (8, 128))


def _tree(op, xs):
    xs = list(xs)
    while len(xs) > 1:
        xs = [op(xs[i], xs[i + 1]) if i + 1 < len(xs) else xs[i] for i in range(0, len(xs), 2)]
    return xs[0]


def _allsub(op, x):
    for sh in (4, 2, 1):
        x = op(x, pltpu.roll(x, sh, 0))
    return x


def _recip(l):
    r = pl.reciprocal(l, approx=True)
    return r * (2.0 - l * r)


def _run(jobs):
    for j in jobs:
        j()


def _weave(main, extra, lo, hi):
    out, k = [], 0
    for n, j in enumerate(main):
        while k < len(extra) and lo * len(main) + k * (hi - lo) * len(main) / len(extra) <= n:
            out.append(extra[k])
            k += 1
        out.append(j)
    return out + list(extra[k:])


def _plan(nt):
    nb = len(VP)
    total = {"QP": 15, "QK": nt, "PM": nt, "WO": 15}
    done, fin, mxu, small = {}, {}, {}, {}

    def issue(b, kind, p, cap):
        k0 = done.get((kind, p), 0)
        n = max(min(total[kind] - k0, cap), 0)
        if n:
            mxu[b].append((kind, p, k0, k0 + n))
            done[(kind, p)] = k0 + n
            if k0 + n == total[kind]:
                fin[(kind, p)] = b
        return n

    def before(key, b):
        return fin.get(key, b) < b

    chains, qlast = {}, {}
    for p in range(NP):
        ch = ["vqp", "xq", "qprepv"] if p in VQ else ["QP", "qprep"]
        qlast[p] = ch[-1]
        if p in XP:
            ch += ["QK", "gs1", "xmax", "gs2", "PM", "orx", "WO", "woacc"]
        else:
            ch += ["QK", "pv", "xmax", "scale"]
            ch += ["xcol", "vwo"] if p in VW else ["xsum", "or2", "WO", "woacc"]
        chains[p] = ch
    for p in VQ:
        fin[("vqp", p)] = -1
    for p in VP[:3]:
        done[("QP", p)] = 15
        fin[("QP", p)] = fin[("qprep", p)] = -1
    done[("QK", VP[0])] = nt
    fin[("QK", VP[0])] = -1
    xq_order = sorted(VQ, key=lambda p: 2 * XP.index(p) + 1 if p in XP else 2 * (VP.index(p) - 3))
    late = []
    b = 0
    while any((chains[p][-1], p) not in fin for p in range(NP)):
        mxu[b], small[b], late = [], late, []
        for p in range(NP):
            for prev, st in zip(chains[p], chains[p][1:]):
                if st in total or (st, p) in fin or not before((prev, p), b):
                    continue
                if st == "xq" and xq_order.index(p) // XQMAX > b:
                    continue
                if st == "pv":
                    if b < nb and VP[b] == p:
                        fin[(st, p)] = b
                    continue
                small[b].append((st, p))
                fin[(st, p)] = b
                if st == "gs2":
                    late.append(("xl", p))
        cap = 10 ** 6
        if b < nb:
            nab = 12 - (SKEW if b == 0 else 0) + (SKEW if b == nb - 1 else 0)
            vload = 95 * nab + 31 + VOFF + sum(VCOST.get(s, 0) for s, _ in small[b])
            cap = CAPS.get(b, 4 * int(round((vload - 147) / 32.0)))
            assert fin.get(("pv", VP[b])) == b
        if b + 1 < nb:
            assert before((qlast[VP[b + 1]], VP[b + 1]), b)
            cap -= issue(b, "QK", VP[b + 1], nt)
        if b + 3 < nb and VP[b + 3] not in VQ:
            cap -= issue(b, "QP", VP[b + 3], 15)
        cands = [("QP", p, None) for p in XP if p not in VQ] + [("QK", p, qlast[p]) for p in XP]
        cands += [("PM", p, "gs2") for p in XP] + [("QP", p, None) for p in VP if p not in VQ]
        cands += [("WO", p, "orx" if p in XP else "or2") for p in VP + XP if p not in VW]
        cands += [("QK", p, qlast[p]) for p in VP]
        for kind, p, need in cands:
            if need is None or before((need, p), b):
                cap -= issue(b, kind, p, cap)
        b += 1
    return mxu, small


def _group_of(p, which):
    return next(i for i, g in enumerate(KVG) if g[which] and g[which][0] <= p < g[which][1])


def _make_kernel(SK, W):
    NC = W // 128
    NC2, NG = NC // 2, NC // 8
    qscale = DH ** -0.5 * math.log2(math.e)
    nk = sum(1 for kr, _ in KVG if kr)
    nv, nw2 = len(KVG), len(W2CUT) - 1

    def kernel(x_hbm, k_hbm, v_hbm, wq_hbm, wo_hbm, w1_hbm, w3_hbm, w2_hbm, o_ref, *scratch):
        kbs, vbs = scratch[:nk], scratch[nk:nk + nv]
        w2s = scratch[nk + nv:nk + nv + nw2]
        (wqb, wob, w1, w3, xb, xs, xrow, lx, stat, csum, qacc, qraw, lq, sraw, pbuf, st, oacc,
         otile, lp, pmraw, lo, woraw, xacc, hcol, sem) = scratch[nk + nv + nw2:]
        k32s = [r.bitcast(u32) for r in kbs]
        v32 = vbs[0].bitcast(u32)
        wq32 = wqb.bitcast(u32)
        wo32 = wob.bitcast(u32)
        wg32 = [w1.bitcast(u32), w3.bitcast(u32)]

        groups = [[(x_hbm, xb), (wq_hbm, wqb), (wo_hbm, wob)]]
        for i, (kr, vr) in enumerate(KVG):
            grp = []
            if kr:
                grp.append((k_hbm.at[kr[0] * AH:kr[1] * AH, :, pl.ds((SK - W) // 256, NC2)], kbs[i]))
            grp.append((v_hbm.at[vr[0] * 2 * AH:vr[1] * 2 * AH, pl.ds((SK - W) // 16, W // 16), :], vbs[i]))
            groups.append(grp)
        gffn = len(groups)
        groups += [[(w1_hbm, w1)], [(w3_hbm, w3)]]
        for i in range(nw2):
            groups.append([(w2_hbm.at[W2CUT[i]:W2CUT[i + 1]], w2s[i])])
        groups = [[pltpu.make_async_copy(s, d, sem.at[g]) for s, d in grp]
                  for g, grp in enumerate(groups)]
        for grp in groups:
            for cp in grp:
                cp.start()

        def gwait(g):
            for cp in groups[g]:
                cp.wait()

        sub = lax.broadcasted_iota(jnp.int32, (8, 128), 0)
        lane = lax.broadcasted_iota(jnp.int32, (8, 128), 1)

        def kvready(i):
            gwait(1 + i)
            if KVG[i][0]:
                k32 = k32s[i]

                def swap(r, carry):
                    a = k32[r, 0, :, 4:8, :]
                    b = k32[r, 1, :, 0:4, :]
                    k32[r, 0, :, 4:8, :] = b
                    k32[r, 1, :, 0:4, :] = a
                    return carry
                lax.fori_loop(0, k32.shape[0], swap, 0)

        def retile(w32, rows):
            n = w32.shape[1] // 2

            def body(rb, carry):
                r = pl.ds(rb * rows, rows)
                a = w32[r, 0:n, 4:8, :]
                b = w32[r, n:2 * n, 0:4, :]
                w32[r, 0:n, 4:8, :] = b
                w32[r, n:2 * n, 0:4, :] = a
                return carry
            lax.fori_loop(0, w32.shape[0] // rows, body, 0)

        def retile_wo(rb, carry):
            r = pl.ds(rb * 4, 4)
            vals = {(e, cc): wo32[r, 4 * (5 * e + cc):4 * (5 * e + cc) + 4, :]
                    for e in range(2) for cc in range(5)}
            for (e, cc), v in vals.items():
                wo32[r, 8 * cc + 4 * e:8 * cc + 4 * e + 4, :] = v
            return carry

        def transpose_wq(i, carry):
            c = i + jnp.where(i >= 3 * NX, 9, 0)
            slot = (c & 1) * 24 + (c >> 1)
            ones = jnp.ones((16, 128), bf16)
            tiles = [_tile(wq32[8 * kk:8 * kk + 8, slot]) for kk in range(5)]
            csum[i] = _tree(jnp.add, [jnp.dot(ones, t, preferred_element_type=f32)[0:8] for t in tiles])
            for kk in range(5):
                wq32[8 * kk:8 * kk + 8, slot] = pltpu.bitcast(tiles[kk].T, u32).reshape(8, 8, 128)
            return carry

        def transpose_v(i, carry):
            a0 = pl.multiple_of((i >> 2) * 16, 16)
            for u in range(4):
                c2 = (i & 3) * 4 + u
                x = vbs[0][pl.ds(a0, 16), pl.ds(pl.multiple_of(c2 * 16, 16), 16), :]
                ts = [x[:, 8 * h:8 * h + 8, :].reshape(128, 128).T for h in range(2)]
                for h in range(2):
                    v32[pl.ds(a0 + 8 * h, 8), pl.ds(pl.multiple_of(c2 * 8, 8), 8), :] = (
                        pltpu.bitcast(ts[h], u32).reshape(8, 8, 128))
            return carry

        gwait(0)
        retile(wq32, 1)
        lax.fori_loop(0, HD // 64, retile_wo, 0)
        if NVQ:
            lax.fori_loop(0, 3 * NVQ, transpose_wq, 0)
        kvready(0)
        lax.fori_loop(0, NX * 3 * NC2 // 4, transpose_v, 0)

        def wq_slot(p, t):
            c = 3 * p + t
            return (c & 1) * 24 + (c >> 1)

        def qp_job(p, k, pin=tuple):
            kk, t = divmod(k, 3)
            qraw[MQ.index(p), 5 * t + kk] = _mm(
                lx[kk], wq32[8 * kk:8 * kk + 8, wq_slot(p, t)], pin())[0:8]

        def keep_rows(dst, t, c, r):
            g, j = divmod(c, 8)
            if t < 2:
                dst[0, t, g, j:j + 1, :] = r[j:j + 1]
            if t > 0:
                dst[1, t - 1, g, j:j + 1, :] = r[8 + j:9 + j]

        def qk_job(p, k, pin=tuple):
            t, c = divmod(k, NC)
            g = _group_of(p, 0)
            r0 = (p - KVG[g][0][0]) * AH + 8 * t
            keep_rows(sraw.at[p], t, c, _mm(lq[p, t], k32s[g][r0:r0 + 8, c & 1, c >> 1], pin()))

        def pm_job(p, k, pin=tuple):
            t, c = divmod(k, NC)
            a0 = p * 2 * AH + 16 * t + 8 * (c & 1)
            w = v32[a0:a0 + 8, 8 * (c >> 1):8 * (c >> 1) + 8, :]
            keep_rows(pmraw.at[p], t, c, _mm(lp[p, c // 8], w, pin()))

        def wo_job(p, k, pin=tuple):
            t, cc = divmod(k, 5)
            r0 = 24 * p + 8 * t
            woraw[MW.index(p), k] = _mm(lo[p, t], wo32[r0:r0 + 8, 8 * cc:8 * cc + 8, :], pin())[0:8]

        def lane_sums(p, src):
            for a in range(2 * AH):
                r = _bc(jnp.sum(src(a), axis=1, keepdims=True))
                t, k = divmod(a, 16)
                otile[p, t, :, 8 * k:8 * k + 8] = r[:, 8 * k:8 * k + 8]

        def xq(p):
            lane_sums(p, lambda a: qacc[VQ.index(p), a])

        def xmax(p):
            for e in range(2):
                st[p, e, 2] = _bc(jnp.max(st[p, e, 0], axis=1, keepdims=True))

        def xl(p):
            for e in range(2):
                st[p, e, 3] = _bc(jnp.sum(st[p, e, 1], axis=1, keepdims=True))

        def xsum(p):
            xl(p)
            lane_sums(p, lambda a: oacc[p % RING, a])

        def xcol(p):
            xl(p)
            for a in range(2 * AH):
                oacc[p % RING, a] = _bc(jnp.sum(oacc[p % RING, a], axis=1, keepdims=True))

        def store_lq(p, t, q):
            qp = _pack(q)
            if t == 1:
                qp = jnp.where((lane >> 6) == (sub >> 2), qp, jnp.uint32(0))
            lq[p, t] = qp

        def qprep(p):
            for t in range(3):
                qv = _tree(jnp.add, [qraw[MQ.index(p), 5 * t + kk] for kk in range(5)])
                store_lq(p, t, _bc(_ln_fix(qv, stat[0], stat[1])[0:1]))

        def vqp_jobs(p):
            def job(t, i):
                w = jnp.stack([wq32[8 * kk + i, wq_slot(p, t)] for kk in range(5)])
                w = pltpu.bitcast(w.reshape(40, 128), bf16).astype(f32).reshape(5, 2, 8, 128)
                acc = _tree(jnp.add, [w[kk] * xrow[kk] for kk in range(5)])
                qacc[VQ.index(p), 16 * t + 2 * i:16 * t + 2 * i + 2] = acc
            return [functools.partial(job, t, i) for t in range(3) for i in range(8)]

        def qprepv(p):
            for t in range(3):
                raw = _allsub(jnp.add, jnp.where((lane & 7) == sub, otile[p, t], 0.0))
                store_lq(p, t, (raw - stat[0] * csum[3 * VQ.index(p) + t]) * stat[1])

        def scores(p, e):
            return [sraw[p, e, 0, g] + sraw[p, e, 1, g] for g in range(NG)]

        def sm_jobs(p, e):
            env = {}

            def head():
                s = scores(p, e)
                mv = _allsub(jnp.maximum, _tree(jnp.maximum, s))
                st[p, e, 0] = mv
                env["p"] = [jnp.exp2(x - mv) for x in s]

            def spread(c0):
                for c in range(c0, c0 + SMG):
                    pbuf[e, c] = _bc(env["p"][c // 8][c % 8:c % 8 + 1])

            def lsum():
                st[p, e, 1] = _allsub(jnp.add, _tree(jnp.add, env["p"]))
            return [head] + [functools.partial(spread, c0) for c0 in range(0, NC, SMG)] + [lsum]

        def pv_jobs(p, e):
            g = _group_of(p, 1)

            def job(a0, c2, env):
                a = (p - KVG[g][1][0]) * 2 * AH + e * AH + a0
                v = vbs[g][a:a + AB, 16 * c2:16 * c2 + 16, :].astype(f32)
                t = v[:, 0:8] * pbuf[e, 2 * c2] + v[:, 8:16] * pbuf[e, 2 * c2 + 1]
                env["acc"] = t if c2 == 0 else env["acc"] + t
                if c2 == NC2 - 1:
                    oacc[p % RING, e * AH + a0:e * AH + a0 + AB] = env["acc"]
            jobs = []
            for a0 in range(0, AH, AB):
                env = {}
                jobs += [functools.partial(job, a0, c2, env) for c2 in range(NC2)]
            return jobs

        def scale_jobs(p):
            def head(e, env):
                env["w"] = jnp.exp2(st[p, e, 0] - st[p, e, 2])
                st[p, e, 1] = env["w"] * st[p, e, 1]

            def job(a, env):
                oacc[p % RING, a:a + ORG] = oacc[p % RING, a:a + ORG] * env["w"]
            jobs = []
            for e in range(2):
                env = {}
                jobs.append(functools.partial(head, e, env))
                jobs += [functools.partial(job, e * AH + a, env) for a in range(0, AH, ORG)]
            return jobs

        def store_lo(p, tiles):
            inv = [_recip(st[p, e, 3]) for e in range(2)]
            invs = [inv[0], jnp.where(lane < 64, inv[0], inv[1]), inv[1]]
            for t in range(3):
                lo[p, t] = _pack(jnp.where((lane & 7) == sub, tiles[t] * invs[t], 0.0))

        def or2(p):
            store_lo(p, [otile[p, t] for t in range(3)])

        def gs1(p):
            for e in range(2):
                st[p, e, 0] = _allsub(jnp.maximum, _tree(jnp.maximum, scores(p, e)))

        def gs2(p):
            ps = [[jnp.exp2(x - st[p, e, 2]) for x in scores(p, e)] for e in range(2)]
            for e in range(2):
                st[p, e, 1] = _allsub(jnp.add, _tree(jnp.add, ps[e]))
            for g in range(NG):
                lp[p, g] = _pack(ps[0][g], ps[1][g])

        def orx(p):
            def part(e, t):
                return _tree(jnp.add, [pmraw[p, e, t, g] for g in range(NG)])
            tiles = [part(0, 0), jnp.where(lane < 64, part(0, 1), part(1, 0)), part(1, 1)]
            store_lo(p, [_allsub(jnp.add, x) for x in tiles])

        def woacc(p):
            raw = woraw.at[MW.index(p)]
            xacc[...] = xacc[...] + (raw[0:5] + raw[5:10] + raw[10:15])

        def vwo_jobs(p):
            def job(e, r, env):
                w = pltpu.bitcast(wo32[24 * p + 12 * e + r], bf16).astype(f32).reshape(5, 16, 128)
                a = e * AH + 2 * r
                t = w[:, 0:8] * oacc[p % RING, a] + w[:, 8:16] * oacc[p % RING, a + 1]
                env["acc"] = t if r == 0 else env["acc"] + t
                if r == AH // 2 - 1:
                    xacc[...] = xacc[...] + env["acc"] * _recip(st[p, e, 3])
            jobs = []
            for e in range(2):
                env = {}
                jobs += [functools.partial(job, e, r, env) for r in range(AH // 2)]
            return jobs

        mxu_fn = {"QP": qp_job, "QK": qk_job, "PM": pm_job, "WO": wo_job}
        xlu_fn = {"xq": xq, "xmax": xmax, "xl": xl, "xsum": xsum, "xcol": xcol}
        valu_fn = {"qprep": qprep, "qprepv": qprepv, "or2": or2, "gs1": gs1, "gs2": gs2, "orx": orx,
                   "woacc": woacc}
        plan_mxu, plan_small = _plan(3 * NC)

        def jobs_of(b):
            mx = [functools.partial(mxu_fn[kind], p, k)
                  for kind, p, k0, k1 in plan_mxu[b] for k in range(k0, k1)]
            xj = [functools.partial(xlu_fn[s], p) for s, p in plan_small[b] if s in xlu_fn]
            vj = [functools.partial(valu_fn[s], p) for s, p in plan_small[b] if s in valu_fn]
            sc = [j for s, p in plan_small[b] if s == "scale" for j in scale_jobs(p)]
            vw = [j for s, p in plan_small[b] if s == "vwo" for j in vwo_jobs(p)]
            return mx, xj, vj, sc, vw

        def block(b):
            p = VP[b]
            mx, xj, vj, sc, vw = jobs_of(b)
            sa, sb = sm_jobs(p, 0), sm_jobs(p, 1)
            pa, pb = pv_jobs(p, 0), pv_jobs(p, 1)
            cut = len(pb) - SKEW * NC2
            if b + 1 < len(VP):
                pb = pb[:cut]
            if b > 0:
                valu = _weave(pv_jobs(VP[b - 1], 1)[cut:], sa, 0.0, 0.9) + pa[:NC2]
            else:
                valu = sa[:3] + _weave(pa[:NC2], sa[3:], 0.0, 1.0 - 1.0 * SMG / NC)
            valu += _weave(pa[NC2:], sb, 0.1, 0.8) + vw
            valu += _weave(pb, vj + sc, 0.0, 0.9) if vj + sc else pb
            k = int(len(mx) * PIN)
            for s, q in plan_small[b]:
                refs = []
                if s in ("xsum", "xl", "xmax", "xcol"):
                    refs += [st.at[q, e, 2 if s == "xmax" else 3] for e in range(2)]
                if s in ("xsum", "xq"):
                    refs += [otile.at[q, t] for t in range(3)]
                for ref in refs:
                    mx[k] = functools.partial(mx[k], pin=lambda ref=ref: (ref[...],))
                    k += PINGAP
                if s == "xcol":
                    k = max(k, PINL)
                    for a in range(2 * AH - 3, 2 * AH):
                        ref = oacc.at[q % RING, a]
                        mx[k] = functools.partial(mx[k], pin=lambda ref=ref: (ref[...],))
                        k += 1
            _run(mx[:MXF] + xj + _weave(valu, mx[MXF:], 0.0, MX1))

        def set_x(x):
            xs[...] = x
            xl_ = _ln_lhs(x)
            for kk in range(5):
                xrow[kk] = x[:, 128 * kk:128 * kk + 128]
                lx[kk] = _pack(xl_[:, 128 * kk:128 * kk + 128])

        def prologue():
            def stats():
                m, r = _ln_stats(xs[...])
                stat[0] = _bc(m)
                stat[1] = _bc(r * qscale)
                xacc[...] = jnp.zeros_like(xacc)
            mx = [stats]
            for p in VP[:3]:
                mx += [functools.partial(qp_job, p, k) for k in range(15)]
                mx.append(functools.partial(qprep, p))
            mx += [functools.partial(qk_job, VP[0], k) for k in range(3 * NC)]
            bulk = [j for p in VQ for j in vqp_jobs(p)]
            _run(mx[:MXF + 1] + _weave(bulk, mx[MXF + 1:], 0.0, MXP) if bulk else mx)

        def finish_layer(first):
            for b in range(len(VP), len(plan_mxu)):
                mx, xj, vj, sc, vw = jobs_of(b)
                _run(xj + sc + vj + vw + mx)
            att = jnp.sum(jnp.concatenate([xacc[cc] for cc in range(5)], axis=1),
                          axis=0, keepdims=True)
            x1 = _rnd(xs[...] + _rnd(att))
            if first:
                xs[...] = x1
                for i in range(2):
                    gwait(gffn + i)
                    retile(wg32[i], 4)
                x1 = xs[...]
            m, r = _ln_stats(x1)
            xl_ = _ln_lhs(x1)
            lf = [_pack(xl_[:, 128 * kk:128 * kk + 128]) for kk in range(5)]
            nh = F // 128
            on_vpu = range(W2CUT[-2] // 128, nh) if first else range(NVH)

            def w2rows(j):
                i = next(i for i in range(nw2) if W2CUT[i] <= 128 * j < W2CUT[i + 1])
                return w2s[i][128 * j - W2CUT[i]:128 * j - W2CUT[i] + 128, :]

            def tile_dot(lhs, w):
                return jnp.dot(pltpu.bitcast(lhs, bf16), w, preferred_element_type=f32)[0:8]

            def gate_up(j):
                slot = (j & 1) * (nh // 2) + (j >> 1)
                parts = [[tile_dot(lf[kk], _tile(wg32[i][8 * kk:8 * kk + 8, slot])) for i in range(2)]
                         for kk in range(5)]
                g, u = [_ln_fix(_tree(jnp.add, [pp[i] for pp in parts]), m, r) for i in range(2)]
                return _rnd(g * jax.nn.sigmoid(g) * u)

            def hcols(h):
                hb = _bc(h[0:1])
                return [_bc(jnp.sum(jnp.where(lane == 8 * a + sub, hb, 0.0), axis=1, keepdims=True))
                        for a in range(16)]

            def vpu_rows(j, cols, yv):
                w = w2rows(j).astype(f32)
                for a in range(16):
                    t = w[8 * a:8 * a + 8] * jnp.tile(cols[a], (1, 5))
                    yv = t if yv is None else yv + t
                return yv

            hs, y, yv = [], None, None
            for j in range(nh):
                hs.append(gate_up(j))
                if j in on_vpu:
                    if first:
                        hcol[...] = jnp.stack(hcols(hs[j]))
                    else:
                        yv = vpu_rows(j, hcols(hs[j]), yv)
            for j in range(nh):
                if first and 128 * j in W2CUT:
                    i = W2CUT.index(128 * j)
                    if i:
                        xs[...] = y
                    gwait(gffn + 2 + i)
                    if i:
                        y = xs[...]
                if j not in on_vpu:
                    lh, w = _pack(hs[j]), w2rows(j)
                    t = jnp.concatenate([tile_dot(lh, w[:, 128 * cc:128 * cc + 128]) for cc in range(5)],
                                        axis=1)
                    y = t if y is None else y + t
                elif first:
                    yv = vpu_rows(j, [hcol[a] for a in range(16)], yv)
            y = y[0:1]
            if yv is not None:
                y = y + jnp.sum(yv, axis=0, keepdims=True)
            if first:
                set_x(_rnd(x1 + _rnd(y)))
            else:
                o_ref[...] = (x1[0:1] + _rnd(y)).astype(o_ref.dtype)

        def layer_body(layer, carry):
            first = layer == 0
            prologue()
            seen = 1
            for b in range(len(VP)):
                need = 1 + max([_group_of(VP[b], 1)] + [_group_of(p, 0) for kind, p, _, _ in plan_mxu[b]
                                                        if kind == "QK"])
                if need > seen:
                    @pl.when(first)
                    def _(lo_=seen, hi_=need):
                        for i in range(lo_, hi_):
                            kvready(i)
                    seen = need
                if ONLY is None or b in ONLY:
                    pl.when(layer < 100 + b)(functools.partial(block, b))
            lax.cond(first, lambda: finish_layer(True), lambda: finish_layer(False))
            return carry

        set_x(jnp.broadcast_to(xb[...].astype(f32), (8, D)))
        lax.fori_loop(0, 2, layer_body, 0)
    return kernel


def _tile_linear(c):
    sk = c.shape[2]
    return (jnp.swapaxes(c, 2, 3).reshape(NA, 8, sk // 128, 128)
            .transpose(0, 2, 1, 3).reshape(NA, sk // 16, 128))


@jax.jit
def pallas_interleave_layers__sliding_block_cached__glu_gated_swiglu__decode_kernel(
    A_x: jax.Array,
    A_k_cache: jax.Array,
    A_v_cache: jax.Array,
    A_wq: jax.Array,
    A_wo: jax.Array,
    B_x: jax.Array,
    B_w1: jax.Array,
    B_w3: jax.Array,
    B_w2: jax.Array,
):
    SK = A_k_cache.shape[2]
    W = min(4096, max(256, SK // 4))
    nc2 = W // 256
    kx = _tile_linear(A_k_cache).reshape(NA // 2, 2, SK // 256, 16, 128)
    vx = _tile_linear(A_v_cache)
    wqz, w1z, w3z = [(w.reshape(D // 16, 2, 8, w.shape[1] // 256, 2, 128).transpose(0, 1, 3, 4, 2, 5)
                      .reshape(D // 16, w.shape[1] // 128, 16, 128)) for w in (A_wq, B_w1, B_w3)]
    woz = (A_wo.reshape(HD // 16, 2, 8, 5, 128).transpose(0, 1, 3, 2, 4)
           .reshape(HD // 16, 80, 128))
    vreg = lambda *lead, dt=f32: pltpu.VMEM(lead + (8, 128), dt)
    scratch = [pltpu.VMEM(((kr[1] - kr[0]) * AH, 2, nc2, 16, 128), bf16) for kr, _ in KVG if kr]
    scratch += [pltpu.VMEM(((vr[1] - vr[0]) * 2 * AH, W // 16, 128), bf16) for _, vr in KVG]
    scratch += [pltpu.VMEM((b - a, D), bf16) for a, b in zip(W2CUT, W2CUT[1:])]
    scratch += [
        pltpu.VMEM((D // 16, 48, 16, 128), bf16),
        pltpu.VMEM((HD // 16, 80, 128), bf16),
        pltpu.VMEM((D // 16, F // 128, 16, 128), bf16),
        pltpu.VMEM((D // 16, F // 128, 16, 128), bf16),
        pltpu.VMEM((1, D), bf16),
        pltpu.VMEM((8, D), f32),
        vreg(5),
        vreg(5, dt=u32),
        vreg(2),
        vreg(max(3 * NVQ, 1)),
        vreg(max(NVQ, 1), 2 * AH),
        vreg(len(MQ), 15),
        vreg(NP, 3, dt=u32),
        vreg(NP, 2, 2, nc2 // 4),
        vreg(2, 2 * nc2),
        vreg(NP, 2, 4),
        vreg(RING, 2 * AH),
        vreg(NP, 3),
        vreg(NX, nc2 // 4, dt=u32),
        vreg(NX, 2, 2, nc2 // 4),
        vreg(NP, 3, dt=u32),
        vreg(len(MW), 15),
        vreg(5),
        vreg(16),
        pltpu.SemaphoreType.DMA((len(KVG) + 2 + len(W2CUT),)),
    ]
    out = pl.pallas_call(
        _make_kernel(SK, W),
        out_shape=jax.ShapeDtypeStruct((1, D), A_x.dtype),
        in_specs=[pl.BlockSpec(memory_space=pl.ANY)] * 8,
        out_specs=pl.BlockSpec(memory_space=pltpu.VMEM),
        scratch_shapes=scratch,
        compiler_params=pltpu.CompilerParams(vmem_limit_bytes=126 * 1024 * 1024,
                                             disable_semaphore_checks=True),
    )(A_x.reshape(1, D), kx, vx, wqz, woz, w1z, w3z, B_w2)
    return out.reshape(1, 1, D)
```

```python
import functools
import math

import jax
import jax.numpy as jnp
from jax import lax
import jax.experimental.pallas as pl
import jax.experimental.pallas.tpu as pltpu

H, DH, D, F = 32, 192, 640, 1536
HD = H * DH
EPS = 1e-5
NA = HD // 8
AH = DH // 8
NP = H // 2
NX = 4
XP = list(range(NX))
VP = list(range(NX, NP))
NVQ = 10
NPX = 1
PQ = VP[:3] + XP[:NPX]
VQ = (XP[NPX:] + VP[3:])[:NVQ]
VQO = sorted(VQ, key=lambda p: 2 * (XP.index(p) - NPX) + 1 if p in XP else 2 * (VP.index(p) - 3))
NVP = 7
VQB = 1
VW = [4,5,6,7,10,11,15]
MQ = [p for p in range(NP) if p not in VQ]
MW = [p for p in range(NP) if p not in VW]
GFROM = 13
GM = VP[GFROM:]
RA = []
NQA = 8
RING = 5
KVG = [((0, 6), (0, 5)), ((6, 8), (5, 8)), ((8, 12), (8, 12)), ((12, 16), (12, 14)), (None, (14, 16))]
W2CUT = (0, 1024, 1408, 1536)
AB = 4
SKEW = 1
VOFF = 70
VCOST = {"qprep": 10, "qprepv": 14, "scale": 14, "or2": 8, "woacc": 4, "gmax": 4, "gs2": 19,
         "orx": 18, "vwo": 186, "vqp": 170, "xsum": 4, "xq": 4}
CAPS = {}
XQMAX = 2
MXF = 4
MX1 = 1.02
MXP = 1.0
PIN = 0.15
PINGAP = 5
PINL = 36
SMG = 4
ORG = 4
NVH = 7
ONLY = None
f32, bf16, u32 = jnp.float32, jnp.bfloat16, jnp.uint32


def _ln_stats(x):
    m = jnp.mean(x, axis=-1, keepdims=True)
    xc = x - m
    v = jnp.mean(xc * xc, axis=-1, keepdims=True)
    return m, lax.rsqrt(v + EPS)


def _ln_lhs(x):
    return jnp.where(lax.broadcasted_iota(jnp.int32, x.shape, 0) < 4, x, 1.0)


def _ln_fix(raw, m, r):
    return (raw - m * pltpu.roll(raw, 4, 0)) * r


def _rnd(x):
    return x.astype(bf16).astype(f32)


def _pack(lo, hi=None):
    return pltpu.bitcast(jnp.concatenate([lo, lo if hi is None else hi], axis=0).astype(bf16), u32)


def _tile(w_u32):
    return pltpu.bitcast(w_u32.reshape(64, 128), bf16)


def _mm(lhs_u32, w_u32, pin=()):
    if pin:
        lhs_u32 = jnp.concatenate([lhs_u32] + [pltpu.bitcast(x, u32) for x in pin], axis=0)
    return jnp.dot(pltpu.bitcast(lhs_u32, bf16), _tile(w_u32), preferred_element_type=f32)[0:16]


def _bc(x):
    return jnp.broadcast_to(x, (8, 128))


def _tree(op, xs):
    xs = list(xs)
    while len(xs) > 1:
        xs = [op(xs[i], xs[i + 1]) if i + 1 < len(xs) else xs[i] for i in range(0, len(xs), 2)]
    return xs[0]


def _allsub(op, x):
    for sh in (4, 2, 1):
        x = op(x, pltpu.roll(x, sh, 0))
    return x


def _recip(l):
    r = pl.reciprocal(l, approx=True)
    return r * (2.0 - l * r)


def _run(jobs):
    for j in jobs:
        j()


def _weave(main, extra, lo, hi):
    out, k = [], 0
    for n, j in enumerate(main):
        while k < len(extra) and lo * len(main) + k * (hi - lo) * len(main) / len(extra) <= n:
            out.append(extra[k])
            k += 1
        out.append(j)
    return out + list(extra[k:])


def _plan(nt):
    nb = len(VP)
    total = {"QP": 15, "QK": nt, "PM": nt, "WO": 15}
    done, fin, mxu, small = {}, {}, {}, {}

    def issue(b, kind, p, cap):
        k0 = done.get((kind, p), 0)
        n = max(min(total[kind] - k0, cap), 0)
        if n:
            mxu[b].append((kind, p, k0, k0 + n))
            done[(kind, p)] = k0 + n
            if k0 + n == total[kind]:
                fin[(kind, p)] = b
        return n

    def before(key, b):
        return fin.get(key, b) < b

    chains, qlast = {}, {}
    for p in range(NP):
        ch = ["vqp", "xq", "qprepv"] if p in VQ else ["QP", "qprep"]
        qlast[p] = ch[-1]
        if p in XP:
            ch += ["QK", "gmax", "gs2", "PM", "orx", "WO", "woacc"]
        else:
            if p in GM:
                ch += ["QK", "gmax", "pv"] + (["skew"] if p != VP[-1] else [])
            else:
                ch += ["QK", "pv", "xmax", "scale"]
            ch += ["xcol", "vwo"] if p in VW else ["xsum", "or2", "WO", "woacc"]
        chains[p] = ch
    for p in VQO[:NVP]:
        fin[("vqp", p)] = -1
    for p in PQ:
        done[("QP", p)] = 15
        fin[("QP", p)] = fin[("qprep", p)] = -1
    done[("QK", VP[0])] = nt
    fin[("QK", VP[0])] = -1
    late = []
    b = 0
    while any((chains[p][-1], p) not in fin for p in range(NP)):
        mxu[b], small[b], late = [], late, []
        for p in VQO[NVP + VQB * b:NVP + VQB * (b + 1)]:
            small[b].append(("vqp", p))
            fin[("vqp", p)] = b
        for p in range(NP):
            for prev, st in zip(chains[p], chains[p][1:]):
                if st in total or (st, p) in fin or not before((prev, p), b):
                    continue
                if st == "xq" and VQO.index(p) // XQMAX > b:
                    continue
                if st == "pv":
                    if b < nb and VP[b] == p:
                        fin[(st, p)] = b
                    continue
                small[b].append((st, p))
                fin[(st, p)] = b
                if st == "gs2":
                    late.append(("xl", p))
        cap = 10 ** 6
        if b < nb:
            nab = 12 - (SKEW if b == 0 else 0) + (SKEW if b == nb - 1 else 0)
            vload = 95 * nab + 31 + VOFF + sum(VCOST.get(s, 0) for s, _ in small[b])
            cap = CAPS.get(b, 4 * int(round((vload - 147) / 32.0)))
            assert fin.get(("pv", VP[b])) == b
        if b + 1 < nb:
            assert before((qlast[VP[b + 1]], VP[b + 1]), b)
            cap -= issue(b, "QK", VP[b + 1], nt)
        if b + 2 < nb and VP[b + 2] in GM:
            assert before((qlast[VP[b + 2]], VP[b + 2]), b)
            cap -= issue(b, "QK", VP[b + 2], nt)
        for d in (3, 4):
            if b + d < nb and VP[b + d] not in VQ and (d == 3 or VP[b + d] in GM):
                cap -= issue(b, "QP", VP[b + d], 15)
        cands = [("QK", p, qlast[p]) for p in VP[b + 2:b + 3] if b in RA]
        cands += [("QP", p, None) for p in XP if p not in VQ] + [("QK", p, qlast[p]) for p in XP]
        cands += [("PM", p, "gs2") for p in XP] + [("QP", p, None) for p in VP if p not in VQ]
        cands += [("WO", p, "orx" if p in XP else "or2") for p in VP + XP if p not in VW]
        cands += [("QK", p, qlast[p]) for p in VP]
        for kind, p, need in cands:
            if need is None or before((need, p), b):
                cap -= issue(b, kind, p, cap)
        b += 1
    return mxu, small


def _group_of(p, which):
    return next(i for i, g in enumerate(KVG) if g[which] and g[which][0] <= p < g[which][1])


def _make_kernel(SK, W):
    NC = W // 128
    NC2, NG = NC // 2, NC // 8
    qscale = DH ** -0.5 * math.log2(math.e)
    nk = sum(1 for kr, _ in KVG if kr)
    nv, nw2 = len(KVG), len(W2CUT) - 1

    def kernel(x_hbm, k_hbm, v_hbm, wq_hbm, wo_hbm, w1_hbm, w3_hbm, w2_hbm, o_ref, *scratch):
        kbs, vbs = scratch[:nk], scratch[nk:nk + nv]
        w2s = scratch[nk + nv:nk + nv + nw2]
        (wqb, wob, w1, w3, xb, xs, xrow, lx, stat, csum, qacc, qraw, lq, sraw, pbuf, st, oacc,
         otile, lp, pmraw, lo, woraw, xacc, hcol, sem) = scratch[nk + nv + nw2:]
        k32s = [r.bitcast(u32) for r in kbs]
        v32 = vbs[0].bitcast(u32)
        wq32 = wqb.bitcast(u32)
        wo32 = wob.bitcast(u32)
        wg32 = [w1.bitcast(u32), w3.bitcast(u32)]

        groups = [[(x_hbm, xb), (wq_hbm, wqb), (wo_hbm, wob)]]
        for i, (kr, vr) in enumerate(KVG):
            grp = []
            if kr:
                grp.append((k_hbm.at[kr[0] * AH:kr[1] * AH, :, pl.ds((SK - W) // 256, NC2)], kbs[i]))
            grp.append((v_hbm.at[vr[0] * 2 * AH:vr[1] * 2 * AH, pl.ds((SK - W) // 16, W // 16), :], vbs[i]))
            groups.append(grp)
        gffn = len(groups)
        groups += [[(w1_hbm, w1)], [(w3_hbm, w3)]]
        for i in range(nw2):
            groups.append([(w2_hbm.at[W2CUT[i]:W2CUT[i + 1]], w2s[i])])
        groups = [[pltpu.make_async_copy(s, d, sem.at[g]) for s, d in grp]
                  for g, grp in enumerate(groups)]
        for grp in groups:
            for cp in grp:
                cp.start()

        def gwait(g):
            for cp in groups[g]:
                cp.wait()

        sub = lax.broadcasted_iota(jnp.int32, (8, 128), 0)
        lane = lax.broadcasted_iota(jnp.int32, (8, 128), 1)

        def kvready(i):
            gwait(1 + i)
            if KVG[i][0]:
                k32 = k32s[i]

                def swap(r, carry):
                    a = k32[r, 0, :, 4:8, :]
                    b = k32[r, 1, :, 0:4, :]
                    k32[r, 0, :, 4:8, :] = b
                    k32[r, 1, :, 0:4, :] = a
                    return carry
                lax.fori_loop(0, k32.shape[0], swap, 0)

        def retile(w32, rows):
            n = w32.shape[1] // 2

            def body(rb, carry):
                r = pl.ds(rb * rows, rows)
                a = w32[r, 0:n, 4:8, :]
                b = w32[r, n:2 * n, 0:4, :]
                w32[r, 0:n, 4:8, :] = b
                w32[r, n:2 * n, 0:4, :] = a
                return carry
            lax.fori_loop(0, w32.shape[0] // rows, body, 0)

        def retile_wo(rb, carry):
            r = pl.ds(rb * 4, 4)
            vals = {(e, cc): wo32[r, 4 * (5 * e + cc):4 * (5 * e + cc) + 4, :]
                    for e in range(2) for cc in range(5)}
            for (e, cc), v in vals.items():
                wo32[r, 8 * cc + 4 * e:8 * cc + 4 * e + 4, :] = v
            return carry

        def transpose_wq(i, carry):
            c = i + 3 * NPX + jnp.where(i >= 3 * (NX - NPX), 9, 0)
            slot = (c & 1) * 24 + (c >> 1)
            ones = jnp.ones((16, 128), bf16)
            tiles = [_tile(wq32[8 * kk:8 * kk + 8, slot]) for kk in range(5)]
            csum[i] = _tree(jnp.add, [jnp.dot(ones, t, preferred_element_type=f32)[0:8] for t in tiles])
            for kk in range(5):
                wq32[8 * kk:8 * kk + 8, slot] = pltpu.bitcast(tiles[kk].T, u32).reshape(8, 8, 128)
            return carry

        def transpose_v(i, carry):
            a0 = pl.multiple_of((i >> 2) * 16, 16)
            for u in range(4):
                c2 = (i & 3) * 4 + u
                x = vbs[0][pl.ds(a0, 16), pl.ds(pl.multiple_of(c2 * 16, 16), 16), :]
                ts = [x[:, 8 * h:8 * h + 8, :].reshape(128, 128).T for h in range(2)]
                for h in range(2):
                    v32[pl.ds(a0 + 8 * h, 8), pl.ds(pl.multiple_of(c2 * 8, 8), 8), :] = (
                        pltpu.bitcast(ts[h], u32).reshape(8, 8, 128))
            return carry

        gwait(0)
        retile(wq32, 1)
        lax.fori_loop(0, HD // 64, retile_wo, 0)
        if NVQ:
            lax.fori_loop(0, 3 * NVQ, transpose_wq, 0)
        kvready(0)
        lax.fori_loop(0, NX * 3 * NC2 // 4, transpose_v, 0)

        def wq_slot(p, t):
            c = 3 * p + t
            return (c & 1) * 24 + (c >> 1)

        def qp_job(p, k, pin=tuple):
            kk, t = divmod(k, 3)
            qraw[MQ.index(p), 5 * t + kk] = _mm(
                lx[kk], wq32[8 * kk:8 * kk + 8, wq_slot(p, t)], pin())[0:8]

        def keep_rows(dst, t, c, r):
            g, j = divmod(c, 8)
            if t < 2:
                dst[0, t, g, j:j + 1, :] = r[j:j + 1]
            if t > 0:
                dst[1, t - 1, g, j:j + 1, :] = r[8 + j:9 + j]

        def qk_job(p, k, pin=tuple):
            t, c = divmod(k, NC)
            g = _group_of(p, 0)
            r0 = (p - KVG[g][0][0]) * AH + 8 * t
            keep_rows(sraw.at[p], t, c, _mm(lq[p, t], k32s[g][r0:r0 + 8, c & 1, c >> 1], pin()))

        def pm_job(p, k, pin=tuple):
            t, c = divmod(k, NC)
            a0 = p * 2 * AH + 16 * t + 8 * (c & 1)
            w = v32[a0:a0 + 8, 8 * (c >> 1):8 * (c >> 1) + 8, :]
            keep_rows(pmraw.at[p], t, c, _mm(lp[p, c // 8], w, pin()))

        def wo_job(p, k, pin=tuple):
            t, cc = divmod(k, 5)
            r0 = 24 * p + 8 * t
            woraw[MW.index(p), k] = _mm(lo[p, t], wo32[r0:r0 + 8, 8 * cc:8 * cc + 8, :], pin())[0:8]

        def lane_sums(p, src):
            for a in range(2 * AH):
                r = _bc(jnp.sum(src(a), axis=1, keepdims=True))
                t, k = divmod(a, 16)
                otile[p, t, :, 8 * k:8 * k + 8] = r[:, 8 * k:8 * k + 8]

        def xq(p):
            lane_sums(p, lambda a: qacc[VQO.index(p) % NQA, a])

        def xmax(p):
            for e in range(2):
                st[p, e, 2] = _bc(jnp.max(st[p, e, 0], axis=1, keepdims=True))

        def xl(p):
            for e in range(2):
                st[p, e, 3] = _bc(jnp.sum(st[p, e, 1], axis=1, keepdims=True))

        def xsum(p):
            xl(p)
            lane_sums(p, lambda a: oacc[p % RING, a])

        def xcol(p):
            xl(p)
            for a in range(2 * AH):
                oacc[p % RING, a] = _bc(jnp.sum(oacc[p % RING, a], axis=1, keepdims=True))

        def store_lq(p, t, q):
            qp = _pack(q)
            if t == 1:
                qp = jnp.where((lane >> 6) == (sub >> 2), qp, jnp.uint32(0))
            lq[p, t] = qp

        def qprep(p):
            for t in range(3):
                qv = _tree(jnp.add, [qraw[MQ.index(p), 5 * t + kk] for kk in range(5)])
                store_lq(p, t, _bc(_ln_fix(qv, stat[0], stat[1])[0:1]))

        def vqp_jobs(p):
            def job(i, kk, env):
                w = jnp.stack([wq32[8 * kk + i, wq_slot(p, t)] for t in range(3)])
                w = pltpu.bitcast(w.reshape(24, 128), bf16).astype(f32).reshape(3, 2, 8, 128)
                t_ = w * xrow[kk]
                env["acc"] = t_ if kk == 0 else env["acc"] + t_
                if kk == 4:
                    for t in range(3):
                        qacc[VQO.index(p) % NQA, 16 * t + 2 * i:16 * t + 2 * i + 2] = env["acc"][t]
            jobs = []
            for i in range(8):
                env = {}
                jobs += [functools.partial(job, i, kk, env) for kk in range(5)]
            return jobs

        def qprepv(p):
            for t in range(3):
                raw = _allsub(jnp.add, jnp.where((lane & 7) == sub, otile[p, t], 0.0))
                store_lq(p, t, (raw - stat[0] * csum[3 * VQ.index(p) + t]) * stat[1])

        def scores(p, e):
            return [sraw[p, e, 0, g] + sraw[p, e, 1, g] for g in range(NG)]

        def gmax(p):
            for e in range(2):
                mv = _tree(jnp.maximum, scores(p, e))
                st[p, e, 2] = _bc(jnp.max(mv, axis=1, keepdims=True))

        def probs(p, e):
            m = _allsub(jnp.maximum, st[p, e, 2])
            return [jnp.exp2(x - m) for x in scores(p, e)]

        def sm_jobs(p, e):
            env = {}

            def head():
                if p in GM:
                    env["p"] = probs(p, e)
                    return
                s = scores(p, e)
                mv = _allsub(jnp.maximum, _tree(jnp.maximum, s))
                st[p, e, 0] = mv
                env["p"] = [jnp.exp2(x - mv) for x in s]

            def spread(c0):
                for c in range(c0, c0 + SMG):
                    pbuf[e, c] = _bc(env["p"][c // 8][c % 8:c % 8 + 1])

            def lsum():
                st[p, e, 1] = _allsub(jnp.add, _tree(jnp.add, env["p"]))
            return [head] + [functools.partial(spread, c0) for c0 in range(0, NC, SMG)] + [lsum]

        def pv_jobs(p, e):
            g = _group_of(p, 1)

            def job(a0, c2, env):
                a = (p - KVG[g][1][0]) * 2 * AH + e * AH + a0
                v = vbs[g][a:a + AB, 16 * c2:16 * c2 + 16, :].astype(f32)
                t = v[:, 0:8] * pbuf[e, 2 * c2] + v[:, 8:16] * pbuf[e, 2 * c2 + 1]
                env["acc"] = t if c2 == 0 else env["acc"] + t
                if c2 == NC2 - 1:
                    oacc[p % RING, e * AH + a0:e * AH + a0 + AB] = env["acc"]
            jobs = []
            for a0 in range(0, AH, AB):
                env = {}
                jobs += [functools.partial(job, a0, c2, env) for c2 in range(NC2)]
            return jobs

        def scale_jobs(p):
            def head(e, env):
                env["w"] = jnp.exp2(st[p, e, 0] - st[p, e, 2])
                st[p, e, 1] = env["w"] * st[p, e, 1]

            def job(a, env):
                oacc[p % RING, a:a + ORG] = oacc[p % RING, a:a + ORG] * env["w"]
            jobs = []
            for e in range(2):
                env = {}
                jobs.append(functools.partial(head, e, env))
                jobs += [functools.partial(job, e * AH + a, env) for a in range(0, AH, ORG)]
            return jobs

        def store_lo(p, tiles):
            inv = [_recip(st[p, e, 3]) for e in range(2)]
            invs = [inv[0], jnp.where(lane < 64, inv[0], inv[1]), inv[1]]
            for t in range(3):
                lo[p, t] = _pack(jnp.where((lane & 7) == sub, tiles[t] * invs[t], 0.0))

        def or2(p):
            store_lo(p, [otile[p, t] for t in range(3)])

        def gs2(p):
            ps = [probs(p, e) for e in range(2)]
            for e in range(2):
                st[p, e, 1] = _allsub(jnp.add, _tree(jnp.add, ps[e]))
            for g in range(NG):
                lp[p, g] = _pack(ps[0][g], ps[1][g])

        def orx(p):
            def part(e, t):
                return _tree(jnp.add, [pmraw[p, e, t, g] for g in range(NG)])
            tiles = [part(0, 0), jnp.where(lane < 64, part(0, 1), part(1, 0)), part(1, 1)]
            store_lo(p, [_allsub(jnp.add, x) for x in tiles])

        def woacc(p):
            raw = woraw.at[MW.index(p)]
            xacc[...] = xacc[...] + (raw[0:5] + raw[5:10] + raw[10:15])

        def vwo_jobs(p):
            def job(e, r, env):
                w = pltpu.bitcast(wo32[24 * p + 12 * e + r], bf16).astype(f32).reshape(5, 16, 128)
                a = e * AH + 2 * r
                t = w[:, 0:8] * oacc[p % RING, a] + w[:, 8:16] * oacc[p % RING, a + 1]
                env["acc"] = t if r == 0 else env["acc"] + t
                if r == AH // 2 - 1:
                    xacc[...] = xacc[...] + env["acc"] * _recip(st[p, e, 3])
            jobs = []
            for e in range(2):
                env = {}
                jobs += [functools.partial(job, e, r, env) for r in range(AH // 2)]
            return jobs

        mxu_fn = {"QP": qp_job, "QK": qk_job, "PM": pm_job, "WO": wo_job}
        xlu_fn = {"xq": xq, "gmax": gmax, "xmax": xmax, "xl": xl, "xsum": xsum, "xcol": xcol}
        valu_fn = {"qprep": qprep, "qprepv": qprepv, "or2": or2, "gs2": gs2, "orx": orx,
                   "woacc": woacc}
        plan_mxu, plan_small = _plan(3 * NC)

        def jobs_of(b):
            mx = [functools.partial(mxu_fn[kind], p, k)
                  for kind, p, k0, k1 in plan_mxu[b] for k in range(k0, k1)]
            xj = [functools.partial(xlu_fn[s], p) for s, p in plan_small[b] if s in xlu_fn]
            vj = [functools.partial(valu_fn[s], p) for s, p in plan_small[b] if s in valu_fn]
            sc = [j for s, p in plan_small[b] if s == "scale" for j in scale_jobs(p)]
            vw = [j for s, p in plan_small[b] if s == "vwo" for j in vwo_jobs(p)]
            vw += [j for s, p in plan_small[b] if s == "vqp" for j in vqp_jobs(p)]
            return mx, xj, vj, sc, vw

        def block(b):
            p = VP[b]
            mx, xj, vj, sc, vw = jobs_of(b)
            sa, sb = sm_jobs(p, 0), sm_jobs(p, 1)
            pa, pb = pv_jobs(p, 0), pv_jobs(p, 1)
            cut = len(pb) - SKEW * NC2
            if b + 1 < len(VP):
                pb = pb[:cut]
            if b > 0:
                valu = _weave(pv_jobs(VP[b - 1], 1)[cut:], sa, 0.0, 0.9) + pa[:NC2]
            else:
                valu = sa[:3] + _weave(pa[:NC2], sa[3:], 0.0, 1.0 - 1.0 * SMG / NC)
            valu += _weave(pa[NC2:], sb, 0.1, 0.8) + vw
            valu += _weave(pb, vj + sc, 0.0, 0.9) if vj + sc else pb
            k = int(len(mx) * PIN)
            for s, q in plan_small[b]:
                refs = []
                if s in ("xsum", "xl", "xmax", "gmax", "xcol"):
                    refs += [st.at[q, e, 2 if "max" in s else 3] for e in range(2)]
                if s in ("xsum", "xq"):
                    refs += [otile.at[q, t] for t in range(3)]
                for ref in refs:
                    mx[k] = functools.partial(mx[k], pin=lambda ref=ref: (ref[...],))
                    k += PINGAP
                if s == "xcol":
                    k = max(k, PINL)
                    for a in range(2 * AH - 3, 2 * AH):
                        ref = oacc.at[q % RING, a]
                        mx[k] = functools.partial(mx[k], pin=lambda ref=ref: (ref[...],))
                        k += 1
            _run(mx[:MXF] + xj + _weave(valu, mx[MXF:], 0.0, MX1))

        def set_x(x):
            xs[...] = x
            xl_ = _ln_lhs(x)
            for kk in range(5):
                xrow[kk] = x[:, 128 * kk:128 * kk + 128]
                lx[kk] = _pack(xl_[:, 128 * kk:128 * kk + 128])

        def prologue():
            def stats():
                m, r = _ln_stats(xs[...])
                stat[0] = _bc(m)
                stat[1] = _bc(r * qscale)
                xacc[...] = jnp.zeros_like(xacc)
            mx = [stats]
            for p in PQ:
                mx += [functools.partial(qp_job, p, k) for k in range(15)]
                mx.append(functools.partial(qprep, p))
            mx += [functools.partial(qk_job, VP[0], k) for k in range(3 * NC)]
            bulk = [j for p in VQO[:NVP] for j in vqp_jobs(p)]
            _run(mx[:MXF + 1] + _weave(bulk, mx[MXF + 1:], 0.0, MXP) if bulk else mx)

        def finish_layer(first):
            for b in range(len(VP), len(plan_mxu)):
                mx, xj, vj, sc, vw = jobs_of(b)
                _run(xj + sc + vj + vw + mx)
            att = jnp.sum(jnp.concatenate([xacc[cc] for cc in range(5)], axis=1),
                          axis=0, keepdims=True)
            x1 = _rnd(xs[...] + _rnd(att))
            if first:
                xs[...] = x1
                for i in range(2):
                    gwait(gffn + i)
                    retile(wg32[i], 4)
                x1 = xs[...]
            m, r = _ln_stats(x1)
            xl_ = _ln_lhs(x1)
            lf = [_pack(xl_[:, 128 * kk:128 * kk + 128]) for kk in range(5)]
            nh = F // 128
            on_vpu = range(W2CUT[-2] // 128, nh) if first else range(NVH)

            def w2rows(j):
                i = next(i for i in range(nw2) if W2CUT[i] <= 128 * j < W2CUT[i + 1])
                return w2s[i][128 * j - W2CUT[i]:128 * j - W2CUT[i] + 128, :]

            def tile_dot(lhs, w):
                return jnp.dot(pltpu.bitcast(lhs, bf16), w, preferred_element_type=f32)[0:8]

            def gate_up(j):
                slot = (j & 1) * (nh // 2) + (j >> 1)
                parts = [[tile_dot(lf[kk], _tile(wg32[i][8 * kk:8 * kk + 8, slot])) for i in range(2)]
                         for kk in range(5)]
                g, u = [_ln_fix(_tree(jnp.add, [pp[i] for pp in parts]), m, r) for i in range(2)]
                return _rnd(g * jax.nn.sigmoid(g) * u)

            def hcols(h):
                hb = _bc(h[0:1])
                return [_bc(jnp.sum(jnp.where(lane == 8 * a + sub, hb, 0.0), axis=1, keepdims=True))
                        for a in range(16)]

            def vpu_rows(j, cols, yv):
                w = w2rows(j).astype(f32)
                for a in range(16):
                    t = w[8 * a:8 * a + 8] * jnp.tile(cols[a], (1, 5))
                    yv = t if yv is None else yv + t
                return yv

            hs, y, yv = [], None, None
            for j in range(nh):
                hs.append(gate_up(j))
                if j in on_vpu:
                    if first:
                        hcol[...] = jnp.stack(hcols(hs[j]))
                    else:
                        yv = vpu_rows(j, hcols(hs[j]), yv)
            for j in range(nh):
                if first and 128 * j in W2CUT:
                    i = W2CUT.index(128 * j)
                    if i:
                        xs[...] = y
                    gwait(gffn + 2 + i)
                    if i:
                        y = xs[...]
                if j not in on_vpu:
                    lh, w = _pack(hs[j]), w2rows(j)
                    t = jnp.concatenate([tile_dot(lh, w[:, 128 * cc:128 * cc + 128]) for cc in range(5)],
                                        axis=1)
                    y = t if y is None else y + t
                elif first:
                    yv = vpu_rows(j, [hcol[a] for a in range(16)], yv)
            y = y[0:1]
            if yv is not None:
                y = y + jnp.sum(yv, axis=0, keepdims=True)
            if first:
                set_x(_rnd(x1 + _rnd(y)))
            else:
                o_ref[...] = (x1[0:1] + _rnd(y)).astype(o_ref.dtype)

        def layer_body(layer, carry):
            first = layer == 0
            prologue()
            seen = 1
            for b in range(len(VP)):
                need = 1 + max([_group_of(VP[b], 1)] + [_group_of(p, 0) for kind, p, _, _ in plan_mxu[b]
                                                        if kind == "QK"])
                if need > seen:
                    @pl.when(first)
                    def _(lo_=seen, hi_=need):
                        for i in range(lo_, hi_):
                            kvready(i)
                    seen = need
                if ONLY is None or b in ONLY:
                    pl.when(layer < 100 + b)(functools.partial(block, b))
            lax.cond(first, lambda: finish_layer(True), lambda: finish_layer(False))
            return carry

        set_x(jnp.broadcast_to(xb[...].astype(f32), (8, D)))
        lax.fori_loop(0, 2, layer_body, 0)
    return kernel


def _tile_linear(c):
    sk = c.shape[2]
    return (jnp.swapaxes(c, 2, 3).reshape(NA, 8, sk // 128, 128)
            .transpose(0, 2, 1, 3).reshape(NA, sk // 16, 128))


@jax.jit
def pallas_interleave_layers__sliding_block_cached__glu_gated_swiglu__decode_kernel(
    A_x: jax.Array,
    A_k_cache: jax.Array,
    A_v_cache: jax.Array,
    A_wq: jax.Array,
    A_wo: jax.Array,
    B_x: jax.Array,
    B_w1: jax.Array,
    B_w3: jax.Array,
    B_w2: jax.Array,
):
    SK = A_k_cache.shape[2]
    W = min(4096, max(256, SK // 4))
    nc2 = W // 256
    kx = _tile_linear(A_k_cache).reshape(NA // 2, 2, SK // 256, 16, 128)
    vx = _tile_linear(A_v_cache)
    wqz, w1z, w3z = [(w.reshape(D // 16, 2, 8, w.shape[1] // 256, 2, 128).transpose(0, 1, 3, 4, 2, 5)
                      .reshape(D // 16, w.shape[1] // 128, 16, 128)) for w in (A_wq, B_w1, B_w3)]
    woz = (A_wo.reshape(HD // 16, 2, 8, 5, 128).transpose(0, 1, 3, 2, 4)
           .reshape(HD // 16, 80, 128))
    vreg = lambda *lead, dt=f32: pltpu.VMEM(lead + (8, 128), dt)
    scratch = [pltpu.VMEM(((kr[1] - kr[0]) * AH, 2, nc2, 16, 128), bf16) for kr, _ in KVG if kr]
    scratch += [pltpu.VMEM(((vr[1] - vr[0]) * 2 * AH, W // 16, 128), bf16) for _, vr in KVG]
    scratch += [pltpu.VMEM((b - a, D), bf16) for a, b in zip(W2CUT, W2CUT[1:])]
    scratch += [
        pltpu.VMEM((D // 16, 48, 16, 128), bf16),
        pltpu.VMEM((HD // 16, 80, 128), bf16),
        pltpu.VMEM((D // 16, F // 128, 16, 128), bf16),
        pltpu.VMEM((D // 16, F // 128, 16, 128), bf16),
        pltpu.VMEM((1, D), bf16),
        pltpu.VMEM((8, D), f32),
        vreg(5),
        vreg(5, dt=u32),
        vreg(2),
        vreg(max(3 * NVQ, 1)),
        vreg(NQA, 2 * AH),
        vreg(len(MQ), 15),
        vreg(NP, 3, dt=u32),
        vreg(NP, 2, 2, nc2 // 4),
        vreg(2, 2 * nc2),
        vreg(NP, 2, 4),
        vreg(RING, 2 * AH),
        vreg(NP, 3),
        vreg(NX, nc2 // 4, dt=u32),
        vreg(NX, 2, 2, nc2 // 4),
        vreg(NP, 3, dt=u32),
        vreg(len(MW), 15),
        vreg(5),
        vreg(16),
        pltpu.SemaphoreType.DMA((len(KVG) + 2 + len(W2CUT),)),
    ]
    out = pl.pallas_call(
        _make_kernel(SK, W),
        out_shape=jax.ShapeDtypeStruct((1, D), A_x.dtype),
        in_specs=[pl.BlockSpec(memory_space=pl.ANY)] * 8,
        out_specs=pl.BlockSpec(memory_space=pltpu.VMEM),
        scratch_shapes=scratch,
        compiler_params=pltpu.CompilerParams(vmem_limit_bytes=126 * 1024 * 1024,
                                             disable_semaphore_checks=True),
    )(A_x.reshape(1, D), kx, vx, wqz, woz, w1z, w3z, B_w2)
    return out.reshape(1, 1, D)
```

```python
import functools
import math

import jax
import jax.numpy as jnp
from jax import lax
import jax.experimental.pallas as pl
import jax.experimental.pallas.tpu as pltpu

H, DH, D, F = 32, 192, 640, 1536
HD = H * DH
EPS = 1e-5
NA = HD // 8
AH = DH // 8
NP = H // 2
NX = 4
XP = list(range(NX))
VP = list(range(NX, NP))
NVQ = 9
BSZ = [1,1,2,2,2,1,1,1,1]
BL = [VP[sum(BSZ[:i]):sum(BSZ[:i + 1])] for i in range(len(BSZ))]
NPV = 4
NPX = 0
PQ = VP[:NPV] + XP[:NPX]
VQ = (XP[NPX:] + VP[NPV:])[:NVQ]
VQO = sorted(VQ, key=lambda p: 2 * (XP.index(p) - NPX) + 2.5 if p in XP else 1.5 * (VP.index(p) - NPV))
NVP = 7
VQB = 1
VW = [4,5,6,7,8,15]
MQ = [p for p in range(NP) if p not in VQ]
MW = [p for p in range(NP) if p not in VW]
GFROM = 13
GM = VP[GFROM:]
RA = [0]
NQA = 8
RING = 8
KVG = [((0, 8), (0, 5)), ((8, 12), (5, 8)), ((12, 16), (8, 12)), (None, (12, 14)), (None, (14, 16))]
W2CUT = (0, 1024, 1408, 1536)
AB = 4
SKEW = 1
VOFF = 70
VOFF2 = 20
VCOST = {"qprep": 10, "qprepv": 14, "scale": 14, "or2": 8, "woacc": 4, "gmax": 4, "gs2": 19,
         "orx": 18, "vwo": 186, "vqp": 170, "xsum": 4, "xq": 4}
CAPS = {}
XQMAX = 4
MXF = 4
MX1 = 1.02
MXP = 1.0
PINK = 22
PINGAP = 5
PINL = 36
SMG = 4
ORG = 4
NVH = 7
ONLY = None
f32, bf16, u32 = jnp.float32, jnp.bfloat16, jnp.uint32


def _ln_stats(x):
    m = jnp.mean(x, axis=-1, keepdims=True)
    xc = x - m
    v = jnp.mean(xc * xc, axis=-1, keepdims=True)
    return m, lax.rsqrt(v + EPS)


def _ln_lhs(x):
    return jnp.where(lax.broadcasted_iota(jnp.int32, x.shape, 0) < 4, x, 1.0)


def _ln_fix(raw, m, r):
    return (raw - m * pltpu.roll(raw, 4, 0)) * r


def _rnd(x):
    return x.astype(bf16).astype(f32)


def _pack(lo, hi=None):
    return pltpu.bitcast(jnp.concatenate([lo, lo if hi is None else hi], axis=0).astype(bf16), u32)


def _tile(w_u32):
    return pltpu.bitcast(w_u32.reshape(64, 128), bf16)


def _mm(lhs_u32, w_u32, pin=()):
    if pin:
        lhs_u32 = jnp.concatenate([lhs_u32] + [pltpu.bitcast(x, u32) for x in pin], axis=0)
    return jnp.dot(pltpu.bitcast(lhs_u32, bf16), _tile(w_u32), preferred_element_type=f32)[0:16]


def _bc(x):
    return jnp.broadcast_to(x, (8, 128))


def _tree(op, xs):
    xs = list(xs)
    while len(xs) > 1:
        xs = [op(xs[i], xs[i + 1]) if i + 1 < len(xs) else xs[i] for i in range(0, len(xs), 2)]
    return xs[0]


def _allsub(op, x):
    for sh in (4, 2, 1):
        x = op(x, pltpu.roll(x, sh, 0))
    return x


def _recip(l):
    r = pl.reciprocal(l, approx=True)
    return r * (2.0 - l * r)


def _run(jobs):
    for j in jobs:
        j()


def _weave(main, extra, lo, hi):
    out, k = [], 0
    for n, j in enumerate(main):
        while k < len(extra) and lo * len(main) + k * (hi - lo) * len(main) / len(extra) <= n:
            out.append(extra[k])
            k += 1
        out.append(j)
    return out + list(extra[k:])


def _plan(nt):
    nb = len(BL)
    total = {"QP": 15, "QK": nt, "PM": nt, "WO": 15}
    done, fin, mxu, small = {}, {}, {}, {}

    def issue(b, kind, p, cap):
        k0 = done.get((kind, p), 0)
        n = max(min(total[kind] - k0, cap), 0)
        if n:
            mxu[b].append((kind, p, k0, k0 + n))
            done[(kind, p)] = k0 + n
            if k0 + n == total[kind]:
                fin[(kind, p)] = b
        return n

    def before(key, b):
        return fin.get(key, b) < b

    chains, qlast = {}, {}
    for p in range(NP):
        ch = ["vqp", "xq", "qprepv"] if p in VQ else ["QP", "qprep"]
        qlast[p] = ch[-1]
        if p in XP:
            ch += ["QK", "gmax", "gs2", "PM", "orx", "WO", "woacc"]
        else:
            if p in GM:
                ch += ["QK", "gmax", "pv"] + (["skew"] if p != VP[-1] else [])
            else:
                ch += ["QK", "pv", "xmax", "scale"]
            ch += ["xcol", "vwo"] if p in VW else ["xsum", "or2", "WO", "woacc"]
        chains[p] = ch
    for p in VQO[:NVP]:
        fin[("vqp", p)] = -1
    for p in PQ:
        done[("QP", p)] = 15
        fin[("QP", p)] = fin[("qprep", p)] = -1
    done[("QK", VP[0])] = nt
    fin[("QK", VP[0])] = -1
    late = []
    b = 0
    while any((chains[p][-1], p) not in fin for p in range(NP)):
        mxu[b], small[b], late = [], late, []
        for p in VQO[NVP + VQB * b:NVP + VQB * (b + 1)]:
            small[b].append(("vqp", p))
            fin[("vqp", p)] = b
        for p in range(NP):
            for prev, st in zip(chains[p], chains[p][1:]):
                if st in total or (st, p) in fin or not before((prev, p), b):
                    continue
                if st == "xq" and VQO.index(p) // XQMAX > b:
                    continue
                if st == "pv":
                    if b < nb and p in BL[b]:
                        fin[(st, p)] = b
                    continue
                small[b].append((st, p))
                fin[(st, p)] = b
                if st == "gs2":
                    late.append(("xl", p))
        cap = 10 ** 6
        if b < nb:
            nab = 12 * BSZ[b] - (SKEW if b == 0 else 0) + (SKEW if b == nb - 1 else 0)
            vload = (95 * nab + (31 + VOFF) * BSZ[b] - VOFF2 * (BSZ[b] - 1)
                     + sum(VCOST.get(s, 0) for s, _ in small[b]))
            cap = CAPS.get(b, 4 * int(round((vload - 147) / 32.0)))
            assert all(fin.get(("pv", p)) == b for p in BL[b])
        for d in (1, 2):
            for p in (BL[b + d] if b + d < nb else []):
                if d == 1 or p in GM:
                    assert ("QK", p) in fin or before((qlast[p], p), b), (b, p)
                    cap -= issue(b, "QK", p, nt)
        for d in (3, 4):
            for p in (BL[b + d] if b + d < nb else []):
                if p not in VQ and (d == 3 or p in GM):
                    cap -= issue(b, "QP", p, 15)
        cands = [("QK", p, qlast[p]) for p in (BL[b + 2] if b + 2 < nb and b in RA else [])]
        cands += [("QP", p, None) for p in XP if p not in VQ] + [("QK", p, qlast[p]) for p in XP]
        cands += [("PM", p, "gs2") for p in XP] + [("QP", p, None) for p in VP if p not in VQ]
        cands += [("WO", p, "orx" if p in XP else "or2") for p in VP + XP if p not in VW]
        cands += [("QK", p, qlast[p]) for p in VP]
        for kind, p, need in cands:
            if need is None or before((need, p), b):
                cap -= issue(b, kind, p, cap)
        b += 1
    return mxu, small


def _group_of(p, which):
    return next(i for i, g in enumerate(KVG) if g[which] and g[which][0] <= p < g[which][1])


def _make_kernel(SK, W):
    NC = W // 128
    NC2, NG = NC // 2, NC // 8
    qscale = DH ** -0.5 * math.log2(math.e)
    nk = sum(1 for kr, _ in KVG if kr)
    nv, nw2 = len(KVG), len(W2CUT) - 1

    def kernel(x_hbm, k_hbm, v_hbm, wq_hbm, wo_hbm, w1_hbm, w3_hbm, w2_hbm, o_ref, *scratch):
        kbs, vbs = scratch[:nk], scratch[nk:nk + nv]
        w2s = scratch[nk + nv:nk + nv + nw2]
        (wqb, wob, w1, w3, xb, xs, xrow, lx, stat, csum, qacc, qraw, lq, sraw, pbuf, st, oacc,
         otile, lp, pmraw, lo, woraw, xacc, hcol, sem) = scratch[nk + nv + nw2:]
        k32s = [r.bitcast(u32) for r in kbs]
        v32 = vbs[0].bitcast(u32)
        wq32 = wqb.bitcast(u32)
        wo32 = wob.bitcast(u32)
        wg32 = [w1.bitcast(u32), w3.bitcast(u32)]

        groups = [[(x_hbm, xb), (wq_hbm, wqb), (wo_hbm, wob)]]
        for i, (kr, vr) in enumerate(KVG):
            grp = []
            if kr:
                grp.append((k_hbm.at[kr[0] * AH:kr[1] * AH, :, pl.ds((SK - W) // 256, NC2)], kbs[i]))
            grp.append((v_hbm.at[vr[0] * 2 * AH:vr[1] * 2 * AH, pl.ds((SK - W) // 16, W // 16), :], vbs[i]))
            groups.append(grp)
        gffn = len(groups)
        groups += [[(w1_hbm, w1)], [(w3_hbm, w3)]]
        for i in range(nw2):
            groups.append([(w2_hbm.at[W2CUT[i]:W2CUT[i + 1]], w2s[i])])
        groups = [[pltpu.make_async_copy(s, d, sem.at[g]) for s, d in grp]
                  for g, grp in enumerate(groups)]
        for grp in groups:
            for cp in grp:
                cp.start()

        def gwait(g):
            for cp in groups[g]:
                cp.wait()

        sub = lax.broadcasted_iota(jnp.int32, (8, 128), 0)
        lane = lax.broadcasted_iota(jnp.int32, (8, 128), 1)

        def kvready(i):
            gwait(1 + i)
            if KVG[i][0]:
                k32 = k32s[i]

                def swap(r, carry):
                    a = k32[r, 0, :, 4:8, :]
                    b = k32[r, 1, :, 0:4, :]
                    k32[r, 0, :, 4:8, :] = b
                    k32[r, 1, :, 0:4, :] = a
                    return carry
                lax.fori_loop(0, k32.shape[0], swap, 0)

        def retile(w32, rows):
            n = w32.shape[1] // 2

            def body(rb, carry):
                r = pl.ds(rb * rows, rows)
                a = w32[r, 0:n, 4:8, :]
                b = w32[r, n:2 * n, 0:4, :]
                w32[r, 0:n, 4:8, :] = b
                w32[r, n:2 * n, 0:4, :] = a
                return carry
            lax.fori_loop(0, w32.shape[0] // rows, body, 0)

        def retile_wo(rb, carry):
            r = pl.ds(rb * 4, 4)
            vals = {(e, cc): wo32[r, 4 * (5 * e + cc):4 * (5 * e + cc) + 4, :]
                    for e in range(2) for cc in range(5)}
            for (e, cc), v in vals.items():
                wo32[r, 8 * cc + 4 * e:8 * cc + 4 * e + 4, :] = v
            return carry

        def transpose_wq(i, carry):
            c = i + 3 * NPX + jnp.where(i >= 3 * (NX - NPX), 3 * NPV, 0)
            slot = (c & 1) * 24 + (c >> 1)
            ones = jnp.ones((16, 128), bf16)
            tiles = [_tile(wq32[8 * kk:8 * kk + 8, slot]) for kk in range(5)]
            csum[i] = _tree(jnp.add, [jnp.dot(ones, t, preferred_element_type=f32)[0:8] for t in tiles])
            for kk in range(5):
                wq32[8 * kk:8 * kk + 8, slot] = pltpu.bitcast(tiles[kk].T, u32).reshape(8, 8, 128)
            return carry

        def transpose_v(i, carry):
            a0 = pl.multiple_of((i >> 2) * 16, 16)
            for u in range(4):
                c2 = (i & 3) * 4 + u
                x = vbs[0][pl.ds(a0, 16), pl.ds(pl.multiple_of(c2 * 16, 16), 16), :]
                ts = [x[:, 8 * h:8 * h + 8, :].reshape(128, 128).T for h in range(2)]
                for h in range(2):
                    v32[pl.ds(a0 + 8 * h, 8), pl.ds(pl.multiple_of(c2 * 8, 8), 8), :] = (
                        pltpu.bitcast(ts[h], u32).reshape(8, 8, 128))
            return carry

        gwait(0)
        retile(wq32, 1)
        lax.fori_loop(0, HD // 64, retile_wo, 0)
        if NVQ:
            lax.fori_loop(0, 3 * NVQ, transpose_wq, 0)
        kvready(0)
        lax.fori_loop(0, NX * 3 * NC2 // 4, transpose_v, 0)

        def wq_slot(p, t):
            c = 3 * p + t
            return (c & 1) * 24 + (c >> 1)

        def qp_job(p, k, pin=tuple):
            kk, t = divmod(k, 3)
            qraw[MQ.index(p), 5 * t + kk] = _mm(
                lx[kk], wq32[8 * kk:8 * kk + 8, wq_slot(p, t)], pin())[0:8]

        def keep_rows(dst, t, c, r):
            g, j = divmod(c, 8)
            if t < 2:
                dst[0, t, g, j:j + 1, :] = r[j:j + 1]
            if t > 0:
                dst[1, t - 1, g, j:j + 1, :] = r[8 + j:9 + j]

        def qk_job(p, k, pin=tuple):
            t, c = divmod(k, NC)
            g = _group_of(p, 0)
            r0 = (p - KVG[g][0][0]) * AH + 8 * t
            keep_rows(sraw.at[p], t, c, _mm(lq[p, t], k32s[g][r0:r0 + 8, c & 1, c >> 1], pin()))

        def pm_job(p, k, pin=tuple):
            t, c = divmod(k, NC)
            a0 = p * 2 * AH + 16 * t + 8 * (c & 1)
            w = v32[a0:a0 + 8, 8 * (c >> 1):8 * (c >> 1) + 8, :]
            keep_rows(pmraw.at[p], t, c, _mm(lp[p, c // 8], w, pin()))

        def wo_job(p, k, pin=tuple):
            t, cc = divmod(k, 5)
            r0 = 24 * p + 8 * t
            woraw[MW.index(p), k] = _mm(lo[p, t], wo32[r0:r0 + 8, 8 * cc:8 * cc + 8, :], pin())[0:8]

        def lane_sums(p, src):
            for a in range(2 * AH):
                r = _bc(jnp.sum(src(a), axis=1, keepdims=True))
                t, k = divmod(a, 16)
                otile[p, t, :, 8 * k:8 * k + 8] = r[:, 8 * k:8 * k + 8]

        def xq(p):
            lane_sums(p, lambda a: qacc[VQO.index(p) % NQA, a])

        def xmax(p):
            for e in range(2):
                st[p, e, 2] = _bc(jnp.max(st[p, e, 0], axis=1, keepdims=True))

        def xl(p):
            for e in range(2):
                st[p, e, 3] = _bc(jnp.sum(st[p, e, 1], axis=1, keepdims=True))

        def xsum(p):
            xl(p)
            lane_sums(p, lambda a: oacc[p % RING, a])

        def xcol(p):
            xl(p)
            for a in range(2 * AH):
                oacc[p % RING, a] = _bc(jnp.sum(oacc[p % RING, a], axis=1, keepdims=True))

        def store_lq(p, t, q):
            qp = _pack(q)
            if t == 1:
                qp = jnp.where((lane >> 6) == (sub >> 2), qp, jnp.uint32(0))
            lq[p, t] = qp

        def qprep(p):
            for t in range(3):
                qv = _tree(jnp.add, [qraw[MQ.index(p), 5 * t + kk] for kk in range(5)])
                store_lq(p, t, _bc(_ln_fix(qv, stat[0], stat[1])[0:1]))

        def vqp_jobs(p):
            def job(i, kk, env):
                w = jnp.stack([wq32[8 * kk + i, wq_slot(p, t)] for t in range(3)])
                w = pltpu.bitcast(w.reshape(24, 128), bf16).astype(f32).reshape(3, 2, 8, 128)
                t_ = w * xrow[kk]
                env["acc"] = t_ if kk == 0 else env["acc"] + t_
                if kk == 4:
                    for t in range(3):
                        qacc[VQO.index(p) % NQA, 16 * t + 2 * i:16 * t + 2 * i + 2] = env["acc"][t]
            jobs = []
            for i in range(8):
                env = {}
                jobs += [functools.partial(job, i, kk, env) for kk in range(5)]
            return jobs

        def qprepv(p):
            for t in range(3):
                raw = _allsub(jnp.add, jnp.where((lane & 7) == sub, otile[p, t], 0.0))
                store_lq(p, t, (raw - stat[0] * csum[3 * VQ.index(p) + t]) * stat[1])

        def scores(p, e):
            return [sraw[p, e, 0, g] + sraw[p, e, 1, g] for g in range(NG)]

        def gmax(p):
            for e in range(2):
                mv = _tree(jnp.maximum, scores(p, e))
                st[p, e, 2] = _bc(jnp.max(mv, axis=1, keepdims=True))

        def probs(p, e):
            m = _allsub(jnp.maximum, st[p, e, 2])
            return [jnp.exp2(x - m) for x in scores(p, e)]

        def sm_jobs(p, e):
            env = {}

            def head():
                if p in GM:
                    env["p"] = probs(p, e)
                    return
                s = scores(p, e)
                mv = _allsub(jnp.maximum, _tree(jnp.maximum, s))
                st[p, e, 0] = mv
                env["p"] = [jnp.exp2(x - mv) for x in s]

            def spread(c0):
                for c in range(c0, c0 + SMG):
                    pbuf[e, c] = _bc(env["p"][c // 8][c % 8:c % 8 + 1])

            def lsum():
                st[p, e, 1] = _allsub(jnp.add, _tree(jnp.add, env["p"]))
            return [head] + [functools.partial(spread, c0) for c0 in range(0, NC, SMG)] + [lsum]

        def pv_jobs(p, e):
            g = _group_of(p, 1)

            def job(a0, c2, env):
                a = (p - KVG[g][1][0]) * 2 * AH + e * AH + a0
                v = vbs[g][a:a + AB, 16 * c2:16 * c2 + 16, :].astype(f32)
                t = v[:, 0:8] * pbuf[e, 2 * c2] + v[:, 8:16] * pbuf[e, 2 * c2 + 1]
                env["acc"] = t if c2 == 0 else env["acc"] + t
                if c2 == NC2 - 1:
                    oacc[p % RING, e * AH + a0:e * AH + a0 + AB] = env["acc"]
            jobs = []
            for a0 in range(0, AH, AB):
                env = {}
                jobs += [functools.partial(job, a0, c2, env) for c2 in range(NC2)]
            return jobs

        def scale_jobs(p):
            def head(e, env):
                env["w"] = jnp.exp2(st[p, e, 0] - st[p, e, 2])
                st[p, e, 1] = env["w"] * st[p, e, 1]

            def job(a, env):
                oacc[p % RING, a:a + ORG] = oacc[p % RING, a:a + ORG] * env["w"]
            jobs = []
            for e in range(2):
                env = {}
                jobs.append(functools.partial(head, e, env))
                jobs += [functools.partial(job, e * AH + a, env) for a in range(0, AH, ORG)]
            return jobs

        def store_lo(p, tiles):
            inv = [_recip(st[p, e, 3]) for e in range(2)]
            invs = [inv[0], jnp.where(lane < 64, inv[0], inv[1]), inv[1]]
            for t in range(3):
                lo[p, t] = _pack(jnp.where((lane & 7) == sub, tiles[t] * invs[t], 0.0))

        def or2(p):
            store_lo(p, [otile[p, t] for t in range(3)])

        def gs2(p):
            ps = [probs(p, e) for e in range(2)]
            for e in range(2):
                st[p, e, 1] = _allsub(jnp.add, _tree(jnp.add, ps[e]))
            for g in range(NG):
                lp[p, g] = _pack(ps[0][g], ps[1][g])

        def orx(p):
            def part(e, t):
                return _tree(jnp.add, [pmraw[p, e, t, g] for g in range(NG)])
            tiles = [part(0, 0), jnp.where(lane < 64, part(0, 1), part(1, 0)), part(1, 1)]
            store_lo(p, [_allsub(jnp.add, x) for x in tiles])

        def woacc(p):
            raw = woraw.at[MW.index(p)]
            xacc[...] = xacc[...] + (raw[0:5] + raw[5:10] + raw[10:15])

        def vwo_jobs(p):
            def job(e, r, env):
                w = pltpu.bitcast(wo32[24 * p + 12 * e + r], bf16).astype(f32).reshape(5, 16, 128)
                a = e * AH + 2 * r
                t = w[:, 0:8] * oacc[p % RING, a] + w[:, 8:16] * oacc[p % RING, a + 1]
                env["acc"] = t if r == 0 else env["acc"] + t
                if r == AH // 2 - 1:
                    xacc[...] = xacc[...] + env["acc"] * _recip(st[p, e, 3])
            jobs = []
            for e in range(2):
                env = {}
                jobs += [functools.partial(job, e, r, env) for r in range(AH // 2)]
            return jobs

        mxu_fn = {"QP": qp_job, "QK": qk_job, "PM": pm_job, "WO": wo_job}
        xlu_fn = {"xq": xq, "gmax": gmax, "xmax": xmax, "xl": xl, "xsum": xsum, "xcol": xcol}
        valu_fn = {"qprep": qprep, "qprepv": qprepv, "or2": or2, "gs2": gs2, "orx": orx,
                   "woacc": woacc}
        plan_mxu, plan_small = _plan(3 * NC)

        def jobs_of(b):
            mx = [functools.partial(mxu_fn[kind], p, k)
                  for kind, p, k0, k1 in plan_mxu[b] for k in range(k0, k1)]
            xj = [functools.partial(xlu_fn[s], p) for s, p in plan_small[b] if s in xlu_fn]
            vj = [functools.partial(valu_fn[s], p) for s, p in plan_small[b] if s in valu_fn]
            sc = [j for s, p in plan_small[b] if s == "scale" for j in scale_jobs(p)]
            vw = [j for s, p in plan_small[b] if s == "vwo" for j in vwo_jobs(p)]
            vw += [j for s, p in plan_small[b] if s == "vqp" for j in vqp_jobs(p)]
            return mx, xj, vj, sc, vw

        def block(b):
            mx, xj, vj, sc, vw = jobs_of(b)
            valu = []
            for n, p in enumerate(BL[b]):
                sa, sb = sm_jobs(p, 0), sm_jobs(p, 1)
                pa, pb = pv_jobs(p, 0), pv_jobs(p, 1)
                cut = len(pb) - SKEW * NC2
                if p != VP[-1]:
                    pb = pb[:cut]
                if p != VP[0]:
                    valu += _weave(pv_jobs(p - 1, 1)[cut:], sa, 0.0, 0.9) + pa[:NC2]
                else:
                    valu += sa[:3] + _weave(pa[:NC2], sa[3:], 0.0, 1.0 - 1.0 * SMG / NC)
                valu += _weave(pa[NC2:], sb, 0.1, 0.8)
                if n == 0:
                    valu += vw + (_weave(pb, vj + sc, 0.0, 0.9) if vj + sc else pb)
                else:
                    valu += pb
            k = PINK
            for s, q in plan_small[b]:
                refs = []
                if s in ("xsum", "xl", "xmax", "gmax", "xcol"):
                    refs += [st.at[q, e, 2 if "max" in s else 3] for e in range(2)]
                if s in ("xsum", "xq"):
                    refs += [otile.at[q, t] for t in range(3)]
                for ref in refs:
                    mx[k] = functools.partial(mx[k], pin=lambda ref=ref: (ref[...],))
                    k += PINGAP
                if s == "xcol":
                    k = max(k, PINL)
                    for a in range(2 * AH - 3, 2 * AH):
                        ref = oacc.at[q % RING, a]
                        mx[k] = functools.partial(mx[k], pin=lambda ref=ref: (ref[...],))
                        k += 1
            _run(mx[:MXF] + xj + _weave(valu, mx[MXF:], 0.0, MX1))

        def set_x(x):
            xs[...] = x
            xl_ = _ln_lhs(x)
            for kk in range(5):
                xrow[kk] = x[:, 128 * kk:128 * kk + 128]
                lx[kk] = _pack(xl_[:, 128 * kk:128 * kk + 128])

        def prologue():
            def stats():
                m, r = _ln_stats(xs[...])
                stat[0] = _bc(m)
                stat[1] = _bc(r * qscale)
                xacc[...] = jnp.zeros_like(xacc)
            mx = [stats]
            for p in PQ:
                mx += [functools.partial(qp_job, p, k) for k in range(15)]
                mx.append(functools.partial(qprep, p))
            mx += [functools.partial(qk_job, VP[0], k) for k in range(3 * NC)]
            bulk = [j for p in VQO[:NVP] for j in vqp_jobs(p)]
            _run(mx[:MXF + 1] + _weave(bulk, mx[MXF + 1:], 0.0, MXP) if bulk else mx)

        def finish_layer(first):
            for b in range(len(BL), len(plan_mxu)):
                mx, xj, vj, sc, vw = jobs_of(b)
                _run(xj + sc + vj + vw + mx)
            att = jnp.sum(jnp.concatenate([xacc[cc] for cc in range(5)], axis=1),
                          axis=0, keepdims=True)
            x1 = _rnd(xs[...] + _rnd(att))
            if first:
                xs[...] = x1
                for i in range(2):
                    gwait(gffn + i)
                    retile(wg32[i], 4)
                x1 = xs[...]
            m, r = _ln_stats(x1)
            xl_ = _ln_lhs(x1)
            lf = [_pack(xl_[:, 128 * kk:128 * kk + 128]) for kk in range(5)]
            nh = F // 128
            on_vpu = range(W2CUT[-2] // 128, nh) if first else range(NVH)

            def w2rows(j):
                i = next(i for i in range(nw2) if W2CUT[i] <= 128 * j < W2CUT[i + 1])
                return w2s[i][128 * j - W2CUT[i]:128 * j - W2CUT[i] + 128, :]

            def tile_dot(lhs, w):
                return jnp.dot(pltpu.bitcast(lhs, bf16), w, preferred_element_type=f32)[0:8]

            def gate_up(j):
                slot = (j & 1) * (nh // 2) + (j >> 1)
                parts = [[tile_dot(lf[kk], _tile(wg32[i][8 * kk:8 * kk + 8, slot])) for i in range(2)]
                         for kk in range(5)]
                g, u = [_ln_fix(_tree(jnp.add, [pp[i] for pp in parts]), m, r) for i in range(2)]
                return _rnd(g * jax.nn.sigmoid(g) * u)

            def hcols(h):
                hb = _bc(h[0:1])
                return [_bc(jnp.sum(jnp.where(lane == 8 * a + sub, hb, 0.0), axis=1, keepdims=True))
                        for a in range(16)]

            def vpu_rows(j, cols, yv):
                w = w2rows(j).astype(f32)
                for a in range(16):
                    t = w[8 * a:8 * a + 8] * jnp.tile(cols[a], (1, 5))
                    yv = t if yv is None else yv + t
                return yv

            hs, y, yv = [], None, None
            for j in range(nh):
                hs.append(gate_up(j))
                if j in on_vpu:
                    if first:
                        hcol[...] = jnp.stack(hcols(hs[j]))
                    else:
                        yv = vpu_rows(j, hcols(hs[j]), yv)
            for j in range(nh):
                if first and 128 * j in W2CUT:
                    i = W2CUT.index(128 * j)
                    if i:
                        xs[...] = y
                    gwait(gffn + 2 + i)
                    if i:
                        y = xs[...]
                if j not in on_vpu:
                    lh, w = _pack(hs[j]), w2rows(j)
                    t = jnp.concatenate([tile_dot(lh, w[:, 128 * cc:128 * cc + 128]) for cc in range(5)],
                                        axis=1)
                    y = t if y is None else y + t
                elif first:
                    yv = vpu_rows(j, [hcol[a] for a in range(16)], yv)
            y = y[0:1]
            if yv is not None:
                y = y + jnp.sum(yv, axis=0, keepdims=True)
            if first:
                set_x(_rnd(x1 + _rnd(y)))
            else:
                o_ref[...] = (x1[0:1] + _rnd(y)).astype(o_ref.dtype)

        def layer_body(layer, carry):
            first = layer == 0
            prologue()
            seen = 1
            for b in range(len(BL)):
                need = 1 + max([_group_of(BL[b][-1], 1)] + [_group_of(p, 0) for kind, p, _, _ in plan_mxu[b]
                                                        if kind == "QK"])
                if need > seen:
                    @pl.when(first)
                    def _(lo_=seen, hi_=need):
                        for i in range(lo_, hi_):
                            kvready(i)
                    seen = need
                if ONLY is None or b in ONLY:
                    pl.when(layer < 100 + b)(functools.partial(block, b))
            lax.cond(first, lambda: finish_layer(True), lambda: finish_layer(False))
            return carry

        set_x(jnp.broadcast_to(xb[...].astype(f32), (8, D)))
        lax.fori_loop(0, 2, layer_body, 0)
    return kernel


def _tile_linear(c):
    sk = c.shape[2]
    return (jnp.swapaxes(c, 2, 3).reshape(NA, 8, sk // 128, 128)
            .transpose(0, 2, 1, 3).reshape(NA, sk // 16, 128))


@jax.jit
def pallas_interleave_layers__sliding_block_cached__glu_gated_swiglu__decode_kernel(
    A_x: jax.Array,
    A_k_cache: jax.Array,
    A_v_cache: jax.Array,
    A_wq: jax.Array,
    A_wo: jax.Array,
    B_x: jax.Array,
    B_w1: jax.Array,
    B_w3: jax.Array,
    B_w2: jax.Array,
):
    SK = A_k_cache.shape[2]
    W = min(4096, max(256, SK // 4))
    nc2 = W // 256
    kx = _tile_linear(A_k_cache).reshape(NA // 2, 2, SK // 256, 16, 128)
    vx = _tile_linear(A_v_cache)
    wqz, w1z, w3z = [(w.reshape(D // 16, 2, 8, w.shape[1] // 256, 2, 128).transpose(0, 1, 3, 4, 2, 5)
                      .reshape(D // 16, w.shape[1] // 128, 16, 128)) for w in (A_wq, B_w1, B_w3)]
    woz = (A_wo.reshape(HD // 16, 2, 8, 5, 128).transpose(0, 1, 3, 2, 4)
           .reshape(HD // 16, 80, 128))
    vreg = lambda *lead, dt=f32: pltpu.VMEM(lead + (8, 128), dt)
    scratch = [pltpu.VMEM(((kr[1] - kr[0]) * AH, 2, nc2, 16, 128), bf16) for kr, _ in KVG if kr]
    scratch += [pltpu.VMEM(((vr[1] - vr[0]) * 2 * AH, W // 16, 128), bf16) for _, vr in KVG]
    scratch += [pltpu.VMEM((b - a, D), bf16) for a, b in zip(W2CUT, W2CUT[1:])]
    scratch += [
        pltpu.VMEM((D // 16, 48, 16, 128), bf16),
        pltpu.VMEM((HD // 16, 80, 128), bf16),
        pltpu.VMEM((D // 16, F // 128, 16, 128), bf16),
        pltpu.VMEM((D // 16, F // 128, 16, 128), bf16),
        pltpu.VMEM((1, D), bf16),
        pltpu.VMEM((8, D), f32),
        vreg(5),
        vreg(5, dt=u32),
        vreg(2),
        vreg(max(3 * NVQ, 1)),
        vreg(NQA, 2 * AH),
        vreg(len(MQ), 15),
        vreg(NP, 3, dt=u32),
        vreg(NP, 2, 2, nc2 // 4),
        vreg(2, 2 * nc2),
        vreg(NP, 2, 4),
        vreg(RING, 2 * AH),
        vreg(NP, 3),
        vreg(NX, nc2 // 4, dt=u32),
        vreg(NX, 2, 2, nc2 // 4),
        vreg(NP, 3, dt=u32),
        vreg(len(MW), 15),
        vreg(5),
        vreg(16),
        pltpu.SemaphoreType.DMA((len(KVG) + 2 + len(W2CUT),)),
    ]
    out = pl.pallas_call(
        _make_kernel(SK, W),
        out_shape=jax.ShapeDtypeStruct((1, D), A_x.dtype),
        in_specs=[pl.BlockSpec(memory_space=pl.ANY)] * 8,
        out_specs=pl.BlockSpec(memory_space=pltpu.VMEM),
        scratch_shapes=scratch,
        compiler_params=pltpu.CompilerParams(vmem_limit_bytes=126 * 1024 * 1024,
                                             disable_semaphore_checks=True),
    )(A_x.reshape(1, D), kx, vx, wqz, woz, w1z, w3z, B_w2)
    return out.reshape(1, 1, D)
```

```python
import functools
import math

import jax
import jax.numpy as jnp
from jax import lax
import jax.experimental.pallas as pl
import jax.experimental.pallas.tpu as pltpu

H, DH, D, F = 32, 192, 640, 1536
HD = H * DH
EPS = 1e-5
NA = HD // 8
AH = DH // 8
NP = H // 2
NX = 4
XP = list(range(NX))
VP = list(range(NX, NP))
NVQ = 10
BSZ = [1,1,2,2,2,1,1,1,1]
BL = [VP[sum(BSZ[:i]):sum(BSZ[:i + 1])] for i in range(len(BSZ))]
NPV = 4
NPX = 0
PQ = VP[:NPV] + XP[:NPX]
VQ = (XP[NPX:] + VP[NPV:])[:NVQ]
XK = 2
VQO = sorted(VQ, key=lambda p: XK * (XP.index(p) - NPX) + 2.5 if p in XP else 1.5 * (VP.index(p) - NPV))
NVP = 7
VQB = 1
VW = [5,6,9,10,11,15]
MQ = [p for p in range(NP) if p not in VQ]
MW = [p for p in range(NP) if p not in VW]
RA = [0,5]
NQA = 8
RING = 8
KVG = [((0, 8), (0, 5)), ((8, 12), (5, 8)), ((12, 16), (8, 12)), (None, (12, 14)), (None, (14, 16))]
W2CUT = (0, 1024, 1408, 1536)
AB = 4
SKEW = 1
VOFF = 70
VOFF2 = 20
VCOST = {"qprep": 10, "qprepv": 14, "scale": 14, "or2": 8, "woacc": 4, "gmax": 4, "gs2": 19,
         "orx": 18, "vwo": 186, "vqp": 170, "xsum": 4, "xq": 4}
CAPS = {}
XQMAX = 4
MXF = 4
MX1 = 1.02
MXP = 1.0
PINK = 14
PINGAP = 6
PINGS = 1
SMG = 4
ORG = 4
NVH = 7
ONLY = None
f32, bf16, u32 = jnp.float32, jnp.bfloat16, jnp.uint32


def _ln_stats(x):
    m = jnp.mean(x, axis=-1, keepdims=True)
    xc = x - m
    v = jnp.mean(xc * xc, axis=-1, keepdims=True)
    return m, lax.rsqrt(v + EPS)


def _ln_lhs(x):
    return jnp.where(lax.broadcasted_iota(jnp.int32, x.shape, 0) < 4, x, 1.0)


def _ln_fix(raw, m, r):
    return (raw - m * pltpu.roll(raw, 4, 0)) * r


def _rnd(x):
    return x.astype(bf16).astype(f32)


def _pack(lo, hi=None):
    return pltpu.bitcast(jnp.concatenate([lo, lo if hi is None else hi], axis=0).astype(bf16), u32)


def _tile(w_u32):
    return pltpu.bitcast(w_u32.reshape(64, 128), bf16)


def _mm(lhs_u32, w_u32, pin=()):
    if pin:
        lhs_u32 = jnp.concatenate([lhs_u32] + [pltpu.bitcast(x, u32) for x in pin], axis=0)
    return jnp.dot(pltpu.bitcast(lhs_u32, bf16), _tile(w_u32), preferred_element_type=f32)[0:16]


def _bc(x):
    return jnp.broadcast_to(x, (8, 128))


def _tree(op, xs):
    xs = list(xs)
    while len(xs) > 1:
        xs = [op(xs[i], xs[i + 1]) if i + 1 < len(xs) else xs[i] for i in range(0, len(xs), 2)]
    return xs[0]


def _allsub(op, x):
    for sh in (4, 2, 1):
        x = op(x, pltpu.roll(x, sh, 0))
    return x


def _recip(l):
    r = pl.reciprocal(l, approx=True)
    return r * (2.0 - l * r)


def _run(jobs):
    for j in jobs:
        j()


def _weave(main, extra, lo, hi):
    out, k = [], 0
    for n, j in enumerate(main):
        while k < len(extra) and lo * len(main) + k * (hi - lo) * len(main) / len(extra) <= n:
            out.append(extra[k])
            k += 1
        out.append(j)
    return out + list(extra[k:])


def _plan(nt):
    nb = len(BL)
    total = {"QP": 15, "QK": nt, "PM": nt, "WO": 15}
    done, fin, mxu, small = {}, {}, {}, {}

    def issue(b, kind, p, cap):
        k0 = done.get((kind, p), 0)
        n = max(min(total[kind] - k0, cap), 0)
        if n:
            mxu[b].append((kind, p, k0, k0 + n))
            done[(kind, p)] = k0 + n
            if k0 + n == total[kind]:
                fin[(kind, p)] = b
        return n

    def before(key, b):
        return fin.get(key, b) < b

    chains, qlast = {}, {}
    for p in range(NP):
        ch = ["vqp", "xq", "qprepv"] if p in VQ else ["QP", "qprep"]
        qlast[p] = ch[-1]
        if p in XP:
            ch += ["QK", "gmax", "gs2", "PM", "orx", "WO", "woacc"]
        else:
            ch += ["QK", "pv", "xmax", "scale"]
            ch += ["xcol", "vwo"] if p in VW else ["xsum", "or2", "WO", "woacc"]
        chains[p] = ch
    for p in VQO[:NVP]:
        fin[("vqp", p)] = -1
    for p in PQ:
        done[("QP", p)] = 15
        fin[("QP", p)] = fin[("qprep", p)] = -1
    done[("QK", VP[0])] = nt
    fin[("QK", VP[0])] = -1
    late = []
    b = 0
    while any((chains[p][-1], p) not in fin for p in range(NP)):
        mxu[b], small[b], late = [], late, []
        for p in VQO[NVP + VQB * b:NVP + VQB * (b + 1)]:
            small[b].append(("vqp", p))
            fin[("vqp", p)] = b
        for p in range(NP):
            for prev, st in zip(chains[p], chains[p][1:]):
                if st in total or (st, p) in fin or not before((prev, p), b):
                    continue
                if st == "xq" and VQO.index(p) // XQMAX > b:
                    continue
                if st == "pv":
                    if b < nb and p in BL[b]:
                        fin[(st, p)] = b
                    continue
                small[b].append((st, p))
                fin[(st, p)] = b
                if st == "gs2":
                    late.append(("xl", p))
        cap = 10 ** 6
        if b < nb:
            nab = 12 * BSZ[b] - (SKEW if b == 0 else 0) + (SKEW if b == nb - 1 else 0)
            vload = (95 * nab + (31 + VOFF) * BSZ[b] - VOFF2 * (BSZ[b] - 1)
                     + sum(VCOST.get(s, 0) for s, _ in small[b]))
            cap = CAPS.get(b, 4 * int(round((vload - 147) / 32.0)))
            assert all(fin.get(("pv", p)) == b for p in BL[b])
        for p in (BL[b + 1] if b + 1 < nb else []):
            assert ("QK", p) in fin or before((qlast[p], p), b)
            cap -= issue(b, "QK", p, nt)
        for p in (BL[b + 3] if b + 3 < nb else []):
            if p not in VQ:
                cap -= issue(b, "QP", p, 15)
        cands = [("QK", p, qlast[p]) for p in (BL[b + 2] if b + 2 < nb and b in RA else [])]
        cands += [("QP", p, None) for p in XP if p not in VQ] + [("QK", p, qlast[p]) for p in XP]
        cands += [("PM", p, "gs2") for p in XP] + [("QP", p, None) for p in VP if p not in VQ]
        cands += [("WO", p, "orx" if p in XP else "or2") for p in VP + XP if p not in VW]
        cands += [("QK", p, qlast[p]) for p in VP]
        for kind, p, need in cands:
            if need is None or before((need, p), b):
                cap -= issue(b, kind, p, cap)
        b += 1
    for p in VP[RING:]:
        assert fin[("vwo" if p - RING in VW else "xsum", p - RING)] < fin[("pv", p)]
    for i in range(NQA, NVQ):
        assert fin[("xq", VQO[i - NQA])] < fin[("vqp", VQO[i])]
    return mxu, small


def _group_of(p, which):
    return next(i for i, g in enumerate(KVG) if g[which] and g[which][0] <= p < g[which][1])


def _make_kernel(SK, W):
    NC = W // 128
    NC2, NG = NC // 2, NC // 8
    qscale = DH ** -0.5 * math.log2(math.e)
    nk = sum(1 for kr, _ in KVG if kr)
    nv, nw2 = len(KVG), len(W2CUT) - 1

    def kernel(x_hbm, k_hbm, v_hbm, wq_hbm, wo_hbm, w1_hbm, w3_hbm, w2_hbm, o_ref, *scratch):
        kbs, vbs = scratch[:nk], scratch[nk:nk + nv]
        w2s = scratch[nk + nv:nk + nv + nw2]
        (wqb, wob, w1, w3, xb, xs, xrow, lx, stat, csum, qacc, qraw, lq, sraw, pbuf, st, oacc,
         otile, lp, pmraw, lo, woraw, xacc, hcol, sem) = scratch[nk + nv + nw2:]
        k32s = [r.bitcast(u32) for r in kbs]
        v32 = vbs[0].bitcast(u32)
        wq32 = wqb.bitcast(u32)
        wo32 = wob.bitcast(u32)
        wg32 = [w1.bitcast(u32), w3.bitcast(u32)]

        groups = [[(x_hbm, xb), (wq_hbm, wqb), (wo_hbm, wob)]]
        for i, (kr, vr) in enumerate(KVG):
            grp = []
            if kr:
                grp.append((k_hbm.at[kr[0] * AH:kr[1] * AH, :, pl.ds((SK - W) // 256, NC2)], kbs[i]))
            grp.append((v_hbm.at[vr[0] * 2 * AH:vr[1] * 2 * AH, pl.ds((SK - W) // 16, W // 16), :], vbs[i]))
            groups.append(grp)
        gffn = len(groups)
        groups += [[(w1_hbm, w1)], [(w3_hbm, w3)]]
        for i in range(nw2):
            groups.append([(w2_hbm.at[W2CUT[i]:W2CUT[i + 1]], w2s[i])])
        groups = [[pltpu.make_async_copy(s, d, sem.at[g]) for s, d in grp]
                  for g, grp in enumerate(groups)]
        for grp in groups:
            for cp in grp:
                cp.start()

        def gwait(g):
            for cp in groups[g]:
                cp.wait()

        sub = lax.broadcasted_iota(jnp.int32, (8, 128), 0)
        lane = lax.broadcasted_iota(jnp.int32, (8, 128), 1)

        def kvready(i):
            gwait(1 + i)
            if KVG[i][0]:
                k32 = k32s[i]

                def swap(r, carry):
                    a = k32[r, 0, :, 4:8, :]
                    b = k32[r, 1, :, 0:4, :]
                    k32[r, 0, :, 4:8, :] = b
                    k32[r, 1, :, 0:4, :] = a
                    return carry
                lax.fori_loop(0, k32.shape[0], swap, 0)

        def retile(w32, rows):
            n = w32.shape[1] // 2

            def body(rb, carry):
                r = pl.ds(rb * rows, rows)
                a = w32[r, 0:n, 4:8, :]
                b = w32[r, n:2 * n, 0:4, :]
                w32[r, 0:n, 4:8, :] = b
                w32[r, n:2 * n, 0:4, :] = a
                return carry
            lax.fori_loop(0, w32.shape[0] // rows, body, 0)

        def retile_wo(rb, carry):
            r = pl.ds(rb * 4, 4)
            vals = {(e, cc): wo32[r, 4 * (5 * e + cc):4 * (5 * e + cc) + 4, :]
                    for e in range(2) for cc in range(5)}
            for (e, cc), v in vals.items():
                wo32[r, 8 * cc + 4 * e:8 * cc + 4 * e + 4, :] = v
            return carry

        def transpose_wq(i, carry):
            c = i + 3 * NPX + jnp.where(i >= 3 * (NX - NPX), 3 * NPV, 0)
            slot = (c & 1) * 24 + (c >> 1)
            ones = jnp.ones((16, 128), bf16)
            tiles = [_tile(wq32[8 * kk:8 * kk + 8, slot]) for kk in range(5)]
            csum[i] = _tree(jnp.add, [jnp.dot(ones, t, preferred_element_type=f32)[0:8] for t in tiles])
            for kk in range(5):
                wq32[8 * kk:8 * kk + 8, slot] = pltpu.bitcast(tiles[kk].T, u32).reshape(8, 8, 128)
            return carry

        def transpose_v(i, carry):
            a0 = pl.multiple_of((i >> 2) * 16, 16)
            for u in range(4):
                c2 = (i & 3) * 4 + u
                x = vbs[0][pl.ds(a0, 16), pl.ds(pl.multiple_of(c2 * 16, 16), 16), :]
                ts = [x[:, 8 * h:8 * h + 8, :].reshape(128, 128).T for h in range(2)]
                for h in range(2):
                    v32[pl.ds(a0 + 8 * h, 8), pl.ds(pl.multiple_of(c2 * 8, 8), 8), :] = (
                        pltpu.bitcast(ts[h], u32).reshape(8, 8, 128))
            return carry

        gwait(0)
        retile(wq32, 1)
        lax.fori_loop(0, HD // 64, retile_wo, 0)
        if NVQ:
            lax.fori_loop(0, 3 * NVQ, transpose_wq, 0)
        kvready(0)
        lax.fori_loop(0, NX * 3 * NC2 // 4, transpose_v, 0)

        def wq_slot(p, t):
            c = 3 * p + t
            return (c & 1) * 24 + (c >> 1)

        def qp_job(p, k, pin=tuple):
            kk, t = divmod(k, 3)
            qraw[MQ.index(p), 5 * t + kk] = _mm(
                lx[kk], wq32[8 * kk:8 * kk + 8, wq_slot(p, t)], pin())[0:8]

        def keep_rows(dst, t, c, r):
            g, j = divmod(c, 8)
            if t < 2:
                dst[0, t, g, j:j + 1, :] = r[j:j + 1]
            if t > 0:
                dst[1, t - 1, g, j:j + 1, :] = r[8 + j:9 + j]

        def qk_job(p, k, pin=tuple):
            t, c = divmod(k, NC)
            g = _group_of(p, 0)
            r0 = (p - KVG[g][0][0]) * AH + 8 * t
            keep_rows(sraw.at[p], t, c, _mm(lq[p, t], k32s[g][r0:r0 + 8, c & 1, c >> 1], pin()))

        def pm_job(p, k, pin=tuple):
            t, c = divmod(k, NC)
            a0 = p * 2 * AH + 16 * t + 8 * (c & 1)
            w = v32[a0:a0 + 8, 8 * (c >> 1):8 * (c >> 1) + 8, :]
            keep_rows(pmraw.at[p], t, c, _mm(lp[p, c // 8], w, pin()))

        def wo_job(p, k, pin=tuple):
            t, cc = divmod(k, 5)
            r0 = 24 * p + 8 * t
            woraw[MW.index(p), k] = _mm(lo[p, t], wo32[r0:r0 + 8, 8 * cc:8 * cc + 8, :], pin())[0:8]

        def lane_sums(p, src):
            for a in range(2 * AH):
                r = _bc(jnp.sum(src(a), axis=1, keepdims=True))
                t, k = divmod(a, 16)
                otile[p, t, :, 8 * k:8 * k + 8] = r[:, 8 * k:8 * k + 8]

        def xq(p):
            lane_sums(p, lambda a: qacc[VQO.index(p) % NQA, a])

        def xmax(p):
            for e in range(2):
                st[p, e, 2] = _bc(jnp.max(st[p, e, 0], axis=1, keepdims=True))

        def xl(p):
            for e in range(2):
                st[p, e, 3] = _bc(jnp.sum(st[p, e, 1], axis=1, keepdims=True))

        def xsum(p):
            xl(p)
            lane_sums(p, lambda a: oacc[p % RING, a])

        def xcol(p):
            xl(p)
            for a in range(2 * AH):
                oacc[p % RING, a] = _bc(jnp.sum(oacc[p % RING, a], axis=1, keepdims=True))

        def store_lq(p, t, q):
            qp = _pack(q)
            if t == 1:
                qp = jnp.where((lane >> 6) == (sub >> 2), qp, jnp.uint32(0))
            lq[p, t] = qp

        def qprep(p):
            for t in range(3):
                qv = _tree(jnp.add, [qraw[MQ.index(p), 5 * t + kk] for kk in range(5)])
                store_lq(p, t, _bc(_ln_fix(qv, stat[0], stat[1])[0:1]))

        def vqp_jobs(p):
            def job(i, kk, env):
                w = jnp.stack([wq32[8 * kk + i, wq_slot(p, t)] for t in range(3)])
                w = pltpu.bitcast(w.reshape(24, 128), bf16).astype(f32).reshape(3, 2, 8, 128)
                t_ = w * xrow[kk]
                env["acc"] = t_ if kk == 0 else env["acc"] + t_
                if kk == 4:
                    for t in range(3):
                        qacc[VQO.index(p) % NQA, 16 * t + 2 * i:16 * t + 2 * i + 2] = env["acc"][t]
            jobs = []
            for i in range(8):
                env = {}
                jobs += [functools.partial(job, i, kk, env) for kk in range(5)]
            return jobs

        def qprepv(p):
            for t in range(3):
                raw = _allsub(jnp.add, jnp.where((lane & 7) == sub, otile[p, t], 0.0))
                store_lq(p, t, (raw - stat[0] * csum[3 * VQ.index(p) + t]) * stat[1])

        def scores(p, e):
            return [sraw[p, e, 0, g] + sraw[p, e, 1, g] for g in range(NG)]

        def gmax(p):
            for e in range(2):
                mv = _tree(jnp.maximum, scores(p, e))
                st[p, e, 2] = _bc(jnp.max(mv, axis=1, keepdims=True))

        def probs(p, e):
            m = _allsub(jnp.maximum, st[p, e, 2])
            return [jnp.exp2(x - m) for x in scores(p, e)]

        def sm_jobs(p, e):
            env = {}

            def head():
                s = scores(p, e)
                mv = _allsub(jnp.maximum, _tree(jnp.maximum, s))
                st[p, e, 0] = mv
                env["p"] = [jnp.exp2(x - mv) for x in s]

            def spread(c0):
                for c in range(c0, c0 + SMG):
                    pbuf[e, c] = _bc(env["p"][c // 8][c % 8:c % 8 + 1])

            def lsum():
                st[p, e, 1] = _allsub(jnp.add, _tree(jnp.add, env["p"]))
            return [head] + [functools.partial(spread, c0) for c0 in range(0, NC, SMG)] + [lsum]

        def pv_jobs(p, e):
            g = _group_of(p, 1)

            def job(a0, c2, env):
                a = (p - KVG[g][1][0]) * 2 * AH + e * AH + a0
                v = vbs[g][a:a + AB, 16 * c2:16 * c2 + 16, :].astype(f32)
                t = v[:, 0:8] * pbuf[e, 2 * c2] + v[:, 8:16] * pbuf[e, 2 * c2 + 1]
                env["acc"] = t if c2 == 0 else env["acc"] + t
                if c2 == NC2 - 1:
                    oacc[p % RING, e * AH + a0:e * AH + a0 + AB] = env["acc"]
            jobs = []
            for a0 in range(0, AH, AB):
                env = {}
                jobs += [functools.partial(job, a0, c2, env) for c2 in range(NC2)]
            return jobs

        def scale_jobs(p):
            def head(e, env):
                env["w"] = jnp.exp2(st[p, e, 0] - st[p, e, 2])
                st[p, e, 1] = env["w"] * st[p, e, 1]

            def job(a, env):
                oacc[p % RING, a:a + ORG] = oacc[p % RING, a:a + ORG] * env["w"]
            jobs = []
            for e in range(2):
                env = {}
                jobs.append(functools.partial(head, e, env))
                jobs += [functools.partial(job, e * AH + a, env) for a in range(0, AH, ORG)]
            return jobs

        def store_lo(p, tiles):
            inv = [_recip(st[p, e, 3]) for e in range(2)]
            invs = [inv[0], jnp.where(lane < 64, inv[0], inv[1]), inv[1]]
            for t in range(3):
                lo[p, t] = _pack(jnp.where((lane & 7) == sub, tiles[t] * invs[t], 0.0))

        def or2(p):
            store_lo(p, [otile[p, t] for t in range(3)])

        def gs2(p):
            ps = [probs(p, e) for e in range(2)]
            for e in range(2):
                st[p, e, 1] = _allsub(jnp.add, _tree(jnp.add, ps[e]))
            for g in range(NG):
                lp[p, g] = _pack(ps[0][g], ps[1][g])

        def orx(p):
            def part(e, t):
                return _tree(jnp.add, [pmraw[p, e, t, g] for g in range(NG)])
            tiles = [part(0, 0), jnp.where(lane < 64, part(0, 1), part(1, 0)), part(1, 1)]
            store_lo(p, [_allsub(jnp.add, x) for x in tiles])

        def woacc(p):
            raw = woraw.at[MW.index(p)]
            xacc[...] = xacc[...] + (raw[0:5] + raw[5:10] + raw[10:15])

        def vwo_jobs(p):
            def job(e, r, env):
                w = pltpu.bitcast(wo32[24 * p + 12 * e + r], bf16).astype(f32).reshape(5, 16, 128)
                a = e * AH + 2 * r
                t = w[:, 0:8] * oacc[p % RING, a] + w[:, 8:16] * oacc[p % RING, a + 1]
                env["acc"] = t if r == 0 else env["acc"] + t
                if r == AH // 2 - 1:
                    xacc[...] = xacc[...] + env["acc"] * _recip(st[p, e, 3])
            jobs = []
            for e in range(2):
                env = {}
                jobs += [functools.partial(job, e, r, env) for r in range(AH // 2)]
            return jobs

        mxu_fn = {"QP": qp_job, "QK": qk_job, "PM": pm_job, "WO": wo_job}
        xlu_fn = {"xq": xq, "gmax": gmax, "xmax": xmax, "xl": xl, "xsum": xsum, "xcol": xcol}
        valu_fn = {"qprep": qprep, "qprepv": qprepv, "or2": or2, "gs2": gs2, "orx": orx,
                   "woacc": woacc}
        plan_mxu, plan_small = _plan(3 * NC)

        def jobs_of(b):
            mx = [functools.partial(mxu_fn[kind], p, k)
                  for kind, p, k0, k1 in plan_mxu[b] for k in range(k0, k1)]
            xj = [functools.partial(xlu_fn[s], p) for s, p in plan_small[b] if s in xlu_fn]
            vj = [functools.partial(valu_fn[s], p) for s, p in plan_small[b] if s in valu_fn]
            sc = [j for s, p in plan_small[b] if s == "scale" for j in scale_jobs(p)]
            vw = [j for s, p in plan_small[b] if s == "vwo" for j in vwo_jobs(p)]
            vw += [j for s, p in plan_small[b] if s == "vqp" for j in vqp_jobs(p)]
            return mx, xj, vj, sc, vw

        def block(b):
            mx, xj, vj, sc, vw = jobs_of(b)
            valu = []
            for n, p in enumerate(BL[b]):
                sa, sb = sm_jobs(p, 0), sm_jobs(p, 1)
                pa, pb = pv_jobs(p, 0), pv_jobs(p, 1)
                cut = len(pb) - SKEW * NC2
                if p != VP[-1]:
                    pb = pb[:cut]
                if p != VP[0]:
                    valu += _weave(pv_jobs(p - 1, 1)[cut:], sa, 0.0, 0.9) + pa[:NC2]
                else:
                    valu += sa[:3] + _weave(pa[:NC2], sa[3:], 0.0, 1.0 - 1.0 * SMG / NC)
                valu += _weave(pa[NC2:], sb, 0.1, 0.8)
                if n == 0:
                    valu += vw + (_weave(pb, vj + sc, 0.0, 0.9) if vj + sc else pb)
                else:
                    valu += pb
            k = PINK
            for s, q in plan_small[b]:
                refs = []
                if s in ("xsum", "xl", "xmax", "gmax", "xcol"):
                    refs += [(st.at[q, e, 2 if "max" in s else 3], PINGS) for e in range(2)]
                if s in ("xsum", "xq"):
                    refs += [(otile.at[q, t], PINGAP) for t in range(3)]
                for ref, gap in refs:
                    k += gap
                    mx[k] = functools.partial(mx[k], pin=lambda ref=ref: (ref[...],))
            _run(mx[:MXF] + xj + _weave(valu, mx[MXF:], 0.0, MX1))

        def set_x(x):
            xs[...] = x
            xl_ = _ln_lhs(x)
            for kk in range(5):
                xrow[kk] = x[:, 128 * kk:128 * kk + 128]
                lx[kk] = _pack(xl_[:, 128 * kk:128 * kk + 128])

        def prologue():
            def stats():
                m, r = _ln_stats(xs[...])
                stat[0] = _bc(m)
                stat[1] = _bc(r * qscale)
                xacc[...] = jnp.zeros_like(xacc)
            mx = [stats]
            for p in PQ:
                mx += [functools.partial(qp_job, p, k) for k in range(15)]
                mx.append(functools.partial(qprep, p))
            mx += [functools.partial(qk_job, VP[0], k) for k in range(3 * NC)]
            bulk = [j for p in VQO[:NVP] for j in vqp_jobs(p)]
            _run(mx[:MXF + 1] + _weave(bulk, mx[MXF + 1:], 0.0, MXP) if bulk else mx)

        def finish_layer(first):
            for b in range(len(BL), len(plan_mxu)):
                mx, xj, vj, sc, vw = jobs_of(b)
                _run(xj + sc + vj + vw + mx)
            att = jnp.sum(jnp.concatenate([xacc[cc] for cc in range(5)], axis=1),
                          axis=0, keepdims=True)
            x1 = _rnd(xs[...] + _rnd(att))
            if first:
                xs[...] = x1
                for i in range(2):
                    gwait(gffn + i)
                    retile(wg32[i], 4)
                x1 = xs[...]
            m, r = _ln_stats(x1)
            xl_ = _ln_lhs(x1)
            lf = [_pack(xl_[:, 128 * kk:128 * kk + 128]) for kk in range(5)]
            nh = F // 128
            on_vpu = range(W2CUT[-2] // 128, nh) if first else range(NVH)

            def w2rows(j):
                i = next(i for i in range(nw2) if W2CUT[i] <= 128 * j < W2CUT[i + 1])
                return w2s[i][128 * j - W2CUT[i]:128 * j - W2CUT[i] + 128, :]

            def tile_dot(lhs, w):
                return jnp.dot(pltpu.bitcast(lhs, bf16), w, preferred_element_type=f32)[0:8]

            def gate_up(j):
                slot = (j & 1) * (nh // 2) + (j >> 1)
                parts = [[tile_dot(lf[kk], _tile(wg32[i][8 * kk:8 * kk + 8, slot])) for i in range(2)]
                         for kk in range(5)]
                g, u = [_ln_fix(_tree(jnp.add, [pp[i] for pp in parts]), m, r) for i in range(2)]
                return _rnd(g * jax.nn.sigmoid(g) * u)

            def hcols(h):
                hb = _bc(h[0:1])
                return [_bc(jnp.sum(jnp.where(lane == 8 * a + sub, hb, 0.0), axis=1, keepdims=True))
                        for a in range(16)]

            def vpu_rows(j, cols, yv):
                w = w2rows(j).astype(f32)
                for a in range(16):
                    t = w[8 * a:8 * a + 8] * jnp.tile(cols[a], (1, 5))
                    yv = t if yv is None else yv + t
                return yv

            hs, y, yv = [], None, None
            for j in range(nh):
                hs.append(gate_up(j))
                if j in on_vpu:
                    if first:
                        hcol[...] = jnp.stack(hcols(hs[j]))
                    else:
                        yv = vpu_rows(j, hcols(hs[j]), yv)
            for j in range(nh):
                if first and 128 * j in W2CUT:
                    i = W2CUT.index(128 * j)
                    if i:
                        xs[...] = y
                    gwait(gffn + 2 + i)
                    if i:
                        y = xs[...]
                if j not in on_vpu:
                    lh, w = _pack(hs[j]), w2rows(j)
                    t = jnp.concatenate([tile_dot(lh, w[:, 128 * cc:128 * cc + 128]) for cc in range(5)],
                                        axis=1)
                    y = t if y is None else y + t
                elif first:
                    yv = vpu_rows(j, [hcol[a] for a in range(16)], yv)
            y = y[0:1]
            if yv is not None:
                y = y + jnp.sum(yv, axis=0, keepdims=True)
            if first:
                set_x(_rnd(x1 + _rnd(y)))
            else:
                o_ref[...] = (x1[0:1] + _rnd(y)).astype(o_ref.dtype)

        def layer_body(layer, carry):
            first = layer == 0
            prologue()
            seen = 1
            for b in range(len(BL)):
                need = 1 + max([_group_of(BL[b][-1], 1)] + [_group_of(p, 0) for kind, p, _, _ in plan_mxu[b]
                                                        if kind == "QK"])
                if need > seen:
                    @pl.when(first)
                    def _(lo_=seen, hi_=need):
                        for i in range(lo_, hi_):
                            kvready(i)
                    seen = need
                if ONLY is None or b in ONLY:
                    pl.when(layer < 100 + b)(functools.partial(block, b))
            lax.cond(first, lambda: finish_layer(True), lambda: finish_layer(False))
            return carry

        set_x(jnp.broadcast_to(xb[...].astype(f32), (8, D)))
        lax.fori_loop(0, 2, layer_body, 0)
    return kernel


def _tile_linear(c):
    sk = c.shape[2]
    return (jnp.swapaxes(c, 2, 3).reshape(NA, 8, sk // 128, 128)
            .transpose(0, 2, 1, 3).reshape(NA, sk // 16, 128))


@jax.jit
def pallas_interleave_layers__sliding_block_cached__glu_gated_swiglu__decode_kernel(
    A_x: jax.Array,
    A_k_cache: jax.Array,
    A_v_cache: jax.Array,
    A_wq: jax.Array,
    A_wo: jax.Array,
    B_x: jax.Array,
    B_w1: jax.Array,
    B_w3: jax.Array,
    B_w2: jax.Array,
):
    SK = A_k_cache.shape[2]
    W = min(4096, max(256, SK // 4))
    nc2 = W // 256
    kx = _tile_linear(A_k_cache).reshape(NA // 2, 2, SK // 256, 16, 128)
    vx = _tile_linear(A_v_cache)
    wqz, w1z, w3z = [(w.reshape(D // 16, 2, 8, w.shape[1] // 256, 2, 128).transpose(0, 1, 3, 4, 2, 5)
                      .reshape(D // 16, w.shape[1] // 128, 16, 128)) for w in (A_wq, B_w1, B_w3)]
    woz = (A_wo.reshape(HD // 16, 2, 8, 5, 128).transpose(0, 1, 3, 2, 4)
           .reshape(HD // 16, 80, 128))
    vreg = lambda *lead, dt=f32: pltpu.VMEM(lead + (8, 128), dt)
    scratch = [pltpu.VMEM(((kr[1] - kr[0]) * AH, 2, nc2, 16, 128), bf16) for kr, _ in KVG if kr]
    scratch += [pltpu.VMEM(((vr[1] - vr[0]) * 2 * AH, W // 16, 128), bf16) for _, vr in KVG]
    scratch += [pltpu.VMEM((b - a, D), bf16) for a, b in zip(W2CUT, W2CUT[1:])]
    scratch += [
        pltpu.VMEM((D // 16, 48, 16, 128), bf16),
        pltpu.VMEM((HD // 16, 80, 128), bf16),
        pltpu.VMEM((D // 16, F // 128, 16, 128), bf16),
        pltpu.VMEM((D // 16, F // 128, 16, 128), bf16),
        pltpu.VMEM((1, D), bf16),
        pltpu.VMEM((8, D), f32),
        vreg(5),
        vreg(5, dt=u32),
        vreg(2),
        vreg(max(3 * NVQ, 1)),
        vreg(NQA, 2 * AH),
        vreg(len(MQ), 15),
        vreg(NP, 3, dt=u32),
        vreg(NP, 2, 2, nc2 // 4),
        vreg(2, 2 * nc2),
        vreg(NP, 2, 4),
        vreg(RING, 2 * AH),
        vreg(NP, 3),
        vreg(NX, nc2 // 4, dt=u32),
        vreg(NX, 2, 2, nc2 // 4),
        vreg(NP, 3, dt=u32),
        vreg(len(MW), 15),
        vreg(5),
        vreg(16),
        pltpu.SemaphoreType.DMA((len(KVG) + 2 + len(W2CUT),)),
    ]
    out = pl.pallas_call(
        _make_kernel(SK, W),
        out_shape=jax.ShapeDtypeStruct((1, D), A_x.dtype),
        in_specs=[pl.BlockSpec(memory_space=pl.ANY)] * 8,
        out_specs=pl.BlockSpec(memory_space=pltpu.VMEM),
        scratch_shapes=scratch,
        compiler_params=pltpu.CompilerParams(vmem_limit_bytes=126 * 1024 * 1024,
                                             disable_semaphore_checks=True),
    )(A_x.reshape(1, D), kx, vx, wqz, woz, w1z, w3z, B_w2)
    return out.reshape(1, 1, D)
```

```python
import functools
import math

import jax
import jax.numpy as jnp
from jax import lax
import jax.experimental.pallas as pl
import jax.experimental.pallas.tpu as pltpu

H, DH, D, F = 32, 192, 640, 1536
HD = H * DH
EPS = 1e-5
NA = HD // 8
AH = DH // 8
NP = H // 2
NX = 4
XP = list(range(NX))
VP = list(range(NX, NP))
BSZ = [1,1,2,2,2,1,1,1,1]
BL = [VP[sum(BSZ[:i]):sum(BSZ[:i + 1])] for i in range(len(BSZ))]
NPV = 4
PQ = VP[:NPV]
NVQ = 10
VQ = (XP + VP[NPV:])[:NVQ]
VQO = sorted(VQ, key=lambda p: 2 * p + 2.5 if p in XP else 1.5 * (VP.index(p) - NPV))
NVP = 7
VW = [5,6,9,10,11,15]
MQ = [p for p in range(NP) if p not in VQ]
MW = [p for p in range(NP) if p not in VW]
NVH = 7
NQA = 8
RING = 8
KVG = [((0, 8), (0, 5)), ((8, 12), (5, 8)), ((12, 16), (8, 12)), (None, (12, 14)), (None, (14, 16))]
W2CUT = (0, 1024, 1408, 1536)
AB = 4
SKEW = 1
VOFF = 70
VOFF2 = 20
VCOST = {"qprep": 10, "qprepv": 14, "scale": 14, "or2": 8, "woacc": 4, "gmax": 4, "gs2": 19,
         "orx": 18, "vwo": 186, "vqp": 170, "xsum": 4, "xq": 4}
CAPS = {}
RA = [0,5]
XQMAX = 4
MXF = 4
MX1 = 1.02
MXP = 1.0
PINK = 14
PINGAP = 6
PINGS = 1
SMG = 4
ORG = 4
ONLY = None
f32, bf16, u32 = jnp.float32, jnp.bfloat16, jnp.uint32


def _ln_stats(x):
    m = jnp.mean(x, axis=-1, keepdims=True)
    xc = x - m
    v = jnp.mean(xc * xc, axis=-1, keepdims=True)
    return m, lax.rsqrt(v + EPS)


def _ln_lhs(x):
    return jnp.where(lax.broadcasted_iota(jnp.int32, x.shape, 0) < 4, x, 1.0)


def _ln_fix(raw, m, r):
    return (raw - m * pltpu.roll(raw, 4, 0)) * r


def _rnd(x):
    return x.astype(bf16).astype(f32)


def _pack(lo, hi=None):
    return pltpu.bitcast(jnp.concatenate([lo, lo if hi is None else hi], axis=0).astype(bf16), u32)


def _tile(w_u32):
    return pltpu.bitcast(w_u32.reshape(64, 128), bf16)


def _mm(lhs_u32, w_u32, pin=()):
    if pin:
        lhs_u32 = jnp.concatenate([lhs_u32] + [pltpu.bitcast(x, u32) for x in pin], axis=0)
    return jnp.dot(pltpu.bitcast(lhs_u32, bf16), _tile(w_u32), preferred_element_type=f32)[0:16]


def _bc(x):
    return jnp.broadcast_to(x, (8, 128))


def _tree(op, xs):
    xs = list(xs)
    while len(xs) > 1:
        xs = [op(xs[i], xs[i + 1]) if i + 1 < len(xs) else xs[i] for i in range(0, len(xs), 2)]
    return xs[0]


def _allsub(op, x):
    for sh in (4, 2, 1):
        x = op(x, pltpu.roll(x, sh, 0))
    return x


def _recip(l):
    r = pl.reciprocal(l, approx=True)
    return r * (2.0 - l * r)


def _run(jobs):
    for j in jobs:
        j()


def _weave(main, extra, lo, hi):
    out, k = [], 0
    for n, j in enumerate(main):
        while k < len(extra) and lo * len(main) + k * (hi - lo) * len(main) / len(extra) <= n:
            out.append(extra[k])
            k += 1
        out.append(j)
    return out + list(extra[k:])


def _plan(nt):
    nb = len(BL)
    total = {"QP": 15, "QK": nt, "PM": nt, "WO": 15}
    done, fin, mxu, small = {}, {}, {}, {}

    def issue(b, kind, p, cap):
        k0 = done.get((kind, p), 0)
        n = max(min(total[kind] - k0, cap), 0)
        if n:
            mxu[b].append((kind, p, k0, k0 + n))
            done[(kind, p)] = k0 + n
            if k0 + n == total[kind]:
                fin[(kind, p)] = b
        return n

    def before(key, b):
        return fin.get(key, b) < b

    chains, qlast = {}, {}
    for p in range(NP):
        ch = ["vqp", "xq", "qprepv"] if p in VQ else ["QP", "qprep"]
        qlast[p] = ch[-1]
        if p in XP:
            ch += ["QK", "gmax", "gs2", "PM", "orx", "WO", "woacc"]
        else:
            ch += ["QK", "pv", "xmax", "scale"]
            ch += ["xcol", "vwo"] if p in VW else ["xsum", "or2", "WO", "woacc"]
        chains[p] = ch
    for p in VQO[:NVP]:
        fin[("vqp", p)] = -1
    for p in PQ:
        done[("QP", p)] = 15
        fin[("QP", p)] = fin[("qprep", p)] = -1
    done[("QK", VP[0])] = nt
    fin[("QK", VP[0])] = -1
    late = []
    b = 0
    while any((chains[p][-1], p) not in fin for p in range(NP)):
        mxu[b], small[b], late = [], late, []
        for p in VQO[NVP + b:NVP + b + 1]:
            small[b].append(("vqp", p))
            fin[("vqp", p)] = b
        for p in range(NP):
            for prev, st in zip(chains[p], chains[p][1:]):
                if st in total or (st, p) in fin or not before((prev, p), b):
                    continue
                if st == "xq" and VQO.index(p) // XQMAX > b:
                    continue
                if st == "pv":
                    if b < nb and p in BL[b]:
                        fin[(st, p)] = b
                    continue
                small[b].append((st, p))
                fin[(st, p)] = b
                if st == "gs2":
                    late.append(("xl", p))
        cap = 10 ** 6
        if b < nb:
            nab = 12 * BSZ[b] + SKEW * AB / 4 * ((b == nb - 1) - (b == 0))
            vload = (95 * nab + (31 + VOFF) * BSZ[b] - VOFF2 * (BSZ[b] - 1)
                     + sum(VCOST.get(s, 0) for s, _ in small[b]))
            cap = CAPS.get(b, 4 * int(round((vload - 147) / 32.0)))
            assert all(fin.get(("pv", p)) == b for p in BL[b])
        for p in (BL[b + 1] if b + 1 < nb else []):
            assert ("QK", p) in fin or before((qlast[p], p), b)
            cap -= issue(b, "QK", p, nt)
        for p in (BL[b + 3] if b + 3 < nb else []):
            if p not in VQ:
                cap -= issue(b, "QP", p, 15)
        cands = [("QK", p, qlast[p]) for p in (BL[b + 2] if b + 2 < nb and b in RA else [])]
        cands += [("QP", p, None) for p in XP if p not in VQ] + [("QK", p, qlast[p]) for p in XP]
        cands += [("PM", p, "gs2") for p in XP] + [("QP", p, None) for p in VP if p not in VQ]
        cands += [("WO", p, "orx" if p in XP else "or2") for p in VP + XP if p not in VW]
        cands += [("QK", p, qlast[p]) for p in VP]
        for kind, p, need in cands:
            if need is None or before((need, p), b):
                cap -= issue(b, kind, p, cap)
        b += 1
    for p in VP[RING:]:
        assert fin[("vwo" if p - RING in VW else "xsum", p - RING)] < fin[("pv", p)]
    for i in range(NQA, NVQ):
        assert fin[("xq", VQO[i - NQA])] < fin[("vqp", VQO[i])]
    return mxu, small


def _group_of(p, which):
    return next(i for i, g in enumerate(KVG) if g[which] and g[which][0] <= p < g[which][1])


def _make_kernel(SK, W):
    NC = W // 128
    NC2, NG = NC // 2, NC // 8
    qscale = DH ** -0.5 * math.log2(math.e)
    nk = sum(1 for kr, _ in KVG if kr)
    nv, nw2 = len(KVG), len(W2CUT) - 1

    def kernel(x_hbm, k_hbm, v_hbm, wq_hbm, wo_hbm, w1_hbm, w3_hbm, w2_hbm, o_ref, *scratch):
        kbs, vbs = scratch[:nk], scratch[nk:nk + nv]
        w2s = scratch[nk + nv:nk + nv + nw2]
        (wqb, wob, w1, w3, xb, xs, xrow, lx, stat, csum, qacc, qraw, lq, sraw, pbuf, st, oacc,
         otile, lp, pmraw, lo, woraw, xacc, hcol, sem) = scratch[nk + nv + nw2:]
        k32s = [r.bitcast(u32) for r in kbs]
        v32 = vbs[0].bitcast(u32)
        wq32 = wqb.bitcast(u32)
        wo32 = wob.bitcast(u32)
        wg32 = [w1.bitcast(u32), w3.bitcast(u32)]

        groups = [[(x_hbm, xb), (wq_hbm, wqb), (wo_hbm, wob)]]
        for i, (kr, vr) in enumerate(KVG):
            grp = []
            if kr:
                grp.append((k_hbm.at[kr[0] * AH:kr[1] * AH, :, pl.ds((SK - W) // 256, NC2)], kbs[i]))
            grp.append((v_hbm.at[vr[0] * 2 * AH:vr[1] * 2 * AH, pl.ds((SK - W) // 16, W // 16), :], vbs[i]))
            groups.append(grp)
        gffn = len(groups)
        groups += [[(w1_hbm, w1)], [(w3_hbm, w3)]]
        for i in range(nw2):
            groups.append([(w2_hbm.at[W2CUT[i]:W2CUT[i + 1]], w2s[i])])
        groups = [[pltpu.make_async_copy(s, d, sem.at[g]) for s, d in grp]
                  for g, grp in enumerate(groups)]
        for grp in groups:
            for cp in grp:
                cp.start()

        def gwait(g):
            for cp in groups[g]:
                cp.wait()

        sub = lax.broadcasted_iota(jnp.int32, (8, 128), 0)
        lane = lax.broadcasted_iota(jnp.int32, (8, 128), 1)

        def kvready(i):
            gwait(1 + i)
            if KVG[i][0]:
                k32 = k32s[i]

                def swap(r, carry):
                    a = k32[r, 0, :, 4:8, :]
                    b = k32[r, 1, :, 0:4, :]
                    k32[r, 0, :, 4:8, :] = b
                    k32[r, 1, :, 0:4, :] = a
                    return carry
                lax.fori_loop(0, k32.shape[0], swap, 0)

        def retile(w32, rows):
            n = w32.shape[1] // 2

            def body(rb, carry):
                r = pl.ds(rb * rows, rows)
                a = w32[r, 0:n, 4:8, :]
                b = w32[r, n:2 * n, 0:4, :]
                w32[r, 0:n, 4:8, :] = b
                w32[r, n:2 * n, 0:4, :] = a
                return carry
            lax.fori_loop(0, w32.shape[0] // rows, body, 0)

        def retile_wo(rb, carry):
            r = pl.ds(rb * 4, 4)
            vals = {(e, cc): wo32[r, 4 * (5 * e + cc):4 * (5 * e + cc) + 4, :]
                    for e in range(2) for cc in range(5)}
            for (e, cc), v in vals.items():
                wo32[r, 8 * cc + 4 * e:8 * cc + 4 * e + 4, :] = v
            return carry

        def transpose_wq(i, carry):
            c = i + jnp.where(i >= 3 * NX, 3 * NPV, 0)
            slot = (c & 1) * 24 + (c >> 1)
            ones = jnp.ones((16, 128), bf16)
            tiles = [_tile(wq32[8 * kk:8 * kk + 8, slot]) for kk in range(5)]
            csum[i] = _tree(jnp.add, [jnp.dot(ones, t, preferred_element_type=f32)[0:8] for t in tiles])
            for kk in range(5):
                wq32[8 * kk:8 * kk + 8, slot] = pltpu.bitcast(tiles[kk].T, u32).reshape(8, 8, 128)
            return carry

        def transpose_v(i, carry):
            a0 = pl.multiple_of((i >> 2) * 16, 16)
            for u in range(4):
                c2 = (i & 3) * 4 + u
                x = vbs[0][pl.ds(a0, 16), pl.ds(pl.multiple_of(c2 * 16, 16), 16), :]
                ts = [x[:, 8 * h:8 * h + 8, :].reshape(128, 128).T for h in range(2)]
                for h in range(2):
                    v32[pl.ds(a0 + 8 * h, 8), pl.ds(pl.multiple_of(c2 * 8, 8), 8), :] = (
                        pltpu.bitcast(ts[h], u32).reshape(8, 8, 128))
            return carry

        gwait(0)
        retile(wq32, 1)
        lax.fori_loop(0, HD // 64, retile_wo, 0)
        if NVQ:
            lax.fori_loop(0, 3 * NVQ, transpose_wq, 0)
        kvready(0)
        lax.fori_loop(0, NX * 3 * NC2 // 4, transpose_v, 0)

        def wq_slot(p, t):
            c = 3 * p + t
            return (c & 1) * 24 + (c >> 1)

        def qp_job(p, k, pin=tuple):
            kk, t = divmod(k, 3)
            qraw[MQ.index(p), 5 * t + kk] = _mm(
                lx[kk], wq32[8 * kk:8 * kk + 8, wq_slot(p, t)], pin())[0:8]

        def keep_rows(dst, t, c, r):
            g, j = divmod(c, 8)
            if t < 2:
                dst[0, t, g, j:j + 1, :] = r[j:j + 1]
            if t > 0:
                dst[1, t - 1, g, j:j + 1, :] = r[8 + j:9 + j]

        def qk_job(p, k, pin=tuple):
            t, c = divmod(k, NC)
            g = _group_of(p, 0)
            r0 = (p - KVG[g][0][0]) * AH + 8 * t
            keep_rows(sraw.at[p], t, c, _mm(lq[p, t], k32s[g][r0:r0 + 8, c & 1, c >> 1], pin()))

        def pm_job(p, k, pin=tuple):
            t, c = divmod(k, NC)
            a0 = p * 2 * AH + 16 * t + 8 * (c & 1)
            w = v32[a0:a0 + 8, 8 * (c >> 1):8 * (c >> 1) + 8, :]
            keep_rows(pmraw.at[p], t, c, _mm(lp[p, c // 8], w, pin()))

        def wo_job(p, k, pin=tuple):
            t, cc = divmod(k, 5)
            r0 = 24 * p + 8 * t
            woraw[MW.index(p), k] = _mm(lo[p, t], wo32[r0:r0 + 8, 8 * cc:8 * cc + 8, :], pin())[0:8]

        def lane_sums(p, src):
            for a in range(2 * AH):
                r = _bc(jnp.sum(src(a), axis=1, keepdims=True))
                t, k = divmod(a, 16)
                otile[p, t, :, 8 * k:8 * k + 8] = r[:, 8 * k:8 * k + 8]

        def xq(p):
            lane_sums(p, lambda a: qacc[VQO.index(p) % NQA, a])

        def xmax(p):
            for e in range(2):
                st[p, e, 2] = _bc(jnp.max(st[p, e, 0], axis=1, keepdims=True))

        def xl(p):
            for e in range(2):
                st[p, e, 3] = _bc(jnp.sum(st[p, e, 1], axis=1, keepdims=True))

        def xsum(p):
            xl(p)
            lane_sums(p, lambda a: oacc[p % RING, a])

        def xcol(p):
            xl(p)
            for a in range(2 * AH):
                oacc[p % RING, a] = _bc(jnp.sum(oacc[p % RING, a], axis=1, keepdims=True))

        def store_lq(p, t, q):
            qp = _pack(q)
            if t == 1:
                qp = jnp.where((lane >> 6) == (sub >> 2), qp, jnp.uint32(0))
            lq[p, t] = qp

        def qprep(p):
            for t in range(3):
                qv = _tree(jnp.add, [qraw[MQ.index(p), 5 * t + kk] for kk in range(5)])
                store_lq(p, t, _bc(_ln_fix(qv, stat[0], stat[1])[0:1]))

        def vqp_jobs(p):
            def job(i, kk, env):
                w = jnp.stack([wq32[8 * kk + i, wq_slot(p, t)] for t in range(3)])
                w = pltpu.bitcast(w.reshape(24, 128), bf16).astype(f32).reshape(3, 2, 8, 128)
                t_ = w * xrow[kk]
                env["acc"] = t_ if kk == 0 else env["acc"] + t_
                if kk == 4:
                    for t in range(3):
                        qacc[VQO.index(p) % NQA, 16 * t + 2 * i:16 * t + 2 * i + 2] = env["acc"][t]
            jobs = []
            for i in range(8):
                env = {}
                jobs += [functools.partial(job, i, kk, env) for kk in range(5)]
            return jobs

        def qprepv(p):
            for t in range(3):
                raw = _allsub(jnp.add, jnp.where((lane & 7) == sub, otile[p, t], 0.0))
                store_lq(p, t, (raw - stat[0] * csum[3 * VQ.index(p) + t]) * stat[1])

        def scores(p, e):
            return [sraw[p, e, 0, g] + sraw[p, e, 1, g] for g in range(NG)]

        def gmax(p):
            for e in range(2):
                mv = _tree(jnp.maximum, scores(p, e))
                st[p, e, 2] = _bc(jnp.max(mv, axis=1, keepdims=True))

        def probs(p, e):
            m = _allsub(jnp.maximum, st[p, e, 2])
            return [jnp.exp2(x - m) for x in scores(p, e)]

        def sm_jobs(p, e):
            env = {}

            def head():
                s = scores(p, e)
                mv = _allsub(jnp.maximum, _tree(jnp.maximum, s))
                st[p, e, 0] = mv
                env["p"] = [jnp.exp2(x - mv) for x in s]

            def spread(c0):
                for c in range(c0, c0 + SMG):
                    pbuf[e, c] = _bc(env["p"][c // 8][c % 8:c % 8 + 1])

            def lsum():
                st[p, e, 1] = _allsub(jnp.add, _tree(jnp.add, env["p"]))
            return [head] + [functools.partial(spread, c0) for c0 in range(0, NC, SMG)] + [lsum]

        def pv_jobs(p, e):
            g = _group_of(p, 1)

            def job(a0, c2, env):
                a = (p - KVG[g][1][0]) * 2 * AH + e * AH + a0
                v = vbs[g][a:a + AB, 16 * c2:16 * c2 + 16, :].astype(f32)
                t = v[:, 0:8] * pbuf[e, 2 * c2] + v[:, 8:16] * pbuf[e, 2 * c2 + 1]
                env["acc"] = t if c2 == 0 else env["acc"] + t
                if c2 == NC2 - 1:
                    oacc[p % RING, e * AH + a0:e * AH + a0 + AB] = env["acc"]
            jobs = []
            for a0 in range(0, AH, AB):
                env = {}
                jobs += [functools.partial(job, a0, c2, env) for c2 in range(NC2)]
            return jobs

        def scale_jobs(p):
            def head(e, env):
                env["w"] = jnp.exp2(st[p, e, 0] - st[p, e, 2])
                st[p, e, 1] = env["w"] * st[p, e, 1]

            def job(a, env):
                oacc[p % RING, a:a + ORG] = oacc[p % RING, a:a + ORG] * env["w"]
            jobs = []
            for e in range(2):
                env = {}
                jobs.append(functools.partial(head, e, env))
                jobs += [functools.partial(job, e * AH + a, env) for a in range(0, AH, ORG)]
            return jobs

        def store_lo(p, tiles):
            inv = [_recip(st[p, e, 3]) for e in range(2)]
            invs = [inv[0], jnp.where(lane < 64, inv[0], inv[1]), inv[1]]
            for t in range(3):
                lo[p, t] = _pack(jnp.where((lane & 7) == sub, tiles[t] * invs[t], 0.0))

        def or2(p):
            store_lo(p, [otile[p, t] for t in range(3)])

        def gs2(p):
            ps = [probs(p, e) for e in range(2)]
            for e in range(2):
                st[p, e, 1] = _allsub(jnp.add, _tree(jnp.add, ps[e]))
            for g in range(NG):
                lp[p, g] = _pack(ps[0][g], ps[1][g])

        def orx(p):
            def part(e, t):
                return _tree(jnp.add, [pmraw[p, e, t, g] for g in range(NG)])
            tiles = [part(0, 0), jnp.where(lane < 64, part(0, 1), part(1, 0)), part(1, 1)]
            store_lo(p, [_allsub(jnp.add, x) for x in tiles])

        def woacc(p):
            raw = woraw.at[MW.index(p)]
            xacc[...] = xacc[...] + (raw[0:5] + raw[5:10] + raw[10:15])

        def vwo_jobs(p):
            def job(e, r, env):
                w = pltpu.bitcast(wo32[24 * p + 12 * e + r], bf16).astype(f32).reshape(5, 16, 128)
                a = e * AH + 2 * r
                t = w[:, 0:8] * oacc[p % RING, a] + w[:, 8:16] * oacc[p % RING, a + 1]
                env["acc"] = t if r == 0 else env["acc"] + t
                if r == AH // 2 - 1:
                    xacc[...] = xacc[...] + env["acc"] * _recip(st[p, e, 3])
            jobs = []
            for e in range(2):
                env = {}
                jobs += [functools.partial(job, e, r, env) for r in range(AH // 2)]
            return jobs

        mxu_fn = {"QP": qp_job, "QK": qk_job, "PM": pm_job, "WO": wo_job}
        xlu_fn = {"xq": xq, "gmax": gmax, "xmax": xmax, "xl": xl, "xsum": xsum, "xcol": xcol}
        valu_fn = {"qprep": qprep, "qprepv": qprepv, "or2": or2, "gs2": gs2, "orx": orx,
                   "woacc": woacc}
        plan_mxu, plan_small = _plan(3 * NC)

        def jobs_of(b):
            mx = [functools.partial(mxu_fn[kind], p, k)
                  for kind, p, k0, k1 in plan_mxu[b] for k in range(k0, k1)]
            xj = [functools.partial(xlu_fn[s], p) for s, p in plan_small[b] if s in xlu_fn]
            vj = [functools.partial(valu_fn[s], p) for s, p in plan_small[b] if s in valu_fn]
            sc = [j for s, p in plan_small[b] if s == "scale" for j in scale_jobs(p)]
            vw = [j for s, p in plan_small[b] if s == "vwo" for j in vwo_jobs(p)]
            vw += [j for s, p in plan_small[b] if s == "vqp" for j in vqp_jobs(p)]
            return mx, xj, vj, sc, vw

        def block(b):
            mx, xj, vj, sc, vw = jobs_of(b)
            valu = []
            for n, p in enumerate(BL[b]):
                sa, sb = sm_jobs(p, 0), sm_jobs(p, 1)
                pa, pb = pv_jobs(p, 0), pv_jobs(p, 1)
                cut = len(pb) - SKEW * NC2
                if p != VP[-1]:
                    pb = pb[:cut]
                if p != VP[0]:
                    valu += _weave(pv_jobs(p - 1, 1)[cut:], sa, 0.0, 0.9) + pa[:NC2]
                else:
                    valu += sa[:3] + _weave(pa[:NC2], sa[3:], 0.0, 1.0 - 1.0 * SMG / NC)
                valu += _weave(pa[NC2:], sb, 0.1, 0.8)
                if n == 0:
                    valu += vw + (_weave(pb, vj + sc, 0.0, 0.9) if vj + sc else pb)
                else:
                    valu += pb
            k = PINK
            for s, q in plan_small[b]:
                refs = []
                if s in ("xsum", "xl", "xmax", "gmax", "xcol"):
                    refs += [(st.at[q, e, 2 if "max" in s else 3], PINGS) for e in range(2)]
                if s in ("xsum", "xq"):
                    refs += [(otile.at[q, t], PINGAP) for t in range(3)]
                for ref, gap in refs:
                    k += gap
                    mx[k] = functools.partial(mx[k], pin=lambda ref=ref: (ref[...],))
            _run(mx[:MXF] + xj + _weave(valu, mx[MXF:], 0.0, MX1))

        def set_x(x):
            xs[...] = x
            xl_ = _ln_lhs(x)
            for kk in range(5):
                xrow[kk] = x[:, 128 * kk:128 * kk + 128]
                lx[kk] = _pack(xl_[:, 128 * kk:128 * kk + 128])

        def prologue():
            def stats():
                m, r = _ln_stats(xs[...])
                stat[0] = _bc(m)
                stat[1] = _bc(r * qscale)
                xacc[...] = jnp.zeros_like(xacc)
            mx = [stats]
            for p in PQ:
                mx += [functools.partial(qp_job, p, k) for k in range(15)]
                mx.append(functools.partial(qprep, p))
            mx += [functools.partial(qk_job, VP[0], k) for k in range(3 * NC)]
            bulk = [j for p in VQO[:NVP] for j in vqp_jobs(p)]
            _run(mx[:MXF + 1] + _weave(bulk, mx[MXF + 1:], 0.0, MXP) if bulk else mx)

        def finish_layer(first):
            for b in range(len(BL), len(plan_mxu)):
                mx, xj, vj, sc, vw = jobs_of(b)
                _run(xj + sc + vj + vw + mx)
            att = jnp.sum(jnp.concatenate([xacc[cc] for cc in range(5)], axis=1),
                          axis=0, keepdims=True)
            x1 = _rnd(xs[...] + _rnd(att))
            if first:
                xs[...] = x1
                for i in range(2):
                    gwait(gffn + i)
                    retile(wg32[i], 4)
                x1 = xs[...]
            m, r = _ln_stats(x1)
            xl_ = _ln_lhs(x1)
            lf = [_pack(xl_[:, 128 * kk:128 * kk + 128]) for kk in range(5)]
            nh = F // 128
            on_vpu = range(W2CUT[-2] // 128, nh) if first else range(NVH)

            def w2rows(j):
                i = next(i for i in range(nw2) if W2CUT[i] <= 128 * j < W2CUT[i + 1])
                return w2s[i][128 * j - W2CUT[i]:128 * j - W2CUT[i] + 128, :]

            def tile_dot(lhs, w):
                return jnp.dot(pltpu.bitcast(lhs, bf16), w, preferred_element_type=f32)[0:8]

            def gate_up(j):
                slot = (j & 1) * (nh // 2) + (j >> 1)
                parts = [[tile_dot(lf[kk], _tile(wg32[i][8 * kk:8 * kk + 8, slot])) for i in range(2)]
                         for kk in range(5)]
                g, u = [_ln_fix(_tree(jnp.add, [pp[i] for pp in parts]), m, r) for i in range(2)]
                return _rnd(g * jax.nn.sigmoid(g) * u)

            def hcols(h):
                hb = _bc(h[0:1])
                return [_bc(jnp.sum(jnp.where(lane == 8 * a + sub, hb, 0.0), axis=1, keepdims=True))
                        for a in range(16)]

            def vpu_rows(j, cols, yv):
                w = w2rows(j).astype(f32)
                for a in range(16):
                    t = w[8 * a:8 * a + 8] * jnp.tile(cols[a], (1, 5))
                    yv = t if yv is None else yv + t
                return yv

            hs, y, yv = [], None, None
            for j in range(nh):
                hs.append(gate_up(j))
                if j in on_vpu:
                    if first:
                        hcol[...] = jnp.stack(hcols(hs[j]))
                    else:
                        yv = vpu_rows(j, hcols(hs[j]), yv)
            for j in range(nh):
                if first and 128 * j in W2CUT:
                    i = W2CUT.index(128 * j)
                    if i:
                        xs[...] = y
                    gwait(gffn + 2 + i)
                    if i:
                        y = xs[...]
                if j not in on_vpu:
                    lh, w = _pack(hs[j]), w2rows(j)
                    t = jnp.concatenate([tile_dot(lh, w[:, 128 * cc:128 * cc + 128]) for cc in range(5)],
                                        axis=1)
                    y = t if y is None else y + t
                elif first:
                    yv = vpu_rows(j, [hcol[a] for a in range(16)], yv)
            y = y[0:1]
            if yv is not None:
                y = y + jnp.sum(yv, axis=0, keepdims=True)
            if first:
                set_x(_rnd(x1 + _rnd(y)))
            else:
                o_ref[...] = (x1[0:1] + _rnd(y)).astype(o_ref.dtype)

        def layer_body(layer, carry):
            first = layer == 0
            prologue()
            seen = 1
            for b in range(len(BL)):
                need = 1 + max([_group_of(BL[b][-1], 1)] + [_group_of(p, 0) for kind, p, _, _ in plan_mxu[b]
                                                        if kind == "QK"])
                if need > seen:
                    @pl.when(first)
                    def _(lo_=seen, hi_=need):
                        for i in range(lo_, hi_):
                            kvready(i)
                    seen = need
                if ONLY is None or b in ONLY:
                    pl.when(layer < 100 + b)(functools.partial(block, b))
            lax.cond(first, lambda: finish_layer(True), lambda: finish_layer(False))
            return carry

        set_x(jnp.broadcast_to(xb[...].astype(f32), (8, D)))
        lax.fori_loop(0, 2, layer_body, 0)
    return kernel


def _tile_linear(c):
    sk = c.shape[2]
    return (jnp.swapaxes(c, 2, 3).reshape(NA, 8, sk // 128, 128)
            .transpose(0, 2, 1, 3).reshape(NA, sk // 16, 128))


@jax.jit
def pallas_interleave_layers__sliding_block_cached__glu_gated_swiglu__decode_kernel(
    A_x: jax.Array,
    A_k_cache: jax.Array,
    A_v_cache: jax.Array,
    A_wq: jax.Array,
    A_wo: jax.Array,
    B_x: jax.Array,
    B_w1: jax.Array,
    B_w3: jax.Array,
    B_w2: jax.Array,
):
    SK = A_k_cache.shape[2]
    W = min(4096, max(256, SK // 4))
    nc2 = W // 256
    kx = _tile_linear(A_k_cache).reshape(NA // 2, 2, SK // 256, 16, 128)
    vx = _tile_linear(A_v_cache)
    wqz, w1z, w3z = [(w.reshape(D // 16, 2, 8, w.shape[1] // 256, 2, 128).transpose(0, 1, 3, 4, 2, 5)
                      .reshape(D // 16, w.shape[1] // 128, 16, 128)) for w in (A_wq, B_w1, B_w3)]
    woz = (A_wo.reshape(HD // 16, 2, 8, 5, 128).transpose(0, 1, 3, 2, 4)
           .reshape(HD // 16, 80, 128))
    vreg = lambda *lead, dt=f32: pltpu.VMEM(lead + (8, 128), dt)
    scratch = [pltpu.VMEM(((kr[1] - kr[0]) * AH, 2, nc2, 16, 128), bf16) for kr, _ in KVG if kr]
    scratch += [pltpu.VMEM(((vr[1] - vr[0]) * 2 * AH, W // 16, 128), bf16) for _, vr in KVG]
    scratch += [pltpu.VMEM((b - a, D), bf16) for a, b in zip(W2CUT, W2CUT[1:])]
    scratch += [
        pltpu.VMEM((D // 16, 48, 16, 128), bf16),
        pltpu.VMEM((HD // 16, 80, 128), bf16),
        pltpu.VMEM((D // 16, F // 128, 16, 128), bf16),
        pltpu.VMEM((D // 16, F // 128, 16, 128), bf16),
        pltpu.VMEM((1, D), bf16),
        pltpu.VMEM((8, D), f32),
        vreg(5),
        vreg(5, dt=u32),
        vreg(2),
        vreg(max(3 * NVQ, 1)),
        vreg(NQA, 2 * AH),
        vreg(len(MQ), 15),
        vreg(NP, 3, dt=u32),
        vreg(NP, 2, 2, nc2 // 4),
        vreg(2, 2 * nc2),
        vreg(NP, 2, 4),
        vreg(RING, 2 * AH),
        vreg(NP, 3),
        vreg(NX, nc2 // 4, dt=u32),
        vreg(NX, 2, 2, nc2 // 4),
        vreg(NP, 3, dt=u32),
        vreg(len(MW), 15),
        vreg(5),
        vreg(16),
        pltpu.SemaphoreType.DMA((len(KVG) + 2 + len(W2CUT),)),
    ]
    out = pl.pallas_call(
        _make_kernel(SK, W),
        out_shape=jax.ShapeDtypeStruct((1, D), A_x.dtype),
        in_specs=[pl.BlockSpec(memory_space=pl.ANY)] * 8,
        out_specs=pl.BlockSpec(memory_space=pltpu.VMEM),
        scratch_shapes=scratch,
        compiler_params=pltpu.CompilerParams(vmem_limit_bytes=126 * 1024 * 1024,
                                             disable_semaphore_checks=True),
    )(A_x.reshape(1, D), kx, vx, wqz, woz, w1z, w3z, B_w2)
    return out.reshape(1, 1, D)
```
